```python
import os as _os
_os.environ.setdefault('JAX_PLATFORMS', 'cpu')
import jax
import jax.numpy as jnp

def _softmax(x, axis=-1):
    return jax.nn.softmax(x, axis=axis)

def _gelu(x):
    return jax.nn.gelu(x, approximate=True)

def _silu(x):
    return jax.nn.silu(x)

def _sigmoid(x):
    return jax.nn.sigmoid(x)

def _layernorm(x, axis=-1, eps=1e-05):
    m = jnp.mean(x, axis=axis, keepdims=True)
    v = jnp.var(x, axis=axis, keepdims=True)
    return (x - m) / jnp.sqrt(v + eps)

def _scatter_add(tgt, idx, src, axis=0):
    return tgt.at[idx].add(src)

def _segment_sum(src, seg, n):
    return jax.ops.segment_sum(src, seg, n)

class _Rng:

    def __init__(self, key):
        self._k = key

    def _next(self):
        self._k, sub = jax.random.split(self._k)
        return sub

    def normal(self, shape):
        return jax.random.normal(self._next(), shape, dtype=jnp.bfloat16)

    def randint(self, lo, hi, shape):
        return jax.random.randint(self._next(), shape, lo, hi, dtype=jnp.int32)

    def uniform(self, shape, lo=0.0, hi=1.0):
        return jax.random.uniform(self._next(), shape, jnp.bfloat16, lo, hi)

    def permutation(self, n):
        return jax.random.permutation(self._next(), n)
kernel_name = 'recurrent_scan__memory_aug_recurrent_mem_tr__mixer_gmlp__prompt'

def setup_inputs():
    _rng = _Rng(jax.random.key(int.from_bytes(__import__("os").urandom(4), "little")))
    _w = lambda a: (lambda t: t.astype(jnp.bfloat16) if jnp.issubdtype(t.dtype, jnp.floating) else t)(jnp.asarray(a))

    def _A_setup():
        B, S, Dm = (1, 2048, 640)
        H, Dh = (32, 128)
        M, seg = (8, 32)
        seg = min(seg, S)
        S = S // seg * seg
        return {'x': _w((lambda *s: _rng.normal(s) * 0.05)(B, S, Dm)), 'mem0': _w((lambda *s: _rng.normal(s) * 0.1)(B, M, Dm)), 'Wq': _w((lambda *s: _rng.normal(s) * 1.6)(Dm, H, Dh) * Dm ** (-0.5)), 'Wk': _w((lambda *s: _rng.normal(s) * 1.6)(Dm, H, Dh) * Dm ** (-0.5)), 'Wv': _w((lambda *s: _rng.normal(s) * 0.1)(Dm, H, Dh) * Dm ** (-0.5)), 'Wo': _w((lambda *s: _rng.normal(s) * 0.1)(H, Dh, Dm) * (H * Dh) ** (-0.5)), 'seg_len': seg}
    _A_in = _A_setup()

    def _B_setup():
        B, S, D, F = (1, 2048, 640, 1728)
        Fh = F // 2
        return {'x': _w((lambda *s: _rng.normal(s) * 0.05)(B, S, D)), 'w_in': _w((lambda *s: _rng.normal(s) * 0.8)(D, 2 * Fh)), 'w_sp': _w(0.01 * (lambda *s: _rng.normal(s) * 0.8)(S, S)), 'b_sp': _w(1.0 + 0.01 * (lambda *s: _rng.normal(s) * 0.05)(S)), 'w_out': _w((lambda *s: _rng.normal(s) * 0.05)(Fh, D))}
    _B_in = _B_setup()
    return {'A_x': _A_in['x'], 'A_mem0': _A_in['mem0'], 'A_Wq': _A_in['Wq'], 'A_Wk': _A_in['Wk'], 'A_Wv': _A_in['Wv'], 'A_Wo': _A_in['Wo'], 'A_seg_len': _A_in['seg_len'], 'B_x': _B_in['x'], 'B_w_in': _B_in['w_in'], 'B_w_sp': _B_in['w_sp'], 'B_b_sp': _B_in['b_sp'], 'B_w_out': _B_in['w_out']}

def reference(A_x, A_mem0, A_Wq, A_Wk, A_Wv, A_Wo, A_seg_len, B_x, B_w_in, B_w_sp, B_b_sp, B_w_out):

    def _A_ref(x, mem0, Wq, Wk, Wv, Wo, seg_len):
        B, S, Dm = x.shape
        H, Dh = (Wq.shape[1], Wq.shape[2])
        M = mem0.shape[1]
        scale = Dh ** (-0.5)
        n_seg = S // seg_len
        L = M + seg_len
        idx = jnp.arange(L)
        mask = (idx[:, None] < M) | (idx[:, None] >= idx[None, :])
        mem = mem0
        outs = []
        for s in range(n_seg):
            xs = x[:, s * seg_len:(s + 1) * seg_len, :].copy()
            h = jnp.concatenate([mem, xs], axis=1)
            q = jnp.einsum('btd,dhe->bhte', h, Wq)
            k = jnp.einsum('btd,dhe->bhte', h, Wk)
            v = jnp.einsum('btd,dhe->bhte', h, Wv)
            scores = jnp.einsum('bhqe,bhke->bhqk', q, k) * scale
            scores = jnp.where(mask[None, None], scores, -1000000000.0)
            p = _softmax(scores, axis=-1)
            o = jnp.einsum('bhqk,bhke->bhqe', p, v)
            o = jnp.einsum('bhte,hed->btd', o, Wo)
            mem = o[:, :M, :].copy()
            outs.append(o[:, M:, :])
        return jnp.concatenate(outs, axis=1)

    def _B_ref(x, w_in, w_sp, b_sp, w_out):
        B, S, D = x.shape
        F = w_in.shape[-1]
        Fh = F // 2
        z = _gelu(jnp.einsum('bsd,df->bsf', x, w_in))
        z1 = z[..., :Fh].copy()
        z2 = _layernorm(z[..., Fh:], axis=-1)
        g = jnp.einsum('ts,bsf->btf', w_sp, z2) + b_sp[None, :, None]
        return jnp.einsum('bsf,fd->bsd', z1 * g, w_out)
    x = A_x
    xn = _layernorm(x, axis=-1)
    s = _A_ref(xn, A_mem0, A_Wq, A_Wk, A_Wv, A_Wo, A_seg_len)
    g = _silu(_B_ref(xn, B_w_in, B_w_sp, B_b_sp, B_w_out))
    return x + s * g
```

```python
import jax
import jax.numpy as jnp
import jax.experimental.pallas as pl
import jax.experimental.pallas.tpu as pltpu

F32 = jnp.float32
BF16 = jnp.bfloat16
U32 = jnp.uint32

S = 2048
DM = 640
H = 32
DH = 128
MEM = 8
SEG = 32
FH = 864
NPAIR = S // (2 * SEG)
EPS = 1e-5
SCALE = DH ** (-0.5)
NEG = -1000000000.0

BCH = 256
NBCH = S // BCH
LAG_S = 2
LAG_O = 5
WG = 4

NT = (((1,), (1,)), ((), ()))


def _as_bf16(u):
    return pltpu.bitcast(u, BF16)


def _as_u32(b):
    return pltpu.bitcast(b, U32)


def _layernorm(v):
    m = jnp.mean(v, axis=-1, keepdims=True)
    c = v - m
    var = jnp.mean(c * c, axis=-1, keepdims=True)
    return c * jax.lax.rsqrt(var + EPS)


def _masks():
    r = jax.lax.broadcasted_iota(jnp.int32, (32, 48), 0)
    c = jax.lax.broadcasted_iota(jnp.int32, (32, 48), 1)
    in_e = c < 40
    keep_e = in_e & ((r < MEM) | (r >= c))
    fill_e = jnp.where(in_e, NEG, -jnp.inf).astype(F32)
    r = jax.lax.broadcasted_iota(jnp.int32, (48, 80), 0)
    c = jax.lax.broadcasted_iota(jnp.int32, (48, 80), 1)
    q_t0 = (r >= 32) & (r < 40)
    qpos = jnp.where(r < MEM, r, jnp.where(r < 32, r + 8, jnp.where(r < 40, r, r - 32)))
    k_t0 = (c >= 32) & (c < 72)
    kpos = jnp.where(c < MEM, c, jnp.where(c < 32, c + 8, jnp.where(c < 72, c - 32, c - 64)))
    in_o = jnp.where(q_t0, 1, 0) == jnp.where(k_t0, 1, 0)
    keep_o = in_o & ((qpos < MEM) | (qpos >= kpos))
    fill_o = jnp.where(in_o, NEG, -jnp.inf).astype(F32)
    return keep_e, fill_e, keep_o, fill_o


def _kernel(x_hbm, mem0_ref, wq_hbm, wk_hbm, wv_hbm, wo_hbm, wint_hbm, wsp_hbm,
            bsp_ref, wout_hbm, out_hbm,
            x_v, xn_v, wint_v, wsp_v, wout_v, stage_v, wqkv_v, wo_v,
            z1_v, z2_v, gate_v, kst_v, vst_v, o_v, out_v,
            sem_x, sem_w, sem_st, sem_out):
    def x_copy(i):
        return pltpu.make_async_copy(x_hbm.at[pl.ds(i * BCH, BCH), :],
                                     x_v.at[pl.ds(i * BCH, BCH), :], sem_x.at[i])

    wint_cp = pltpu.make_async_copy(wint_hbm.bitcast(U32), wint_v, sem_w.at[0])
    wsp_cp = pltpu.make_async_copy(wsp_hbm.bitcast(U32), wsp_v, sem_w.at[1])
    wout_cp = pltpu.make_async_copy(wout_hbm.bitcast(U32), wout_v, sem_w.at[2])
    wo_cp = pltpu.make_async_copy(wo_hbm.bitcast(U32), wo_v, sem_w.at[3])
    w_hbms = (wq_hbm, wk_hbm, wv_hbm)

    def stage_copy(m, j):
        return pltpu.make_async_copy(w_hbms[m].bitcast(U32).at[:, j, :],
                                     stage_v.at[m * 16 + j], sem_st.at[m * 16 + j])

    x_copy(0).start()
    wint_cp.start()
    for i in range(1, NBCH):
        x_copy(i).start()
    wsp_cp.start()
    wout_cp.start()
    for m in range(3):
        for j in range(16):
            stage_copy(m, j).start()
    wo_cp.start()

    wint_cp.wait()

    def b1_body(i, carry):
        r0 = pl.multiple_of(i * BCH, BCH)
        h0 = pl.multiple_of(i * (BCH // 2), BCH // 2)
        pltpu.make_async_copy(x_hbm.at[pl.ds(r0, BCH), :], x_v.at[pl.ds(r0, BCH), :],
                              sem_x.at[i]).wait()
        xn = _layernorm(x_v[pl.ds(r0, BCH), :].astype(F32)).astype(BF16)
        xn_v[pl.ds(h0, BCH // 2), :] = _as_u32(xn)
        z1 = jax.lax.dot_general(xn, _as_bf16(wint_v[0:FH // 2, :]), NT,
                                 preferred_element_type=F32)
        z1_v[pl.ds(h0, BCH // 2), :] = _as_u32(jax.nn.gelu(z1, approximate=True).astype(BF16))
        z2 = jax.lax.dot_general(xn, _as_bf16(wint_v[FH // 2:FH, :]), NT,
                                 preferred_element_type=F32)
        z2 = _layernorm(jax.nn.gelu(z2, approximate=True))
        z2_v[pl.ds(h0, BCH // 2), :] = _as_u32(z2.astype(BF16))
        return carry

    jax.lax.fori_loop(0, NBCH, b1_body, 0)

    wsp_cp.wait()
    wout_cp.wait()
    eye = (jax.lax.broadcasted_iota(jnp.int32, (128, 128), 0)
           == jax.lax.broadcasted_iota(jnp.int32, (128, 128), 1))

    def unpack(p):
        w = stage_v[p]
        lo = pltpu.bitcast(w << 16, F32).astype(BF16)
        hi = pltpu.bitcast(w & jnp.uint32(0xFFFF0000), F32).astype(BF16)
        wqkv_v[2 * p] = _as_u32(lo)
        wqkv_v[2 * p + 1] = _as_u32(hi)

    def b2_body(i, carry):
        r0 = pl.multiple_of(i * BCH, BCH)
        h0 = pl.multiple_of(i * (BCH // 2), BCH // 2)
        bs = bsp_ref[...].astype(F32)
        sel = jax.lax.broadcasted_iota(jnp.int32, (16, 128), 0)
        cols = []
        for c in range(BCH // 128):
            brow = jnp.sum(jnp.where(sel == i * (BCH // 128) + c, bs, 0.0), axis=0, keepdims=True)
            cols.append(jnp.sum(jnp.where(eye, brow, 0.0), axis=1, keepdims=True))
        bcol = jnp.concatenate(cols, axis=0)
        g = jnp.dot(_as_bf16(wsp_v[pl.ds(h0, BCH // 2), :]), _as_bf16(z2_v[...]),
                    preferred_element_type=F32) + bcol
        u = (_as_bf16(z1_v[pl.ds(h0, BCH // 2), :]).astype(F32) * g).astype(BF16)
        bo = jnp.dot(u, _as_bf16(wout_v[...]), preferred_element_type=F32)
        gate_v[pl.ds(r0, BCH), :] = bo * jax.nn.sigmoid(bo)
        for jj in range(48 // NBCH):
            p = i * (48 // NBCH) + jj
            pltpu.make_async_copy(stage_v.at[p], stage_v.at[p], sem_st.at[p]).wait()
            unpack(p)
        return carry

    jax.lax.fori_loop(0, NBCH, b2_body, 0)
    wo_cp.wait()

    keep_e, fill_e, keep_o, fill_o = _masks()

    def step(hq, hkv, odd):
        keep, fill = (keep_o, fill_o) if odd else (keep_e, fill_e)
        rows = hq.shape[0]
        qs, ks, vs, ps = {}, {}, {}, {}
        acc = None
        nslots = H + H // WG
        for t in range(nslots):
            if t < H:
                qs[t] = jnp.dot(hq, _as_bf16(wqkv_v[t]), preferred_element_type=F32).astype(BF16)
                k = jnp.dot(hkv, _as_bf16(wqkv_v[H + t]), preferred_element_type=F32).astype(BF16)
                v = jnp.dot(hkv, _as_bf16(wqkv_v[2 * H + t]), preferred_element_type=F32).astype(BF16)
                if odd:
                    k = jnp.concatenate([k, _as_bf16(kst_v[t])], axis=0)
                    v = jnp.concatenate([v, _as_bf16(vst_v[t])], axis=0)
                else:
                    kst_v[t] = _as_u32(k)
                    vst_v[t] = _as_u32(v)
                ks[t], vs[t] = k, v
            else:
                g = t - H
                og = _as_bf16(o_v[0:rows // 2, g * WG * DH:(g + 1) * WG * DH])
                part = jnp.dot(og, _as_bf16(wo_v[g * WG * DH // 2:(g + 1) * WG * DH // 2, :]),
                               preferred_element_type=F32)
                acc = part if acc is None else acc + part
            hs = t - LAG_S
            if 0 <= hs < H:
                sc = jax.lax.dot_general(qs.pop(hs), ks.pop(hs), NT,
                                         preferred_element_type=F32) * SCALE
                sc = jnp.where(keep, sc, fill)
                e = jnp.exp(sc - jnp.max(sc, axis=-1, keepdims=True))
                inv = 1.0 / jnp.sum(e, axis=-1, keepdims=True)
                ps[hs] = (e.astype(BF16), inv)
            ho = t - LAG_O
            if 0 <= ho < H:
                e, inv = ps.pop(ho)
                o = jnp.dot(e, vs.pop(ho), preferred_element_type=F32) * inv
                o_v[0:rows // 2, ho * DH:(ho + 1) * DH] = _as_u32(o.astype(BF16))
        return acc

    def pair_body(i, mem):
        r0 = pl.multiple_of(i * 64, 64)
        h0 = pl.multiple_of(i * 32, 32)
        xs = _as_bf16(xn_v[pl.ds(h0, 32), :]).astype(F32)
        hkv_e = jnp.concatenate([mem, xs[0:40]], axis=0).astype(BF16)
        acc_e = step(hkv_e[0:32], hkv_e, odd=False)
        mem_o = acc_e[0:MEM]
        hq_o = jnp.concatenate([mem_o, xs[40:64], xs[24:40]], axis=0).astype(BF16)
        acc_o = step(hq_o, hq_o[0:32], odd=True)
        s_rows = jnp.concatenate([acc_e[8:32], acc_o[32:48], acc_o[8:32]], axis=0)
        res = x_v[pl.ds(r0, 64), :].astype(F32) + s_rows * gate_v[pl.ds(r0, 64), :]
        out_v[pl.ds(r0, 64), :] = res.astype(BF16)
        pltpu.make_async_copy(out_v.at[pl.ds(r0, 64), :], out_hbm.at[pl.ds(r0, 64), :],
                              sem_out).start()
        return acc_o[0:MEM]

    jax.lax.fori_loop(0, NPAIR, pair_body, mem0_ref[...].astype(F32))
    pltpu.make_async_copy(out_v, out_hbm, sem_out).wait()


@jax.jit
def pallas_recurrent_scan__memory_aug_recurrent_mem_tr__mixer_gmlp__prompt_kernel(
    A_x: jax.Array,
    A_mem0: jax.Array,
    A_Wq: jax.Array,
    A_Wk: jax.Array,
    A_Wv: jax.Array,
    A_Wo: jax.Array,
    A_seg_len: jax.Array,
    B_x: jax.Array,
    B_w_in: jax.Array,
    B_w_sp: jax.Array,
    B_b_sp: jax.Array,
    B_w_out: jax.Array,
):
    del A_seg_len, B_x
    hbm = pl.BlockSpec(memory_space=pl.ANY)
    vmem = pl.BlockSpec(memory_space=pltpu.VMEM)
    out = pl.pallas_call(
        _kernel,
        out_shape=jax.ShapeDtypeStruct((S, DM), BF16),
        in_specs=[hbm, vmem, hbm, hbm, hbm, hbm, hbm, hbm, vmem, hbm],
        out_specs=hbm,
        scratch_shapes=[
            pltpu.VMEM((S, DM), BF16),
            pltpu.VMEM((S // 2, DM), U32),
            pltpu.VMEM((FH, DM), U32),
            pltpu.VMEM((S // 2, S), U32),
            pltpu.VMEM((FH // 2, DM), U32),
            pltpu.VMEM((48, DM, DH), U32),
            pltpu.VMEM((3 * H, DM // 2, DH), U32),
            pltpu.VMEM((H * DH // 2, DM), U32),
            pltpu.VMEM((S // 2, FH), U32),
            pltpu.VMEM((S // 2, FH), U32),
            pltpu.VMEM((S, DM), F32),
            pltpu.VMEM((H, 24, DH), U32),
            pltpu.VMEM((H, 24, DH), U32),
            pltpu.VMEM((24, H * DH), U32),
            pltpu.VMEM((S, DM), BF16),
            pltpu.SemaphoreType.DMA((NBCH,)),
            pltpu.SemaphoreType.DMA((4,)),
            pltpu.SemaphoreType.DMA((48,)),
            pltpu.SemaphoreType.DMA,
        ],
        compiler_params=pltpu.CompilerParams(vmem_limit_bytes=110 * 1024 * 1024),
    )(
        A_x.reshape(S, DM),
        A_mem0.reshape(MEM, DM),
        A_Wq, A_Wk, A_Wv,
        A_Wo.reshape(H * DH, DM),
        B_w_in.T,
        B_w_sp,
        B_b_sp.reshape(16, 128),
        B_w_out,
    )
    return out.reshape(1, S, DM)
```

```python
import jax
import jax.numpy as jnp
import jax.experimental.pallas as pl
import jax.experimental.pallas.tpu as pltpu

F32 = jnp.float32
BF16 = jnp.bfloat16
U32 = jnp.uint32

S = 2048
DM = 640
H = 32
DH = 128
MEM = 8
SEG = 32
FH = 864
NPAIR = S // (2 * SEG)
NTILE = S // 128
EPS = 1e-5
SCALE = DH ** (-0.5)
NEG = -1000000000.0

XCH = 256
T1 = 4
T2 = 4
RB = 144
LAG_S = 2
LAG_O = 6
WG = 4
GSPLIT = 128
WIN_PIECES = (2, 4, 6)

NT = (((1,), (1,)), ((), ()))


def _as_bf16(u):
    return pltpu.bitcast(u, BF16)


def _as_u32(b):
    return pltpu.bitcast(b, U32)


def _layernorm(v):
    m = jnp.mean(v, axis=-1, keepdims=True)
    c = v - m
    var = jnp.mean(c * c, axis=-1, keepdims=True)
    return c * jax.lax.rsqrt(var + EPS)


def _gelu(v):
    return jax.nn.gelu(v, approximate=True)


def _mult(v, m):
    return v if isinstance(v, int) else pl.multiple_of(v, m)


def _masks():
    r = jax.lax.broadcasted_iota(jnp.int32, (32, 48), 0)
    c = jax.lax.broadcasted_iota(jnp.int32, (32, 48), 1)
    in_e = c < 40
    keep_e = in_e & ((r < MEM) | (r >= c))
    fill_e = jnp.where(in_e, NEG, -jnp.inf).astype(F32)
    r = jax.lax.broadcasted_iota(jnp.int32, (48, 80), 0)
    c = jax.lax.broadcasted_iota(jnp.int32, (48, 80), 1)
    q_t0 = (r >= 32) & (r < 40)
    qpos = jnp.where(r < MEM, r, jnp.where(r < 32, r + 8, jnp.where(r < 40, r, r - 32)))
    k_t0 = (c >= 32) & (c < 72)
    kpos = jnp.where(c < MEM, c, jnp.where(c < 32, c + 8, jnp.where(c < 72, c - 32, c - 64)))
    in_o = jnp.where(q_t0, 1, 0) == jnp.where(k_t0, 1, 0)
    keep_o = in_o & ((qpos < MEM) | (qpos >= kpos))
    fill_o = jnp.where(in_o, NEG, -jnp.inf).astype(F32)
    return keep_e, fill_e, keep_o, fill_o


def _kernel(x_hbm, mem0_hbm, wq_hbm, wk_hbm, wv_hbm, wo_hbm, wint_hbm, wsp_hbm,
            bsp_hbm, wout_hbm, out_hbm,
            x_v, xn_v, xa_v, xb_v, mem0_v, bsp_v, bsp32_v, zero_v, wint_v, wsp_v, wout_v,
            stage_v, wqkv_v, wo_v, zg_v, st_v, z1t_v, z2t_v, u_v, kst_v, vst_v, o_v, out_v,
            sem_x, sem_w, sem_st, sem_out):
    NRB = FH // RB
    NG = RB // 8
    HT = T1 // 2
    NB2 = NTILE // T2
    PPB = 48 // NB2

    x_parts = [(0, XCH), (XCH, XCH), (2 * XCH, XCH), (3 * XCH, S - 3 * XCH)]
    x_cps = [pltpu.make_async_copy(x_hbm.at[pl.ds(o, n), :], x_v.at[pl.ds(o, n), :], sem_x.at[k])
             for k, (o, n) in enumerate(x_parts)]
    wint_u = wint_hbm.bitcast(U32)
    blk_row = lambda k: (FH + k * RB) if k < NRB else (k - NRB) * RB
    wint_cps, k0 = [], 0
    for k, nb in enumerate(WIN_PIECES):
        o, n = blk_row(k0) // 2, nb * RB // 2
        wint_cps.append(pltpu.make_async_copy(wint_u.at[pl.ds(o, n), :], wint_v.at[pl.ds(o, n), :],
                                              sem_w.at[k]))
        k0 += nb
    wsp_cp = pltpu.make_async_copy(wsp_hbm.bitcast(U32), wsp_v, sem_w.at[3])
    wout_cp = pltpu.make_async_copy(wout_hbm.bitcast(U32), wout_v, sem_w.at[4])
    wo_cp = pltpu.make_async_copy(wo_hbm.bitcast(U32), wo_v, sem_w.at[5])
    mem0_cp = pltpu.make_async_copy(mem0_hbm, mem0_v, sem_w.at[6])
    bsp_cp = pltpu.make_async_copy(bsp_hbm, bsp_v, sem_w.at[7])
    w_hbms = (wq_hbm, wk_hbm, wv_hbm)

    def stage_copy(m, j):
        p = m * 16 + j
        return pltpu.make_async_copy(w_hbms[m].bitcast(U32).at[:, j, :],
                                     stage_v.at[p, pl.ds(0, DM), :], sem_st.at[p // PPB])

    x_cps[0].start()
    x_cps[1].start()
    for cp in wint_cps:
        cp.start()
    x_cps[2].start()
    x_cps[3].start()
    bsp_cp.start()
    wsp_cp.start()
    for m in range(3):
        for j in range(16):
            stage_copy(m, j).start()
    wout_cp.start()
    wo_cp.start()
    mem0_cp.start()

    zero_v[...] = jnp.zeros((8, 128), U32)

    def dep_of(v):
        return pltpu.bitcast(v[0:8, :], U32) & zero_v[...]

    def ln_rows(r0, n, dst, d0, dep=None):
        xr = x_v[pl.ds(r0, n), :].astype(F32)
        if dep is not None:
            d = jnp.concatenate([dep] * (n // 8), axis=0)
            xr = pltpu.bitcast(pltpu.bitcast(xr, U32) | jnp.concatenate([d] * (DM // 128), axis=1), F32)
        xn = _as_u32(_layernorm(xr).astype(BF16))
        xn_v[pl.ds(_mult(r0 // 2, n // 2), n // 2), :] = xn
        dst[d0 // 2:(d0 + n) // 2, :] = xn

    def win_block(nt, f0):
        src = xa_v if nt < HT else xb_v
        xt = _as_bf16(src[(nt % HT) * 64:(nt % HT + 1) * 64, :])
        return jax.lax.dot_general(_as_bf16(wint_v[f0 // 2:(f0 + RB) // 2, :]), xt, NT,
                                   preferred_element_type=F32)

    def z2_block(nt, rb):
        z = win_block(nt, FH + rb * RB)
        g = _gelu(z)
        zg_v[nt, rb * RB:(rb + 1) * RB, :] = g
        g3 = g.reshape(NG, 8, 128)
        bm = jnp.sum(g3, axis=0) * (1.0 / NG)
        c = g3 - bm
        st_v[nt, rb * 8:(rb + 1) * 8, :] = bm
        st_v[nt, (NRB + rb) * 8:(NRB + rb + 1) * 8, :] = jnp.sum(c * c, axis=0)
        return z

    def z2_stats(nt):
        bm = st_v[nt, 0:NRB * 8, :]
        m = jnp.sum(bm, axis=0, keepdims=True) * (1.0 / (NRB * 8))
        dm = bm - m
        m2 = jnp.sum(st_v[nt, NRB * 8:2 * NRB * 8, :] + dm * dm * NG, axis=0, keepdims=True)
        r = jax.lax.rsqrt(m2 * (1.0 / FH) + EPS)
        return jnp.broadcast_to(m, (8, 128)), jnp.broadcast_to(r, (8, 128))

    def z2_norm(nt, tile, rb, m, r, dep):
        m = pltpu.bitcast(pltpu.bitcast(m, U32) | dep, F32)
        g3 = zg_v[nt, rb * RB:(rb + 1) * RB, :].reshape(NG, 8, 128)
        z2t_v[tile, rb * RB // 2:(rb + 1) * RB // 2, :] = _as_u32(
            ((g3 - m) * r).reshape(RB, 128).astype(BF16))

    def z1_block(nt, tile, rb):
        z = win_block(nt, rb * RB)
        z1t_v[tile, rb * RB // 2:(rb + 1) * RB // 2, :] = _as_u32(_gelu(z).astype(BF16))
        return z

    def z1_tile(nt, tile, side=None):
        m, r = z2_stats(nt)
        for rb in range(NRB):
            z = z1_block(nt, tile, rb)
            if rb < NRB - 1:
                z2_norm(nt, tile, rb, m, r, dep_of(z))
            if rb == NRB - 2:
                z2_norm(nt, tile, NRB - 1, m, r, dep_of(z[RB - 8:RB]))
            if side is not None:
                side(rb, z)

    x_cps[0].wait()
    ln_rows(0, XCH, xa_v, 0)
    x_cps[1].wait()
    ln_rows(XCH, XCH, xb_v, 0)
    wint_cps[0].wait()
    for nt in range(T1):
        for rb in range(WIN_PIECES[0]):
            z2_block(nt, rb)
    wint_cps[1].wait()
    for nt in range(T1):
        for rb in range(WIN_PIECES[0], NRB):
            z2_block(nt, rb)
    wint_cps[2].wait()
    x_cps[2].wait()
    for nt in range(T1):
        def side(rb, z, nt=nt):
            if nt >= HT and rb < 4:
                d0 = (nt - HT) * 128 + rb * 32
                ln_rows(T1 * 128 + d0, 16, xa_v, d0, dep_of(z))
                ln_rows(T1 * 128 + d0 + 16, 16, xa_v, d0 + 16, dep_of(z[RB // 2:]))
        z1_tile(nt, nt, side)
    x_cps[3].wait()

    def b1_body(i, carry):
        for nt in range(T1):
            tile = i * T1 + nt
            if nt < HT:
                base, dst = (tile + HT) * 128, xb_v
            else:
                base, dst = jnp.minimum(tile + HT, NTILE - 1) * 128, xa_v
            d0 = (nt % HT) * 128

            def ln_piece(k, z):
                ln_rows(pl.multiple_of(base + k * 16, 16), 16, dst, d0 + k * 16, dep_of(z))

            for rb in range(NRB):
                z = z2_block(nt, rb)
                if rb < 4:
                    ln_piece(rb, z[RB // 2:])
            z1_tile(nt, tile, lambda rb, z: ln_piece(4 + rb, z[RB // 2:]) if rb < 4 else None)
        return carry

    jax.lax.fori_loop(1, NTILE // T1, b1_body, 0)

    wsp_cp.wait()
    bsp_cp.wait()
    bsp32_v[...] = bsp_v[...].astype(F32)

    def unpack(p, half, g):
        r = half * (DM // 2)
        nv = DM // 32
        ng = g.shape[0] // 8
        deps = [dep_of(g[8 * k:8 * k + 8, :]) for k in range(ng)]
        dep = jnp.concatenate([deps[(j * ng) // nv] for j in range(nv)], axis=0)
        a = stage_v[p, pl.ds(r, DM // 4, stride=2), :] | dep
        b = stage_v[p, pl.ds(r + 1, DM // 4, stride=2), :] | dep
        wqkv_v[2 * p, r // 2:r // 2 + DM // 4, :] = (a & jnp.uint32(0xFFFF)) | (b << 16)
        wqkv_v[2 * p + 1, r // 2:r // 2 + DM // 4, :] = (a >> 16) | (b & jnp.uint32(0xFFFF0000))

    fblocks = [(f0, min(128, FH - f0)) for f0 in range(0, FH, 128)]

    def u_transpose(tile):
        for f0, fn in fblocks:
            ut = _as_bf16(z1t_v[tile, f0 // 2:(f0 + fn) // 2, :]).astype(F32)
            u_v[:, f0:f0 + fn] = _as_u32(ut.T.astype(BF16))

    def b2_body(i, carry):
        group = stage_v.at[pl.ds(i * PPB, PPB), pl.ds(0, DM), :]
        pltpu.make_async_copy(group, group, sem_st.at[i]).wait()
        u_transpose(0)
        piece = 0
        for nt in range(T2):
            tile = i * T2 + nt
            h0 = pl.multiple_of(tile * 64, 64)
            brow = bsp32_v[pl.ds(tile, 1), :]
            for f0, fn in fblocks:
                ws = _as_bf16(wsp_v[pl.ds(h0, 64), :])
                z2 = jnp.concatenate(
                    [_as_bf16(z2t_v[k, f0 // 2:(f0 + fn) // 2, :]) for k in range(NTILE)], axis=1)
                g = jax.lax.dot_general(z2, ws, NT, preferred_element_type=F32)
                z1 = _as_bf16(z1t_v[tile, f0 // 2:(f0 + fn) // 2, :]).astype(F32)
                z1t_v[tile, f0 // 2:(f0 + fn) // 2, :] = _as_u32((z1 * (g + brow)).astype(BF16))
                if piece < 2 * PPB:
                    unpack(i * PPB + piece // 2, piece % 2, g)
                    piece += 1
        return carry

    jax.lax.fori_loop(0, NB2, b2_body, 0)
    wout_cp.wait()
    wo_cp.wait()
    mem0_cp.wait()

    keep_e, fill_e, keep_o, fill_o = _masks()

    def step(hq, hkv, odd):
        keep, fill = (keep_o, fill_o) if odd else (keep_e, fill_e)
        rows = hq.shape[0]
        qs, ks, vs, ps = {}, {}, {}, {}
        acc = None
        nslots = H + H // WG
        for t in range(nslots):
            if t < H:
                qs[t] = jnp.dot(hq, _as_bf16(wqkv_v[t]), preferred_element_type=F32).astype(BF16)
                k = jnp.dot(hkv, _as_bf16(wqkv_v[H + t]), preferred_element_type=F32).astype(BF16)
                v = jnp.dot(hkv, _as_bf16(wqkv_v[2 * H + t]), preferred_element_type=F32).astype(BF16)
                if odd:
                    k = jnp.concatenate([k, _as_bf16(kst_v[t])], axis=0)
                    v = jnp.concatenate([v, _as_bf16(vst_v[t])], axis=0)
                else:
                    kst_v[t] = _as_u32(k)
                    vst_v[t] = _as_u32(v)
                ks[t], vs[t] = k, v
            else:
                g = t - H
                og = _as_bf16(o_v[0:rows // 2, g * WG * DH:(g + 1) * WG * DH])
                part = jnp.dot(og, _as_bf16(wo_v[g * WG * DH // 2:(g + 1) * WG * DH // 2, :]),
                               preferred_element_type=F32)
                acc = part if acc is None else acc + part
            hs = t - LAG_S
            if 0 <= hs < H:
                sc = jax.lax.dot_general(qs.pop(hs), ks.pop(hs), NT,
                                         preferred_element_type=F32) * SCALE
                sc = jnp.where(keep, sc, fill)
                e = jnp.exp(sc - jnp.max(sc, axis=-1, keepdims=True))
                inv = 1.0 / jnp.sum(e, axis=-1, keepdims=True)
                ps[hs] = (e * inv).astype(BF16)
            ho = t - LAG_O
            if 0 <= ho < H:
                o = jnp.dot(ps.pop(ho), vs.pop(ho), preferred_element_type=F32)
                o_v[0:rows // 2, ho * DH:(ho + 1) * DH] = _as_u32(o.astype(BF16))
        return acc

    def gate_cols(uu, c0, c1):
        bo = jnp.dot(_as_bf16(u_v[uu * 32:(uu + 1) * 32, :]), _as_bf16(wout_v[:, c0:c1]),
                     preferred_element_type=F32)
        return bo * jax.nn.sigmoid(bo)

    def pair(j, uu, mem):
        i = j * 2 + uu
        r0 = pl.multiple_of(i * 64, 64)
        h0 = pl.multiple_of(i * 32, 32)
        gate_b = gate_cols(uu, GSPLIT, DM)
        xs = _as_bf16(xn_v[pl.ds(h0, 32), :]).astype(F32)
        hkv_e = jnp.concatenate([mem, xs[0:40]], axis=0).astype(BF16)
        acc_e = step(hkv_e[0:32], hkv_e, odd=False)
        gate_a = gate_cols(uu, 0, GSPLIT)
        if uu == 1:
            u_transpose(jnp.minimum(j + 1, NTILE - 1))
        mem_o = acc_e[0:MEM]
        hq_o = jnp.concatenate([mem_o, xs[40:64], xs[24:40]], axis=0).astype(BF16)
        acc_o = step(hq_o, hq_o[0:32], odd=True)
        s_rows = jnp.concatenate([acc_e[8:32], acc_o[32:48], acc_o[8:32]], axis=0)
        gate = jnp.concatenate([gate_a, gate_b], axis=1)
        res = x_v[pl.ds(r0, 64), :].astype(F32) + s_rows * gate
        out_v[pl.ds(r0, 64), :] = res.astype(BF16)
        pltpu.make_async_copy(out_v.at[pl.ds(r0, 64), :],
                              out_hbm.at[pl.ds(r0, 64), :], sem_out).start()
        return acc_o[0:MEM]

    def tile_body(j, mem):
        for uu in range(2):
            mem = pair(j, uu, mem)
        return mem

    jax.lax.fori_loop(0, NTILE, tile_body, mem0_v[...].astype(F32))
    pltpu.make_async_copy(out_v, out_hbm, sem_out).wait()


@jax.jit
def pallas_recurrent_scan__memory_aug_recurrent_mem_tr__mixer_gmlp__prompt_kernel(
    A_x: jax.Array,
    A_mem0: jax.Array,
    A_Wq: jax.Array,
    A_Wk: jax.Array,
    A_Wv: jax.Array,
    A_Wo: jax.Array,
    A_seg_len: jax.Array,
    B_x: jax.Array,
    B_w_in: jax.Array,
    B_w_sp: jax.Array,
    B_b_sp: jax.Array,
    B_w_out: jax.Array,
):
    del A_seg_len, B_x
    hbm = pl.BlockSpec(memory_space=pl.ANY)
    out = pl.pallas_call(
        _kernel,
        out_shape=jax.ShapeDtypeStruct((S, DM), BF16),
        in_specs=[hbm] * 10,
        out_specs=hbm,
        scratch_shapes=[
            pltpu.VMEM((S, DM), BF16),
            pltpu.VMEM((S // 2, DM), U32),
            pltpu.VMEM((T1 * 32, DM), U32),
            pltpu.VMEM((T1 * 32, DM), U32),
            pltpu.VMEM((MEM, DM), BF16),
            pltpu.VMEM((16, 128), BF16),
            pltpu.VMEM((16, 128), F32),
            pltpu.VMEM((8, 128), U32),
            pltpu.VMEM((FH, DM), U32),
            pltpu.VMEM((S // 2, S), U32),
            pltpu.VMEM((FH // 2, DM), U32),
            pltpu.VMEM((48, DM + 8, DH), U32),
            pltpu.VMEM((3 * H, DM // 2, DH), U32),
            pltpu.VMEM((H * DH // 2, DM), U32),
            pltpu.VMEM((T1, FH, 128), F32),
            pltpu.VMEM((T1, 2 * (FH // RB) * 8, 128), F32),
            pltpu.VMEM((NTILE, FH // 2, 128), U32),
            pltpu.VMEM((NTILE, FH // 2, 128), U32),
            pltpu.VMEM((64, FH), U32),
            pltpu.VMEM((H, 24, DH), U32),
            pltpu.VMEM((H, 24, DH), U32),
            pltpu.VMEM((24, H * DH), U32),
            pltpu.VMEM((S, DM), BF16),
            pltpu.SemaphoreType.DMA((4,)),
            pltpu.SemaphoreType.DMA((8,)),
            pltpu.SemaphoreType.DMA((NTILE // T2,)),
            pltpu.SemaphoreType.DMA,
        ],
        compiler_params=pltpu.CompilerParams(vmem_limit_bytes=110 * 1024 * 1024),
    )(
        A_x.reshape(S, DM),
        A_mem0.reshape(MEM, DM),
        A_Wq, A_Wk, A_Wv,
        A_Wo.reshape(H * DH, DM),
        B_w_in.T,
        B_w_sp,
        B_b_sp.reshape(16, 128),
        B_w_out,
    )
    return out.reshape(1, S, DM)
```

```python
import jax
import jax.numpy as jnp
import jax.experimental.pallas as pl
import jax.experimental.pallas.tpu as pltpu

F32 = jnp.float32
BF16 = jnp.bfloat16
U32 = jnp.uint32

S = 2048
DM = 640
H = 32
DH = 128
MEM = 8
SEG = 32
FH = 864
NTILE = S // 128
EPS = 1e-5
SCALE = DH ** (-0.5)
NEG = -1000000000.0

XCH = 256
T1 = 4
T2 = 4
RB = 144
WIN_PIECES = (2, 4, 6)
SBLK = (144, 144, 144)
LN_DEADLINE = 5
STRASSEN = (True, True, True, True)
LAG_V = 2
FAST_RCP = True
LAG_S = 2
LAG_O = 6
WG = 4
GSPLIT = 128

NT = (((1,), (1,)), ((), ()))


def _as_bf16(u):
    return pltpu.bitcast(u, BF16)


def _as_u32(b):
    return pltpu.bitcast(b, U32)


def _layernorm(v):
    m = jnp.mean(v, axis=-1, keepdims=True)
    c = v - m
    var = jnp.mean(c * c, axis=-1, keepdims=True)
    return c * jax.lax.rsqrt(var + EPS)


def _gelu(v):
    return jax.nn.gelu(v, approximate=True)


def _mult(v, m):
    return v if isinstance(v, int) else pl.multiple_of(v, m)


def _lanes(tile):
    return pl.ds(_mult(tile * 128, 128), 128)


def _mask(qgroups, kgroups):
    shape = (8 * len(qgroups), 8 * len(kgroups))

    def table(groups, axis):
        idx = jax.lax.broadcasted_iota(jnp.int32, shape, axis)
        seg = jnp.full(shape, groups[-1][0], jnp.int32)
        pos = idx + (groups[-1][1] - 8 * (len(groups) - 1))
        for g in range(len(groups) - 2, -1, -1):
            inside = idx < 8 * (g + 1)
            seg = jnp.where(inside, groups[g][0], seg)
            pos = jnp.where(inside, idx + (groups[g][1] - 8 * g), pos)
        return seg, pos

    qseg, qpos = table(qgroups, 0)
    kseg, kpos = table(kgroups, 1)
    same = qseg == kseg
    keep = same & ((qpos < MEM) | (qpos >= kpos))
    return keep, jnp.where(same, NEG, -jnp.inf).astype(F32)


def _masks():
    own = lambda sg: [(sg, 0), (sg, 16), (sg, 24), (sg, 32)]
    k0 = [(0, 0), (0, 8), (0, 16), (0, 24), (0, 32), (1, 8)]
    k2 = own(2) + [(2, 8), (3, 8)]
    return [
        _mask(k0[:4], k0),
        _mask(own(1) + k0[4:], own(1) + k0),
        _mask(own(2), k2),
        _mask(own(3) + k2[4:], own(3) + k2),
    ]


def _pre_a(a11, a12, a21, a22):
    return [a11 + a22, a21 + a22, a11, a22, a11 + a12, a21 - a11, a12 - a22]


def _pre_b(b11, b12, b21, b22):
    return [b11 + b22, b12 - b22, b21 - b11, b11 + b12, b21 + b22]


def _post(m):
    return (m[0] + m[3] - m[4] + m[6], m[2] + m[4], m[1] + m[3], m[0] - m[1] + m[2] + m[5])


def _kernel(x_hbm, mem0_hbm, wq_hbm, wk_hbm, wv_hbm, wo_hbm, wint_hbm, wsp_hbm,
            bsp_hbm, wout_hbm, out_hbm,
            x_v, xn_v, xa_v, xb_v, mem0_v, bsp_v, bsp32_v, zero_v, wint_v, wsp_v, wout_v,
            stage_v, wqkv_v, wc_v, wo_v, woc_v, zg_v, st_v, z1t_v, za_v, ta_v, tb_v, u_v, q_v, k_v, v_v, o_v, oc_v, cap_v, out_v,
            sem_x, sem_w, sem_st, sem_wo, sem_out):
    NRB = FH // RB
    NG = RB // 8
    HT = T1 // 2
    NB2 = NTILE // T2
    PPB = 48 // NB2

    x_parts = [(0, XCH), (XCH, XCH), (2 * XCH, XCH), (3 * XCH, S - 3 * XCH)]
    x_cps = [pltpu.make_async_copy(x_hbm.at[pl.ds(o, n), :], x_v.at[pl.ds(o, n), :], sem_x.at[k])
             for k, (o, n) in enumerate(x_parts)]
    wint_u = wint_hbm.bitcast(U32)
    blk_row = lambda k: (FH + k * RB) if k < NRB else (k - NRB) * RB
    wint_cps, k0 = [], 0
    for k, nb in enumerate(WIN_PIECES):
        o, n = blk_row(k0) // 2, nb * RB // 2
        wint_cps.append(pltpu.make_async_copy(wint_u.at[pl.ds(o, n), :], wint_v.at[pl.ds(o, n), :],
                                              sem_w.at[k]))
        k0 += nb
    wsp_cp = pltpu.make_async_copy(wsp_hbm.bitcast(U32), wsp_v, sem_w.at[3])
    wout_cp = pltpu.make_async_copy(wout_hbm.bitcast(U32), wout_v, sem_w.at[4])
    WOQ = H * DH // 2 // NB2

    def wo_copy(i):
        r0 = _mult(i * WOQ, WOQ)
        return pltpu.make_async_copy(wo_hbm.bitcast(U32).at[pl.ds(r0, WOQ), :],
                                     wo_v.at[pl.ds(r0, WOQ), :], sem_wo.at[i])

    mem0_cp = pltpu.make_async_copy(mem0_hbm, mem0_v, sem_w.at[5])
    bsp_cp = pltpu.make_async_copy(bsp_hbm, bsp_v, sem_w.at[6])
    w_hbms = (wq_hbm, wk_hbm, wv_hbm)

    def stage_copy(m, j):
        p = m * 16 + j
        return pltpu.make_async_copy(w_hbms[m].bitcast(U32).at[:, j, :],
                                     stage_v.at[p, pl.ds(0, DM), :], sem_st.at[p // PPB])

    x_cps[0].start()
    x_cps[1].start()
    for cp in wint_cps:
        cp.start()
    x_cps[2].start()
    x_cps[3].start()
    bsp_cp.start()
    wsp_cp.start()
    for p in range(48):
        stage_copy(p // 16, p % 16).start()
        if (p + 1) % PPB == 0:
            wo_copy(p // PPB).start()
    wout_cp.start()
    mem0_cp.start()

    zero_v[...] = jnp.zeros((8, 128), U32)

    pending = []
    first_round = [True]

    def dep_of(v):
        return pltpu.bitcast(v[0:8, :], U32) & zero_v[...]

    def ln_rows(r0, n, dst, d0, dep=None):
        xr = x_v[pl.ds(r0, n), :].astype(F32)
        if dep is not None:
            d = jnp.concatenate([dep] * (n // 8), axis=0)
            xr = pltpu.bitcast(pltpu.bitcast(xr, U32) | jnp.concatenate([d] * (DM // 128), axis=1), F32)
        xn = _as_u32(_layernorm(xr).astype(BF16))
        xn_v[pl.ds(_mult(r0 // 2, n // 2), n // 2), :] = xn
        if dst is not None:
            dst[d0 // 2:(d0 + n) // 2, :] = xn
        if dep is not None:
            pending.append([LN_DEADLINE, xn[0:8, DM - 128:DM] & zero_v[...]])

    def win_block(nt, f0):
        if first_round[0]:
            xt = _as_bf16(xn_v[nt * 64:(nt + 1) * 64, :])
        else:
            src = xa_v if nt < HT else xb_v
            xt = _as_bf16(src[(nt % HT) * 64:(nt % HT + 1) * 64, :])
        w = wint_v[f0 // 2:(f0 + RB) // 2, :]
        due = None
        for e in pending:
            e[0] -= 1
            if e[0] == 0:
                due = e[1] if due is None else due | e[1]
        pending[:] = [e for e in pending if e[0] > 0]
        if due is not None:
            top = jnp.concatenate([w[0:8, 0:128] | due, w[0:8, 128:]], axis=1)
            w = jnp.concatenate([top, w[8:]], axis=0)
        return jax.lax.dot_general(_as_bf16(w), xt, NT, preferred_element_type=F32)

    def z2_block(nt, rb):
        z = win_block(nt, FH + rb * RB)
        g = _gelu(z)
        zg_v[nt, rb * RB:(rb + 1) * RB, :] = g
        g3 = g.reshape(NG, 8, 128)
        bm = jnp.sum(g3, axis=0) * (1.0 / NG)
        c = g3 - bm
        st_v[nt, rb * 8:(rb + 1) * 8, :] = bm
        st_v[nt, (NRB + rb) * 8:(NRB + rb + 1) * 8, :] = jnp.sum(c * c, axis=0)
        return z

    def z2_stats(nt):
        bm = st_v[nt, 0:NRB * 8, :]
        m = jnp.sum(bm, axis=0, keepdims=True) * (1.0 / (NRB * 8))
        dm = bm - m
        m2 = jnp.sum(st_v[nt, NRB * 8:2 * NRB * 8, :] + dm * dm * NG, axis=0, keepdims=True)
        r = jax.lax.rsqrt(m2 * (1.0 / FH) + EPS)
        return jnp.broadcast_to(m, (8, 128)), jnp.broadcast_to(r, (8, 128))

    def z2_norm(ne, tp, k, st, dep):
        (me, re), (mo, ro) = st
        me = pltpu.bitcast(pltpu.bitcast(me, U32) | dep, F32)
        mo = pltpu.bitcast(pltpu.bitcast(mo, U32) | dep, F32)
        nrm = lambda nt, f0, m, r: ((zg_v[nt, f0:f0 + 16, :].reshape(2, 8, 128) - m) * r).reshape(16, 128)
        a11, a21 = nrm(ne, 16 * k, me, re), nrm(ne, FH // 2 + 16 * k, me, re)
        a12, a22 = nrm(ne + 1, 16 * k, mo, ro), nrm(ne + 1, FH // 2 + 16 * k, mo, ro)
        s1 = a21 + a22
        s2 = s1 - a11
        ops = jnp.concatenate([a11, a12, a12 - s2, a22, s1, s2, a11 - a21], axis=1)
        za_v.at[tp][8 * k:8 * k + 8, :] = _as_u32(ops.astype(BF16))

    def z1_block(nt, tile, rb):
        z = win_block(nt, rb * RB)
        z1t_v[rb * RB // 2:(rb + 1) * RB // 2, _lanes(tile)] = _as_u32(_gelu(z).astype(BF16))
        return z

    def z1_pair(ne, tile, side=None):
        st = (z2_stats(ne), z2_stats(ne + 1))
        npc, nbl = FH // 32, 2 * NRB - 1
        for b in range(2 * NRB):
            z = z1_block(ne + b // NRB, tile + b // NRB, b % NRB)
            ks = range(b * npc // nbl, min((b + 1) * npc // nbl, npc))
            for q, k in enumerate(ks):
                z2_norm(ne, tile // 2, k, st, dep_of(z[q * 48:]))
            if side is not None:
                side(b, z)

    x_cps[0].wait()
    ln_rows(0, XCH, None, 0)
    x_cps[1].wait()
    ln_rows(XCH, XCH, None, 0)
    wint_cps[0].wait()
    for nt in range(T1):
        for rb in range(WIN_PIECES[0]):
            z2_block(nt, rb)
    wint_cps[1].wait()
    for nt in range(T1):
        for rb in range(WIN_PIECES[0], NRB):
            z2_block(nt, rb)
    wint_cps[2].wait()
    x_cps[2].wait()
    for ne in range(0, T1, 2):
        def side(b, z, ne=ne):
            k = ne * NRB + b
            if k < HT * 8:
                ln_rows(T1 * 128 + k * 16, 16, xa_v, k * 16, dep_of(z[RB // 2:]))
        z1_pair(ne, ne, side)
    x_cps[3].wait()
    pending.clear()
    first_round[0] = False

    def b1_body(i, carry):
        for ne in range(0, T1, 2):
            tile = i * T1 + ne
            if ne < HT:
                base, dst = (tile + HT) * 128, xb_v
            else:
                base, dst = jnp.minimum(tile + HT, NTILE - HT) * 128, xa_v

            def ln_piece(k, z):
                if k < HT * 8:
                    ln_rows(pl.multiple_of(base + k * 16, 16), 16, dst, k * 16, dep_of(z[RB // 2:]))

            for b in range(2 * NRB):
                ln_piece(b, z2_block(ne + b // NRB, b % NRB))
            z1_pair(ne, tile, lambda b, z: ln_piece(2 * NRB + b, z))
        pending.clear()
        return carry

    jax.lax.fori_loop(1, NTILE // T1, b1_body, 0)

    wsp_cp.wait()
    bsp_cp.wait()
    bsp32_v[...] = bsp_v[...].astype(F32)

    def split_rows(p, r0, dep):
        a = stage_v[p, pl.ds(2 * r0, 8, stride=2), :] | dep
        b = stage_v[p, pl.ds(2 * r0 + 1, 8, stride=2), :] | dep
        lo = (a & jnp.uint32(0xFFFF)) | (b << 16)
        hi = (a >> 16) | (b & jnp.uint32(0xFFFF0000))
        wqkv_v[2 * p, r0:r0 + 8, :] = lo
        wqkv_v[2 * p + 1, r0:r0 + 8, :] = hi
        return lo, hi

    def up(u):
        return _as_bf16(u).astype(F32)

    def unpack(p, part, g):
        ng = g.shape[0] // 8
        groups = range(part * 16 // 3, (part + 1) * 16 // 3)
        rest = range(part * 8 // 3, (part + 1) * 8 // 3)
        n = len(groups) + len(rest)
        dep = lambda q: dep_of(g[8 * ((q * ng) // n):])
        for q, k in enumerate(groups):
            b11, b12 = split_rows(p, 8 * k, dep(q))
            b21, b22 = split_rows(p, 128 + 8 * k, dep(q))
            sums = jnp.concatenate(_pre_b(up(b11), up(b12), up(b21), up(b22)), axis=1)
            wc_v.at[p][8 * k:8 * k + 8, :] = _as_u32(sums.astype(BF16))
        for q, k in enumerate(rest):
            split_rows(p, 256 + 8 * k, dep(len(groups) + q))

    def wo_sums(hp, g):
        ng = g.shape[0] // 8
        for k in range(8):
            d = dep_of(g[8 * ((k * ng) // 8):])
            d = jnp.concatenate([d] * 4, axis=1)
            r0 = pl.multiple_of(hp * 128 + 8 * k, 8)
            we = up(wo_v[pl.ds(r0, 8), 0:512] | d)
            wo = up(wo_v[pl.ds(r0 + 64, 8), 0:512] | d)
            sums = jnp.concatenate(_pre_b(we[:, 0:256], we[:, 256:512], wo[:, 0:256], wo[:, 256:512]), axis=1)
            woc_v.at[hp][8 * k:8 * k + 8, :] = _as_u32(sums.astype(BF16))

    fblocks = [(f0, min(128, FH - f0)) for f0 in range(0, FH, 128)]

    def u_transpose(tile):
        for f0, fn in fblocks:
            ut = _as_bf16(z1t_v[f0 // 2:(f0 + fn) // 2, _lanes(tile)]).astype(F32)
            u_v[:, f0:f0 + fn] = _as_u32(ut.T.astype(BF16))

    NK = NTILE // 2

    def t_piece(tp, dst, pc, dep=None):
        rg, kk = pc // (NK // 2), pc % (NK // 2)
        h0 = _mult(tp * 128 + rg * 8, 8)
        we = wsp_v[pl.ds(h0, 8), kk * 512:(kk + 1) * 512]
        wo = wsp_v[pl.ds(h0 + 64, 8), kk * 512:(kk + 1) * 512]
        if dep is not None:
            d = jnp.concatenate([dep] * 4, axis=1)
            we, wo = we | d, wo | d
        we, wo = _as_bf16(we).astype(F32), _as_bf16(wo).astype(F32)
        ev = lambda w: jnp.concatenate([w[:, 0:128], w[:, 256:384]], axis=1)
        od = lambda w: jnp.concatenate([w[:, 128:256], w[:, 384:512]], axis=1)
        b11, b21, b12, b22 = ev(we), od(we), ev(wo), od(wo)
        t1 = b12 - b11
        t2 = b22 - t1
        ops = jnp.concatenate([t1, t2, b22 - b12, t2 - b21], axis=1)
        dst[rg * 8:(rg + 1) * 8, kk * 1024:(kk + 1) * 1024] = _as_u32(ops.astype(BF16))

    NTP = 8 * (NK // 2)
    for pc in range(NTP):
        t_piece(0, ta_v, pc)

    def b2_body(i, carry):
        group = stage_v.at[pl.ds(i * PPB, PPB), pl.ds(0, DM), :]
        pltpu.make_async_copy(group, group, sem_st.at[i]).wait()
        wo_copy(i).wait()
        u_transpose(0)
        piece = [0]
        for lp in range(2):
            tp = i * 2 + lp
            cur, nxt = (ta_v, tb_v) if lp == 0 else (tb_v, ta_v)
            tpn = jnp.minimum(tp + 1, NK - 1)
            he = pl.multiple_of(tp * 128, 128)
            raw = lambda odd_t, odd_s: jnp.concatenate(
                [wsp_v[pl.ds(he + odd_t * 64, 64), (2 * k + odd_s) * 128:(2 * k + odd_s + 1) * 128]
                 for k in range(NK)], axis=1)
            tj = lambda j: jnp.concatenate(
                [cur[:, (k // 2) * 1024 + j * 256 + (k % 2) * 128:(k // 2) * 1024 + j * 256 + (k % 2 + 1) * 128]
                 for k in range(NK)], axis=1)
            rhs = [lambda: raw(0, 0), lambda: raw(0, 1), lambda: raw(1, 1), lambda: tj(3),
                   lambda: tj(0), lambda: tj(1), lambda: tj(2)]
            nprod = [0]
            total = 7 * len(SBLK)

            def prod(j, f0, fn):
                lhs = jnp.concatenate(
                    [za_v[k, f0 // 2:(f0 + fn) // 2, j * 128:(j + 1) * 128] for k in range(NK)], axis=1)
                p = jax.lax.dot_general(_as_bf16(lhs), _as_bf16(rhs[j]()), NT, preferred_element_type=F32)
                n = nprod[0]
                pcs = range(n * NTP // (total - 1), min((n + 1) * NTP // (total - 1), NTP))
                for q, pc in enumerate(pcs):
                    t_piece(tpn, nxt, pc, dep_of(p[q * 48:]))
                if piece[0] < 3 * PPB:
                    unpack(i * PPB + piece[0] // 3, piece[0] % 3, p)
                elif piece[0] < 3 * PPB + 16 // NB2:
                    wo_sums(i * (16 // NB2) + piece[0] - 3 * PPB, p)
                piece[0] += 1
                nprod[0] += 1
                return p

            def finish(c, f0, fn, odd_t):
                tile = tp * 2 + odd_t
                z1 = _as_bf16(z1t_v[f0 // 2:(f0 + fn) // 2, _lanes(tile)]).astype(F32)
                brow = bsp32_v[pl.ds(tile, 1), :]
                z1t_v[f0 // 2:(f0 + fn) // 2, _lanes(tile)] = _as_u32((z1 * (c + brow)).astype(BF16))

            f0 = 0
            for fn in SBLK:
                p1 = prod(0, f0, fn)
                finish(p1 + prod(1, f0, fn), f0, fn, 0)
                u2 = p1 + prod(5, f0, fn)
                u3 = u2 + prod(6, f0, fn)
                p5 = prod(4, f0, fn)
                finish(u3 + p5, FH // 2 + f0, fn, 1)
                u4 = u2 + p5
                finish(u3 - prod(3, f0, fn), FH // 2 + f0, fn, 0)
                finish(u4 + prod(2, f0, fn), f0, fn, 1)
                f0 += fn
        assert piece[0] >= 3 * PPB + 16 // NB2
        return carry

    jax.lax.fori_loop(0, NB2, b2_body, 0)
    wout_cp.wait()
    mem0_cp.wait()

    masks = _masks()
    for n, (keep, fill) in enumerate(masks):
        cap_v[n, 0:keep.shape[0], 0:keep.shape[1]] = jnp.where(keep, 0.0, fill)
    dot = lambda l, r: jnp.dot(l, r, preferred_element_type=F32)

    def proj64(ops, rest, m, j):
        p = m * 16 + j
        sm = lambda q: _as_bf16(wc_v[p, :, q * 128:(q + 1) * 128])
        rhs = [sm(0), _as_bf16(wqkv_v[2 * p, 0:128, :]), sm(1), sm(2),
               _as_bf16(wqkv_v[2 * p + 1, 128:256, :]), sm(3), sm(4)]
        c11, c12, c21, c22 = _post([dot(ops[q], rhs[q]) for q in range(7)])
        ce = jnp.concatenate([c11, c21], axis=0) + dot(rest, _as_bf16(wqkv_v[2 * p, 256:320, :]))
        co = jnp.concatenate([c12, c22], axis=0) + dot(rest, _as_bf16(wqkv_v[2 * p + 1, 256:320, :]))
        return ce, co

    def step(n, h, hx):
        odd = n % 2 == 1
        hb = h.astype(BF16)
        if n == 0:
            ops = [o.astype(BF16) for o in
                   _pre_a(h[0:32, 0:256], h[0:32, 256:512], h[32:64, 0:256], h[32:64, 256:512])]
            rest = h[:, 512:640].astype(BF16)
        ps, os_ = {}, {}
        qb = 24 * n
        kb = 40 * (n // 2) + (0 if odd else 16)
        nq, nk = (24, 40) if odd else (16, 24)

        def put(buf, r0, t, v):
            buf[r0:r0 + v.shape[0] // 2, _lanes(t)] = _as_u32(v.astype(BF16))

        def project(m, t):
            buf, r0 = (q_v, k_v, v_v)[m], (qb if m == 0 else kb)
            w = lambda: _as_bf16(wqkv_v[m * H + t])
            if n == 0 and STRASSEN[m]:
                if t % 2 == 0:
                    for tt, r in zip((t, t + 1), proj64(ops, rest, m, t // 2)):
                        if m == 0:
                            put(buf, 0, tt, r[0:32])
                            put(buf, 24 + 16, tt, r[32:48])
                            put(buf, 72 + 16, tt, r[48:64])
                        else:
                            put(buf, 16, tt, r[0:48])
                            put(buf, 40 + 32, tt, r[48:64])
            elif n == 0:
                put(buf, r0, t, dot(hb[0:32 if m == 0 else 48], w()))
            elif STRASSEN[m] or (odd if m > 0 else not odd):
                put(buf, r0, t, dot(hb, w()))
            else:
                put(buf, r0, t, dot(jnp.concatenate([hb, hx[n // 2]], axis=0), w()))

        wrows = 48 if odd else 32
        if STRASSEN[3] and odd:
            wrows = 32 if n == 1 else 64
        acc = None
        for t in range(H + H // WG):
            if t < H:
                project(1, t)
            if 0 <= t - LAG_V < H:
                project(2, t - LAG_V)
            if t < H:
                project(0, t)
            else:
                c0, c1 = (t - H) * WG * DH, (t - H + 1) * WG * DH
                if wrows == 64:
                    prs = range((t - H) * WG // 2, (t - H + 1) * WG // 2)
                    cat = lambda f, ax: _as_bf16(jnp.concatenate([f(j) for j in prs], axis=ax))
                    sa = lambda q: cat(lambda j: oc_v[:, (j * 5 + q) * 128:(j * 5 + q + 1) * 128], 1)
                    sb = lambda q: cat(lambda j: woc_v[j, :, q * 256:(q + 1) * 256], 0)
                    lhs = [sa(0), sa(1), cat(lambda j: o_v[0:16, 2 * j * 128:(2 * j + 1) * 128], 1),
                           cat(lambda j: o_v[16:32, (2 * j + 1) * 128:(2 * j + 2) * 128], 1),
                           sa(2), sa(3), sa(4)]
                    rhs = [sb(0), cat(lambda j: wo_v[j * 128:j * 128 + 64, 0:256], 0), sb(1), sb(2),
                           cat(lambda j: wo_v[j * 128 + 64:j * 128 + 128, 256:512], 0), sb(3), sb(4)]
                    c11, c12, c21, c22 = _post([dot(lhs[q], rhs[q]) for q in range(7)])
                    last = dot(_as_bf16(o_v[:, c0:c1]), _as_bf16(wo_v[c0 // 2:c1 // 2, 512:640]))
                    part = jnp.concatenate([jnp.concatenate([c11, c21], axis=0),
                                            jnp.concatenate([c12, c22], axis=0), last], axis=1)
                else:
                    part = dot(_as_bf16(o_v[0:wrows // 2, c0:c1]), _as_bf16(wo_v[c0 // 2:c1 // 2, :]))
                acc = part if acc is None else acc + part
            ho = t - LAG_O
            if 0 <= ho < H:
                o = dot(ps.pop(ho), _as_bf16(v_v[kb:kb + nk, _lanes(ho)]))
                cols = slice(ho * DH, (ho + 1) * DH)
                if STRASSEN[3] and n == 1:
                    o_v[0:16, cols] = _as_u32(o[0:32].astype(BF16))
                    o_v[24:32, cols] = _as_u32(o[32:48].astype(BF16))
                else:
                    o_v[0:o.shape[0] // 2, cols] = _as_u32(o.astype(BF16))
                if wrows == 64:
                    os_[ho] = jnp.concatenate([o, up(o_v[24:32, cols])], axis=0)
                    if ho % 2 == 1:
                        oe, oo = os_.pop(ho - 1), os_.pop(ho)
                        al = _pre_a(oe[0:32], oo[0:32], oe[32:64], oo[32:64])
                        sums = jnp.concatenate([al[0], al[1], al[4], al[5], al[6]], axis=1)
                        oc_v[:, (ho // 2) * 640:(ho // 2 + 1) * 640] = _as_u32(sums.astype(BF16))
            hs = t - LAG_S
            if 0 <= hs < H:
                sc = jax.lax.dot_general(_as_bf16(q_v[qb:qb + nq, _lanes(hs)]),
                                         _as_bf16(k_v[kb:kb + nk, _lanes(hs)]), NT,
                                         preferred_element_type=F32) * SCALE
                cap = cap_v[n, 0:sc.shape[0], 0:sc.shape[1]]
                sc = jnp.where(cap == 0.0, sc, cap)
                e = jnp.exp(sc - jnp.max(sc, axis=-1, keepdims=True))
                l = jnp.sum(e, axis=-1, keepdims=True)
                if FAST_RCP:
                    inv = pl.reciprocal(l, approx=True)
                    inv = inv * (2.0 - l * inv)
                else:
                    inv = 1.0 / l
                ps[hs] = (e * inv).astype(BF16)
        return acc

    def gate_cols(uu, c0, c1):
        bo = dot(_as_bf16(u_v[uu * 32:(uu + 1) * 32, :]), _as_bf16(wout_v[:, c0:c1]))
        hb = 0.5 * bo
        return hb + hb * jnp.tanh(hb)

    def tile_body(j, mem):
        r0 = pl.multiple_of(j * 128, 128)
        xs = _as_bf16(xn_v[pl.ds(pl.multiple_of(j * 64, 64), 64), :]).astype(F32)
        g0b = gate_cols(0, GSPLIT, DM)
        h0 = jnp.concatenate([mem, xs[0:40], xs[64:72], xs[96:104]], axis=0)
        hx = [h0[32:48].astype(BF16), h0[48:64].astype(BF16)]
        a0 = step(0, h0, hx)
        g0a = gate_cols(0, 0, GSPLIT)
        a1 = step(1, jnp.concatenate([a0[0:MEM], xs[40:64]], axis=0), hx)
        g1b = gate_cols(1, GSPLIT, DM)
        a2 = step(2, jnp.concatenate([a1[0:MEM], xs[72:96]], axis=0), hx)
        g1a = gate_cols(1, 0, GSPLIT)
        u_transpose(jnp.minimum(j + 1, NTILE - 1))
        a3 = step(3, jnp.concatenate([a2[0:MEM], xs[104:128]], axis=0), hx)
        mid = a3[48:64] if STRASSEN[3] else a1[32:48]
        s_rows = jnp.concatenate([a0[8:32], mid, a1[8:32], a3[32:40], a2[8:32], a3[40:48], a3[8:32]],
                                 axis=0)
        gate = jnp.concatenate([jnp.concatenate([g0a, g0b], axis=1),
                                jnp.concatenate([g1a, g1b], axis=1)], axis=0)
        res = x_v[pl.ds(r0, 128), :].astype(F32) + s_rows * gate
        out_v[pl.ds(r0, 128), :] = res.astype(BF16)
        pltpu.make_async_copy(out_v.at[pl.ds(r0, 128), :],
                              out_hbm.at[pl.ds(r0, 128), :], sem_out).start()
        return a3[0:MEM]

    jax.lax.fori_loop(0, NTILE, tile_body, mem0_v[...].astype(F32))
    pltpu.make_async_copy(out_v, out_hbm, sem_out).wait()


@jax.jit
def pallas_recurrent_scan__memory_aug_recurrent_mem_tr__mixer_gmlp__prompt_kernel(
    A_x: jax.Array,
    A_mem0: jax.Array,
    A_Wq: jax.Array,
    A_Wk: jax.Array,
    A_Wv: jax.Array,
    A_Wo: jax.Array,
    A_seg_len: jax.Array,
    B_x: jax.Array,
    B_w_in: jax.Array,
    B_w_sp: jax.Array,
    B_b_sp: jax.Array,
    B_w_out: jax.Array,
):
    del A_seg_len, B_x
    hbm = pl.BlockSpec(memory_space=pl.ANY)
    out = pl.pallas_call(
        _kernel,
        out_shape=jax.ShapeDtypeStruct((S, DM), BF16),
        in_specs=[hbm] * 10,
        out_specs=hbm,
        scratch_shapes=[
            pltpu.VMEM((S, DM), BF16),
            pltpu.VMEM((S // 2, DM), U32),
            pltpu.VMEM((T1 * 32, DM), U32),
            pltpu.VMEM((T1 * 32, DM), U32),
            pltpu.VMEM((MEM, DM), BF16),
            pltpu.VMEM((16, 128), BF16),
            pltpu.VMEM((16, 128), F32),
            pltpu.VMEM((8, 128), U32),
            pltpu.VMEM((FH, DM), U32),
            pltpu.VMEM((S // 2, S), U32),
            pltpu.VMEM((FH // 2, DM), U32),
            pltpu.VMEM((48, DM + 8, DH), U32),
            pltpu.VMEM((3 * H, DM // 2, DH), U32),
            pltpu.VMEM((48, 128, 5 * 128), U32),
            pltpu.VMEM((H * DH // 2, DM), U32),
            pltpu.VMEM((H // 2, 64, 5 * 256), U32),
            pltpu.VMEM((T1, FH, 128), F32),
            pltpu.VMEM((T1, 2 * (FH // RB) * 8, 128), F32),
            pltpu.VMEM((FH // 2, S), U32),
            pltpu.VMEM((NTILE // 2, FH // 4, 7 * 128), U32),
            pltpu.VMEM((64, 4 * S // 2), U32),
            pltpu.VMEM((64, 4 * S // 2), U32),
            pltpu.VMEM((64, FH), U32),
            pltpu.VMEM((96, H * DH), U32),
            pltpu.VMEM((80, H * DH), U32),
            pltpu.VMEM((80, H * DH), U32),
            pltpu.VMEM((32, H * DH), U32),
            pltpu.VMEM((16, (H // 2) * 5 * 128), U32),
            pltpu.VMEM((4, 48, 80), F32),
            pltpu.VMEM((S, DM), BF16),
            pltpu.SemaphoreType.DMA((4,)),
            pltpu.SemaphoreType.DMA((7,)),
            pltpu.SemaphoreType.DMA((NTILE // T2,)),
            pltpu.SemaphoreType.DMA((NTILE // T2,)),
            pltpu.SemaphoreType.DMA,
        ],
        compiler_params=pltpu.CompilerParams(vmem_limit_bytes=120 * 1024 * 1024),
    )(
        A_x.reshape(S, DM),
        A_mem0.reshape(MEM, DM),
        A_Wq, A_Wk, A_Wv,
        A_Wo.reshape(H * DH, DM),
        B_w_in.T,
        B_w_sp,
        B_b_sp.reshape(16, 128),
        B_w_out,
    )
    return out.reshape(1, S, DM)
```

```python
import functools

import jax
import jax.numpy as jnp
import jax.experimental.pallas as pl
import jax.experimental.pallas.tpu as pltpu

F32 = jnp.float32
BF16 = jnp.bfloat16
U32 = jnp.uint32

S = 2048
DM = 640
H = 32
DH = 128
MEM = 8
SEG = 32
FH = 864
NTILE = S // 128
EPS = 1e-5
SCALE = DH ** (-0.5)
NEG = -1000000000.0

XCH = 256
T1 = 4
T2 = 4
RB = 144
WIN_PIECES = (2, 4, 6)
SBLK = (144, 144, 144)
SIDE_TAIL = 36
WSP_HEAD = 640
LN_DEADLINE = 5
ORDER0 = (1, 0, 2)
PIPE = ((250, 540, 100, 0), (230, 540, 128, 2), (230, 600, 112, 1), (250, 600, 128, 2))
WG = 4
FILL = (320, 224, 224)

NT = (((1,), (1,)), ((), ()))


def _as_bf16(u):
    return pltpu.bitcast(u, BF16)


def _as_u32(b):
    return pltpu.bitcast(b, U32)


def _layernorm(v):
    m = jnp.mean(v, axis=-1, keepdims=True)
    c = v - m
    var = jnp.mean(c * c, axis=-1, keepdims=True)
    return c * jax.lax.rsqrt(var + EPS)


def _gelu(v):
    return jax.nn.gelu(v, approximate=True)


def _mult(v, m):
    return v if isinstance(v, int) else pl.multiple_of(v, m)


def _lanes(tile):
    return pl.ds(_mult(tile * 128, 128), 128)


def _mask(qgroups, kgroups):
    shape = (8 * len(qgroups), 8 * len(kgroups))

    def table(groups, axis):
        idx = jax.lax.broadcasted_iota(jnp.int32, shape, axis)
        seg = jnp.full(shape, groups[-1][0], jnp.int32)
        pos = idx + (groups[-1][1] - 8 * (len(groups) - 1))
        for g in range(len(groups) - 2, -1, -1):
            inside = idx < 8 * (g + 1)
            seg = jnp.where(inside, groups[g][0], seg)
            pos = jnp.where(inside, idx + (groups[g][1] - 8 * g), pos)
        return seg, pos

    qseg, qpos = table(qgroups, 0)
    kseg, kpos = table(kgroups, 1)
    same = qseg == kseg
    keep = same & ((qpos < MEM) | (qpos >= kpos))
    return keep, jnp.where(same, NEG, -jnp.inf).astype(F32)


def _masks():
    own = lambda sg: [(sg, 0), (sg, 16), (sg, 24), (sg, 32)]
    k0 = [(0, 0), (0, 8), (0, 16), (0, 24), (0, 32), (1, 8)]
    k2 = own(2) + [(2, 8), (3, 8)]
    return [
        _mask(k0[:4], k0),
        _mask(own(1) + k0[4:], own(1) + k0),
        _mask(own(2), k2),
        _mask(own(3) + k2[4:], own(3) + k2),
    ]


def _fast_table(types):
    lines = {0: ((1, 0), (1, -1)), 1: ((0, 1), (1, -1)), 2: ((1, 0), (0, 1))}
    neg = lambda f: (-f[0], -f[1])

    def dual(u, v):
        det = u[0] * v[1] - u[1] * v[0]
        return (v[1] * det, -v[0] * det), (-u[1] * det, u[0] * det)

    n = len(types)
    diag = {(i, k): {(i, i): 1} for i in range(n) for k in range(2)}
    units = [[] for _ in range(n)]
    for i in range(n):
        u = lines[types[i]]
        units[i] += [('p', [(i, u[k])], diag[i, k], [(i, dual(*u)[k])]) for k in range(2)]
        for j in range(i + 1, n):
            if types[i] == types[j]:
                units[i] += [('b', i, j), ('b', j, i)]
                continue
            w = lines[types[j]]
            (ci, cj), = [(x, y) for x in range(2) for y in range(2) if u[x] == w[y]]
            (p, q), = [(x, y) for x in (u[1 - ci], neg(u[1 - ci])) for y in (w[1 - cj], neg(w[1 - cj]))
                       if (x[0] - y[0], x[1] - y[1]) == u[ci]]
            sd, td = dual(p, q)
            units[i] += [('p', [(i, p), (j, q)], {(i, j): 1, (j, i): 1}, [(i, td), (j, sd)]),
                         ('p', [(i, q), (j, q)], {(i, j): 1}, [(i, neg(td)), (j, td)]),
                         ('p', [(i, p), (j, p)], {(j, i): 1}, [(i, sd), (j, neg(sd))])]
            diag[i, ci][i, j] = 1
            diag[i, 1 - ci][j, i] = -1
            diag[j, 1 - cj][i, j] = -1
            diag[j, cj][j, i] = 1
    out = []
    for i in range(n):
        row = []
        for un in units[i]:
            if un[0] == 'p' and [c for c in un[1][0][1] if c][0] < 0:
                un = ('p', [(k, neg(f)) for k, f in un[1]], un[2], [(k, neg(f)) for k, f in un[3]])
            row.append(un)
        out.append(row)
    return out


GH = 5
NGRP = H // GH
UNITS = _fast_table((0, 1, 2, 0, 1))
SUMS = [un[2] for row in UNITS for un in row if un[0] == 'p' and len(un[2]) > 1]
NSUM = len(SUMS)


def _signed_sum(terms):
    terms = sorted(terms, key=lambda cv: -cv[0])
    acc = terms[0][1]
    for c, v in terms[1:]:
        acc = acc + v if c > 0 else acc - v
    return acc


def _lhs_operands(top, bot):
    forms = {}

    def form(i, f):
        sign = 1 if [c for c in f if c][0] > 0 else -1
        key = (i, (sign * f[0], sign * f[1]))
        if key not in forms:
            forms[key] = {(1, 0): lambda: top[i], (0, 1): lambda: bot[i],
                          (1, -1): lambda: top[i] - bot[i]}[key[1]]()
        return sign, forms[key]

    return lambda un: _signed_sum([form(i, f) for i, f in un[1]]).astype(BF16)


class _Acc:
    def __init__(self):
        self.v = {}

    def add(self, key, c, p):
        if key not in self.v:
            self.v[key] = (c, p)
        else:
            sign, v = self.v[key]
            self.v[key] = (sign, v + p if sign == c else v - p)

    def pop(self, key):
        sign, v = self.v.pop(key)
        return v if sign > 0 else -v


def _kernel(x_hbm, mem0_hbm, wq_hbm, wk_hbm, wv_hbm, wo_hbm, wint_hbm, wsp_hbm,
            bsp_hbm, wout_hbm, out_hbm,
            x_v, xn_v, xa_v, xb_v, mem0_v, bsp_v, bsp32_v, zero_v, wint_v, wsp_v, wout_v, woutc_v,
            stage_v, wqkv_v, wc_v, wo_v, woc_v, zg_v, st_v, z1t_v, za_v, ta_v, tb_v, u_v, q_v, k_v, v_v, o_v, cap_v, out_v,
            sem_x, sem_w, sem_st, sem_wo, sem_out):
    NRB = FH // RB
    NG = RB // 8
    HT = T1 // 2
    NB2 = NTILE // T2
    PPB = 48 // NB2

    x_parts = [(0, XCH), (XCH, XCH), (2 * XCH, XCH), (3 * XCH, S - 3 * XCH)]
    x_cps = [pltpu.make_async_copy(x_hbm.at[pl.ds(o, n), :], x_v.at[pl.ds(o, n), :], sem_x.at[k])
             for k, (o, n) in enumerate(x_parts)]
    wint_u = wint_hbm.bitcast(U32)
    blk_row = lambda k: (FH + k * RB) if k < NRB else (k - NRB) * RB
    wint_cps, k0 = [], 0
    for k, nb in enumerate(WIN_PIECES):
        o, n = blk_row(k0) // 2, nb * RB // 2
        wint_cps.append(pltpu.make_async_copy(wint_u.at[pl.ds(o, n), :], wint_v.at[pl.ds(o, n), :],
                                              sem_w.at[k]))
        k0 += nb
    wsp_u = wsp_hbm.bitcast(U32)
    wsp_cp = pltpu.make_async_copy(wsp_u.at[pl.ds(0, WSP_HEAD), :], wsp_v.at[pl.ds(0, WSP_HEAD), :],
                                   sem_w.at[3])
    wsp_cp2 = pltpu.make_async_copy(wsp_u.at[pl.ds(WSP_HEAD, S // 2 - WSP_HEAD), :],
                                    wsp_v.at[pl.ds(WSP_HEAD, S // 2 - WSP_HEAD), :], sem_w.at[7])
    wout_cp = pltpu.make_async_copy(wout_hbm.bitcast(U32), wout_v, sem_w.at[4])
    WOQ = H * DH // 2 // NB2

    def wo_copy(i):
        r0 = _mult(i * WOQ, WOQ)
        return pltpu.make_async_copy(wo_hbm.bitcast(U32).at[pl.ds(r0, WOQ), :],
                                     wo_v.at[pl.ds(r0, WOQ), :], sem_wo.at[i])

    mem0_cp = pltpu.make_async_copy(mem0_hbm, mem0_v, sem_w.at[5])
    bsp_cp = pltpu.make_async_copy(bsp_hbm, bsp_v, sem_w.at[6])
    w_hbms = (wq_hbm, wk_hbm, wv_hbm)

    def stage_copy(m, j):
        p = m * 16 + j
        return pltpu.make_async_copy(w_hbms[m].bitcast(U32).at[:, j, :],
                                     stage_v.at[p, pl.ds(0, DM), :], sem_st.at[p // PPB])

    x_cps[0].start()
    x_cps[1].start()
    for cp in wint_cps:
        cp.start()
    x_cps[2].start()
    x_cps[3].start()
    bsp_cp.start()
    wsp_cp.start()
    wout_cp.start()
    for p in range(48):
        stage_copy(p // 16, p % 16).start()
        if (p + 1) % PPB == 0:
            wo_copy(p // PPB).start()
        if p + 1 == 2 * PPB:
            wsp_cp2.start()
    mem0_cp.start()

    zero_v[...] = jnp.zeros((8, 128), U32)

    pending = []
    first_round = [True]

    def dep_of(v):
        return pltpu.bitcast(v[0:8, :], U32) & zero_v[...]

    def ln_rows(r0, n, dst, d0, dep=None):
        xr = x_v[pl.ds(r0, n), :].astype(F32)
        if dep is not None:
            d = jnp.concatenate([dep] * (n // 8), axis=0)
            xr = pltpu.bitcast(pltpu.bitcast(xr, U32) | jnp.concatenate([d] * (DM // 128), axis=1), F32)
        xn = _as_u32(_layernorm(xr).astype(BF16))
        xn_v[pl.ds(_mult(r0 // 2, n // 2), n // 2), :] = xn
        if dst is not None:
            dst[d0 // 2:(d0 + n) // 2, :] = xn
        if dep is not None:
            pending.append([LN_DEADLINE, xn[0:8, DM - 128:DM] & zero_v[...]])

    def win_block(nt, f0):
        if first_round[0]:
            xt = _as_bf16(xn_v[nt * 64:(nt + 1) * 64, :])
        else:
            src = xa_v if nt < HT else xb_v
            xt = _as_bf16(src[(nt % HT) * 64:(nt % HT + 1) * 64, :])
        w = wint_v[f0 // 2:(f0 + RB) // 2, :]
        due = None
        for e in pending:
            e[0] -= 1
            if e[0] == 0:
                due = e[1] if due is None else due | e[1]
        pending[:] = [e for e in pending if e[0] > 0]
        if due is not None:
            top = jnp.concatenate([w[0:8, 0:128] | due, w[0:8, 128:]], axis=1)
            w = jnp.concatenate([top, w[8:]], axis=0)
        return jax.lax.dot_general(_as_bf16(w), xt, NT, preferred_element_type=F32)

    def z2_block(nt, rb):
        z = win_block(nt, FH + rb * RB)
        g = _gelu(z)
        zg_v[nt, rb * RB:(rb + 1) * RB, :] = g
        g3 = g.reshape(NG, 8, 128)
        bm = jnp.sum(g3, axis=0) * (1.0 / NG)
        c = g3 - bm
        st_v[nt, rb * 8:(rb + 1) * 8, :] = bm
        st_v[nt, (NRB + rb) * 8:(NRB + rb + 1) * 8, :] = jnp.sum(c * c, axis=0)
        return z

    def z2_stats(nt):
        bm = st_v[nt, 0:NRB * 8, :]
        m = jnp.sum(bm, axis=0, keepdims=True) * (1.0 / (NRB * 8))
        dm = bm - m
        m2 = jnp.sum(st_v[nt, NRB * 8:2 * NRB * 8, :] + dm * dm * NG, axis=0, keepdims=True)
        r = jax.lax.rsqrt(m2 * (1.0 / FH) + EPS)
        return jnp.broadcast_to(m, (8, 128)), jnp.broadcast_to(r, (8, 128))

    def z2_norm(ne, tp, k, st, dep):
        (me, re), (mo, ro) = st
        me = pltpu.bitcast(pltpu.bitcast(me, U32) | dep, F32)
        mo = pltpu.bitcast(pltpu.bitcast(mo, U32) | dep, F32)
        nrm = lambda nt, f0, m, r: ((zg_v[nt, f0:f0 + 16, :].reshape(2, 8, 128) - m) * r).reshape(16, 128)
        a11, a21 = nrm(ne, 16 * k, me, re), nrm(ne, FH // 2 + 16 * k, me, re)
        a12, a22 = nrm(ne + 1, 16 * k, mo, ro), nrm(ne + 1, FH // 2 + 16 * k, mo, ro)
        s1 = a21 + a22
        s2 = s1 - a11
        ops = jnp.concatenate([a11, a12, a12 - s2, a22, s1, s2, a11 - a21], axis=1)
        za_v.at[tp][8 * k:8 * k + 8, :] = _as_u32(ops.astype(BF16))

    def z1_block(nt, tile, rb):
        z = win_block(nt, rb * RB)
        z1t_v[rb * RB // 2:(rb + 1) * RB // 2, _lanes(tile)] = _as_u32(_gelu(z).astype(BF16))
        return z

    def z1_pair(ne, tile, side=None):
        st = (z2_stats(ne), z2_stats(ne + 1))
        npc, nbl = FH // 32, 2 * NRB - 1
        for b in range(2 * NRB):
            z = z1_block(ne + b // NRB, tile + b // NRB, b % NRB)
            ks = range(b * npc // nbl, min((b + 1) * npc // nbl, npc))
            for q, k in enumerate(ks):
                z2_norm(ne, tile // 2, k, st, dep_of(z[q * 48:]))
            if side is not None:
                side(b, z)

    x_cps[0].wait()
    ln_rows(0, XCH, None, 0)
    x_cps[1].wait()
    ln_rows(XCH, XCH, None, 0)
    wint_cps[0].wait()
    for nt in range(T1):
        for rb in range(WIN_PIECES[0]):
            z2_block(nt, rb)
    wint_cps[1].wait()
    for nt in range(T1):
        for rb in range(WIN_PIECES[0], NRB):
            z2_block(nt, rb)
    wint_cps[2].wait()
    x_cps[2].wait()
    for ne in range(0, T1, 2):
        def side(b, z, ne=ne):
            k = ne * NRB + b
            if k < HT * 8:
                ln_rows(T1 * 128 + k * 16, 16, xa_v, k * 16, dep_of(z[RB // 2:]))
        z1_pair(ne, ne, side)
    x_cps[3].wait()
    pending.clear()
    first_round[0] = False

    def b1_body(i, carry):
        for ne in range(0, T1, 2):
            tile = i * T1 + ne
            if ne < HT:
                base, dst = (tile + HT) * 128, xb_v
            else:
                base, dst = jnp.minimum(tile + HT, NTILE - HT) * 128, xa_v

            def ln_piece(k, z):
                if k < HT * 8:
                    ln_rows(pl.multiple_of(base + k * 16, 16), 16, dst, k * 16, dep_of(z[RB // 2:]))

            for b in range(2 * NRB):
                ln_piece(b, z2_block(ne + b // NRB, b % NRB))
            z1_pair(ne, tile, lambda b, z: ln_piece(2 * NRB + b, z))
        pending.clear()
        return carry

    jax.lax.fori_loop(1, NTILE // T1, b1_body, 0)

    wsp_cp.wait()
    wout_cp.wait()
    bsp_cp.wait()
    bsp32_v[...] = bsp_v[...].astype(F32)

    def split_rows(p, r0, dep):
        a = stage_v[p, pl.ds(2 * r0, 8, stride=2), :] | dep
        b = stage_v[p, pl.ds(2 * r0 + 1, 8, stride=2), :] | dep
        lo = (a & jnp.uint32(0xFFFF)) | (b << 16)
        hi = (a >> 16) | (b & jnp.uint32(0xFFFF0000))
        wqkv_v[2 * p, r0:r0 + 8, :] = lo
        wqkv_v[2 * p + 1, r0:r0 + 8, :] = hi
        return lo, hi

    def up(u):
        return _as_bf16(u).astype(F32)

    def weight_sums(block, dst, idx, k, dep):
        cache = {}

        def blk(ij):
            if ij not in cache:
                cache[ij] = up(block(ij[0], ij[1], k) | dep)
            return cache[ij]

        mine = [un[2] for un in UNITS[idx] if un[0] == 'p' and len(un[2]) > 1]
        c0 = SUMS.index(mine[0])
        sums = jnp.concatenate([_signed_sum([(c, blk(ij)) for ij, c in r.items()]) for r in mine], axis=1)
        dst[pl.ds(_mult(8 * k, 8), 8), c0 * 128:(c0 + len(mine)) * 128] = _as_u32(sums.astype(BF16))

    fblocks = [(f0, min(128, FH - f0)) for f0 in range(0, FH, 128)]

    def u_transpose(tile):
        for f0, fn in fblocks:
            ut = _as_bf16(z1t_v[f0 // 2:(f0 + fn) // 2, _lanes(tile)]).astype(F32)
            u_v[:, f0:f0 + fn] = _as_u32(ut.T.astype(BF16))

    NK = NTILE // 2

    def t_piece(tp, dst, pc, dep=None):
        rg, kk = pc // (NK // 2), pc % (NK // 2)
        h0 = _mult(tp * 128 + rg * 8, 8)
        we = wsp_v[pl.ds(h0, 8), kk * 512:(kk + 1) * 512]
        wo = wsp_v[pl.ds(h0 + 64, 8), kk * 512:(kk + 1) * 512]
        if dep is not None:
            d = jnp.concatenate([dep] * 4, axis=1)
            we, wo = we | d, wo | d
        we, wo = _as_bf16(we).astype(F32), _as_bf16(wo).astype(F32)
        ev = lambda w: jnp.concatenate([w[:, 0:128], w[:, 256:384]], axis=1)
        od = lambda w: jnp.concatenate([w[:, 128:256], w[:, 384:512]], axis=1)
        b11, b21, b12, b22 = ev(we), od(we), ev(wo), od(wo)
        t1 = b12 - b11
        t2 = b22 - t1
        ops = jnp.concatenate([t1, t2, b22 - b12, t2 - b21], axis=1)
        dst[rg * 8:(rg + 1) * 8, kk * 1024:(kk + 1) * 1024] = _as_u32(ops.astype(BF16))

    NTP = 8 * (NK // 2)
    for pc in range(NTP):
        t_piece(0, ta_v, pc)

    def b2_body(i, carry):
        group = stage_v.at[pl.ds(i * PPB, PPB), pl.ds(0, DM), :]
        pltpu.make_async_copy(group, group, sem_st.at[i]).wait()
        wo_copy(i).wait()

        @pl.when(i == 2)
        def _():
            wsp_cp2.wait()

        u_transpose(0)
        for lp in range(2):
            tp = i * 2 + lp
            cur, nxt = (ta_v, tb_v) if lp == 0 else (tb_v, ta_v)
            tpn = jnp.minimum(tp + 1, NK - 1)
            he = pl.multiple_of(tp * 128, 128)
            raw = lambda odd_t, odd_s: lambda k: wsp_v[
                pl.ds(he + odd_t * 64, 64), (2 * k + odd_s) * 128:(2 * k + odd_s + 1) * 128]
            tj = lambda j: lambda k: cur[
                :, (k // 2) * 1024 + j * 256 + (k % 2) * 128:(k // 2) * 1024 + j * 256 + (k % 2 + 1) * 128]
            rhs = [raw(0, 0), raw(0, 1), raw(1, 1), tj(3), tj(0), tj(1), tj(2)]

            kinds = [[(5, functools.partial(t_piece, tpn, nxt, pc)) for pc in range(NTP)], [], []]
            if lp == 0:
                kinds[1] = [(1, functools.partial(split_rows, i * PPB + pp, 8 * k))
                            for pp in range(PPB) for k in range(DM // 16)]
            else:
                for sl in range(5):
                    gid = jnp.minimum((9 * i) // 2 + sl, (9 * i + 9) // 2 - 1)
                    f0h = (gid // NGRP) * H + (gid % NGRP) * GH
                    block = lambda bi, bj, k, f0h=f0h: wqkv_v[f0h + bj, 64 * bi + 8 * k:64 * bi + 8 * k + 8, :]
                    kinds[1] += [(3, functools.partial(weight_sums, block, wc_v.at[gid], idx, k))
                                 for k in range(8) for idx in range(GH)]
            gid = jnp.minimum((3 * i) // 2 + lp, (3 * i + 3) // 2 - 1)
            block = lambda bi, bj, k, gid=gid: wo_v[
                pl.ds(pl.multiple_of((gid * GH + bi) * 64 + 8 * k, 8), 8), bj * 128:(bj + 1) * 128]
            kinds[2] = [(3, functools.partial(weight_sums, block, woc_v.at[gid], idx, k))
                        for k in range(8) for idx in range(GH)]
            block = lambda bi, bj, k: wout_v[pl.ds(pl.multiple_of(64 * bi + 8 * k, 8), 8), bj * 128:(bj + 1) * 128]
            kinds.append([(3, functools.partial(weight_sums, block, woutc_v, idx, 2 * i + lp))
                          for idx in range(GH)])
            order = sorted(((q + 0.5) / len(kd), kn, q) for kn, kd in enumerate(kinds) for q in range(len(kd)))
            tasks = [kinds[kn][q] for _, kn, q in order]
            budget = sum(c for c, _ in tasks) / (2 * 7 * (FH // 2) // 8 - SIDE_TAIL)
            state = [0.0]

            def side(p):
                for g in range(p.shape[0] // 8):
                    state[0] += budget
                    while tasks and state[0] > 0:
                        c, fn = tasks.pop(0)
                        fn(dep_of(p[8 * g:]))
                        state[0] -= c

            def prod(j, f0, fn):
                p = None
                for ks in (range(NK // 2), range(NK // 2, NK)):
                    lhs = jnp.concatenate(
                        [za_v[k, f0 // 2:(f0 + fn) // 2, j * 128:(j + 1) * 128] for k in ks], axis=1)
                    r = jnp.concatenate([rhs[j](k) for k in ks], axis=1)
                    q = jax.lax.dot_general(_as_bf16(lhs), _as_bf16(r), NT, preferred_element_type=F32)
                    side(q)
                    p = q if p is None else p + q
                return p

            def finish(c, f0, fn, odd_t):
                tile = tp * 2 + odd_t
                z1 = _as_bf16(z1t_v[f0 // 2:(f0 + fn) // 2, _lanes(tile)]).astype(F32)
                brow = bsp32_v[pl.ds(tile, 1), :]
                z1t_v[f0 // 2:(f0 + fn) // 2, _lanes(tile)] = _as_u32((z1 * (c + brow)).astype(BF16))

            f0 = 0
            for fn in SBLK:
                p1 = prod(0, f0, fn)
                finish(p1 + prod(1, f0, fn), f0, fn, 0)
                u2 = p1 + prod(5, f0, fn)
                u3 = u2 + prod(6, f0, fn)
                p5 = prod(4, f0, fn)
                finish(u3 + p5, FH // 2 + f0, fn, 1)
                u4 = u2 + p5
                finish(u3 - prod(3, f0, fn), FH // 2 + f0, fn, 0)
                finish(u4 + prod(2, f0, fn), f0, fn, 1)
                f0 += fn
            assert not tasks
        return carry

    jax.lax.fori_loop(0, NB2, b2_body, 0)
    mem0_cp.wait()

    masks = _masks()
    for n, (keep, fill) in enumerate(masks):
        cap_v[n, 0:keep.shape[0], 0:keep.shape[1]] = jnp.where(keep, 0.0, fill)
    dot = lambda l, r: jnp.dot(l, r, preferred_element_type=F32)

    def fast_units(lhs_of, both, raw, sums, acc, done):
        items = []
        for i, row in enumerate(UNITS):
            for q, un in enumerate(row):
                def fn(un=un, last=(q == len(row) - 1), i=i):
                    if un[0] == 'b':
                        p = dot(both(un[1]), raw(un[1], un[2]))
                        hr = p.shape[0] // 2
                        acc.add((0, un[2]), 1, p[0:hr])
                        acc.add((1, un[2]), 1, p[hr:])
                    else:
                        r = un[2]
                        p = dot(lhs_of(un), raw(*list(r)[0]) if len(r) == 1 else sums(SUMS.index(r)))
                        for k, f in un[3]:
                            for half in range(2):
                                if f[half]:
                                    acc.add((half, k), f[half], p)
                    if last:
                        done(i)
                items.append((16 if un[0] == 'b' else 8, fn))
        return items

    def step(n, h):
        odd = n % 2 == 1
        hb = h.astype(BF16)
        qb = 24 * n
        kb = 40 * (n // 2) + (0 if odd else 16)
        nq, nk = (24, 40) if odd else (16, 24)
        clock = [0]
        d_s, d_o, gap, lag_v = PIPE[n]
        ready, s_at, o_at, ps = {}, {}, {}, {}

        def put(buf, r0, t, v):
            buf[r0:r0 + v.shape[0] // 2, _lanes(t)] = _as_u32(v.astype(BF16))

        def put64(m, t, top, bot):
            buf = (q_v, k_v, v_v)[m]
            if m == 0:
                put(buf, 0, t, top)
                put(buf, 24 + 16, t, bot[0:16])
                put(buf, 72 + 16, t, bot[16:32])
            else:
                put(buf, 16, t, top)
                put(buf, 32, t, bot[0:16])
                put(buf, 40 + 32, t, bot[16:32])
            ready[m, t] = clock[0]

        def plain(m, t):
            r = dot(hb, _as_bf16(wqkv_v[m * H + t]))
            if n == 0:
                put64(m, t, r[0:32], r[32:64])
            else:
                put((q_v, k_v, v_v)[m], qb if m == 0 else kb, t, r)
                ready[m, t] = clock[0]

        work = []
        if n == 0:
            cols = lambda i: slice(i * 128, (i + 1) * 128)
            make = _lhs_operands([h[0:32, cols(i)] for i in range(GH)], [h[32:64, cols(i)] for i in range(GH)])
            ops = {id(un): make(un) for row in UNITS for un in row if un[0] == 'p'}
            for g in range(NGRP):
                for m in ORDER0:
                    if g == NGRP - 1 and m == 2:
                        work += [(80, functools.partial(plain, mm, t))
                                 for t in range(NGRP * GH, H) for mm in (1, 0)]
                    acc = _Acc()
                    work += fast_units(
                        lambda un: ops[id(un)], lambda i: hb[:, cols(i)],
                        lambda i, j, m=m, g=g: _as_bf16(wqkv_v[m * H + g * GH + j, 64 * i:64 * i + 64, :]),
                        lambda q, m=m, g=g: _as_bf16(wc_v[m * NGRP + g, :, q * 128:(q + 1) * 128]),
                        acc, lambda j, m=m, g=g, acc=acc: put64(m, g * GH + j, acc.pop((0, j)), acc.pop((1, j))))
            work += [(80, functools.partial(plain, 2, t)) for t in range(NGRP * GH, H)]
        else:
            for t in range(H + lag_v):
                for m, tt in ((1, t), (2, t - lag_v), (0, t)):
                    if 0 <= tt < H:
                        work.append((40, functools.partial(plain, m, tt)))
        work = [(c, fn, -1) for c, fn in work]

        res = []
        if n == 3:
            acc = _Acc()
            for g in range(NGRP):
                hc = lambda i, g=g: slice((g * GH + i) * DH, (g * GH + i + 1) * DH)
                box = []

                def lhs_of(un, box=box, hc=hc):
                    if not box:
                        box.append(_lhs_operands([up(o_v[0:16, hc(i)]) for i in range(GH)],
                                                 [up(o_v[16:32, hc(i)]) for i in range(GH)]))
                    return box[0](un)

                items = fast_units(
                    lhs_of, lambda i, hc=hc: _as_bf16(o_v[:, hc(i)]),
                    lambda i, j, g=g: _as_bf16(wo_v[(g * GH + i) * 64:(g * GH + i + 1) * 64, j * 128:(j + 1) * 128]),
                    lambda q, g=g: _as_bf16(woc_v[g, :, q * 128:(q + 1) * 128]), acc, lambda j: None)
                work += [(c, fn, g * GH + GH - 1) for c, fn in items]

            def tail():
                c0 = NGRP * GH * DH
                part = dot(_as_bf16(o_v[:, c0:]), _as_bf16(wo_v[c0 // 2:, :]))
                res.append(part + jnp.concatenate(
                    [jnp.concatenate([acc.pop((hf, j)) for j in range(GH)], axis=1) for hf in range(2)], axis=0))

            work.append((160, tail, H - 1))
        else:
            def wgroup(g):
                c0, c1 = g * WG * DH, (g + 1) * WG * DH
                part = dot(_as_bf16(o_v[0:16, c0:c1]), _as_bf16(wo_v[c0 // 2:c1 // 2, :]))
                res[:] = [part + res[0]] if res else [part]

            work += [(40 * WG, functools.partial(wgroup, g), (g + 1) * WG - 1) for g in range(H // WG)]

        def scores(t):
            sc = jax.lax.dot_general(_as_bf16(q_v[qb:qb + nq, _lanes(t)]),
                                     _as_bf16(k_v[kb:kb + nk, _lanes(t)]), NT,
                                     preferred_element_type=F32) * SCALE
            cap = cap_v[n, 0:sc.shape[0], 0:sc.shape[1]]
            sc = jnp.where(cap == 0.0, sc, cap)
            e = jnp.exp(sc - jnp.max(sc, axis=-1, keepdims=True))
            l = jnp.sum(e, axis=-1, keepdims=True)
            inv = pl.reciprocal(l, approx=True)
            inv = inv * (2.0 - l * inv)
            ps[t] = (e * inv).astype(BF16)
            s_at[t] = clock[0]
            clock[0] += nq // 2

        def values(t):
            o = dot(ps.pop(t), _as_bf16(v_v[kb:kb + nk, _lanes(t)]))
            if n == 1:
                put(o_v, 0, t, o[0:32])
                put(o_v, 24, t, o[32:48])
            else:
                put(o_v, 0, t, o)
            o_at[t] = clock[0]
            clock[0] += nq // 2

        def drain(upto):
            while True:
                to, ts = len(o_at), len(s_at)
                if to < ts and (2, to) in ready and (
                        to <= upto or clock[0] >= max(s_at[to] + d_o, ready[2, to] + d_s)):
                    values(to)
                elif ts < H and (0, ts) in ready and (1, ts) in ready and (
                        ts <= upto or clock[0] >= max(ready[0, ts] + d_s, ready[1, ts] + d_s,
                                                      s_at.get(ts - 1, -gap) + gap)):
                    scores(ts)
                else:
                    return

        for c, fn, need in work:
            drain(need)
            clock[0] += c
            fn()
        return res[0]

    def gate_work():
        acc = _Acc()
        cols = lambda i: slice(i * 128, (i + 1) * 128)
        box = []

        def lhs_of(un):
            if not box:
                box.append(_lhs_operands([up(u_v[0:32, cols(i)]) for i in range(GH)],
                                         [up(u_v[32:64, cols(i)]) for i in range(GH)]))
            return box[0](un)

        items = [(2 * c, fn) for c, fn in fast_units(
            lhs_of, lambda i: _as_bf16(u_v[:, cols(i)]),
            lambda i, j: _as_bf16(wout_v[64 * i:64 * i + 64, cols(j)]),
            lambda q: _as_bf16(woutc_v[:, cols(q)]), acc, lambda j: None)]

        def rest(j):
            p = dot(_as_bf16(u_v[:, DM:FH]), _as_bf16(wout_v[DM // 2:FH // 2, cols(j)]))
            acc.add((0, j), 1, p[0:64])
            acc.add((1, j), 1, p[64:128])

        items = [(64, functools.partial(rest, j)) for j in range(GH)] + items

        def chunk(budget):
            box.clear()
            while items and budget > 0:
                c, fn = items.pop(0)
                fn()
                budget -= c

        def result():
            hb = 0.5 * jnp.concatenate(
                [jnp.concatenate([acc.pop((hf, j)) for j in range(GH)], axis=1) for hf in range(2)], axis=0)
            return hb + hb * jnp.tanh(hb)

        return chunk, result

    def tile_body(j, mem):
        r0 = pl.multiple_of(j * 128, 128)
        xs = _as_bf16(xn_v[pl.ds(pl.multiple_of(j * 64, 64), 64), :]).astype(F32)
        chunk, gate_result = gate_work()
        chunk(FILL[0])
        a0 = step(0, jnp.concatenate([mem, xs[0:40], xs[64:72], xs[96:104]], axis=0))
        chunk(FILL[1])
        a1 = step(1, jnp.concatenate([a0[0:MEM], xs[40:64]], axis=0))
        chunk(FILL[2])
        a2 = step(2, jnp.concatenate([a1[0:MEM], xs[72:96]], axis=0))
        chunk(10 ** 6)
        gate = gate_result()
        u_transpose(jnp.minimum(j + 1, NTILE - 1))
        a3 = step(3, jnp.concatenate([a2[0:MEM], xs[104:128]], axis=0))
        s_rows = jnp.concatenate([a0[8:32], a3[48:64], a1[8:32], a3[32:40], a2[8:32], a3[40:48], a3[8:32]],
                                 axis=0)
        res = x_v[pl.ds(r0, 128), :].astype(F32) + s_rows * gate
        out_v[pl.ds(r0, 128), :] = res.astype(BF16)
        pltpu.make_async_copy(out_v.at[pl.ds(r0, 128), :],
                              out_hbm.at[pl.ds(r0, 128), :], sem_out).start()
        return a3[0:MEM]

    jax.lax.fori_loop(0, NTILE, tile_body, mem0_v[...].astype(F32))
    pltpu.make_async_copy(out_v, out_hbm, sem_out).wait()


@jax.jit
def pallas_recurrent_scan__memory_aug_recurrent_mem_tr__mixer_gmlp__prompt_kernel(
    A_x: jax.Array,
    A_mem0: jax.Array,
    A_Wq: jax.Array,
    A_Wk: jax.Array,
    A_Wv: jax.Array,
    A_Wo: jax.Array,
    A_seg_len: jax.Array,
    B_x: jax.Array,
    B_w_in: jax.Array,
    B_w_sp: jax.Array,
    B_b_sp: jax.Array,
    B_w_out: jax.Array,
):
    del A_seg_len, B_x
    hbm = pl.BlockSpec(memory_space=pl.ANY)
    out = pl.pallas_call(
        _kernel,
        out_shape=jax.ShapeDtypeStruct((S, DM), BF16),
        in_specs=[hbm] * 10,
        out_specs=hbm,
        scratch_shapes=[
            pltpu.VMEM((S, DM), BF16),
            pltpu.VMEM((S // 2, DM), U32),
            pltpu.VMEM((T1 * 32, DM), U32),
            pltpu.VMEM((T1 * 32, DM), U32),
            pltpu.VMEM((MEM, DM), BF16),
            pltpu.VMEM((16, 128), BF16),
            pltpu.VMEM((16, 128), F32),
            pltpu.VMEM((8, 128), U32),
            pltpu.VMEM((FH, DM), U32),
            pltpu.VMEM((S // 2, S), U32),
            pltpu.VMEM((FH // 2, DM), U32),
            pltpu.VMEM((64, NSUM * 128), U32),
            pltpu.VMEM((48, DM + 8, DH), U32),
            pltpu.VMEM((3 * H, DM // 2, DH), U32),
            pltpu.VMEM((3 * NGRP, 64, NSUM * 128), U32),
            pltpu.VMEM((H * DH // 2, DM), U32),
            pltpu.VMEM((NGRP, 64, NSUM * 128), U32),
            pltpu.VMEM((T1, FH, 128), F32),
            pltpu.VMEM((T1, 2 * (FH // RB) * 8, 128), F32),
            pltpu.VMEM((FH // 2, S), U32),
            pltpu.VMEM((NTILE // 2, FH // 4, 7 * 128), U32),
            pltpu.VMEM((64, 4 * S // 2), U32),
            pltpu.VMEM((64, 4 * S // 2), U32),
            pltpu.VMEM((64, FH), U32),
            pltpu.VMEM((96, H * DH), U32),
            pltpu.VMEM((80, H * DH), U32),
            pltpu.VMEM((80, H * DH), U32),
            pltpu.VMEM((32, H * DH), U32),
            pltpu.VMEM((4, 48, 80), F32),
            pltpu.VMEM((S, DM), BF16),
            pltpu.SemaphoreType.DMA((4,)),
            pltpu.SemaphoreType.DMA((8,)),
            pltpu.SemaphoreType.DMA((NTILE // T2,)),
            pltpu.SemaphoreType.DMA((NTILE // T2,)),
            pltpu.SemaphoreType.DMA,
        ],
        compiler_params=pltpu.CompilerParams(vmem_limit_bytes=120 * 1024 * 1024),
    )(
        A_x.reshape(S, DM),
        A_mem0.reshape(MEM, DM),
        A_Wq, A_Wk, A_Wv,
        A_Wo.reshape(H * DH, DM),
        B_w_in.T,
        B_w_sp,
        B_b_sp.reshape(16, 128),
        B_w_out,
    )
    return out.reshape(1, S, DM)
```

```python
import functools

import jax
import jax.numpy as jnp
import jax.experimental.pallas as pl
import jax.experimental.pallas.tpu as pltpu

F32 = jnp.float32
BF16 = jnp.bfloat16
U32 = jnp.uint32

S = 2048
DM = 640
H = 32
DH = 128
MEM = 8
SEG = 32
FH = 864
NTILE = S // 128
EPS = 1e-5
SCALE = DH ** (-0.5)
NEG = -1000000000.0

XCH = 256
T1 = 4
T2 = 4
RB = 144
WIN_PIECES = (2, 4, 6)
SBLK = (144, 144, 144)
SIDE_TAIL = 1
WSP_HEAD = 640
LN_DEADLINE = 5
ORDER0 = (1, 0, 2)
PIPE = ((250, 540, 100, 0), (230, 540, 128, 2), (230, 600, 112, 1), (250, 600, 128, 2))
WG = 4
FILL = (320, 224, 224)

NT = (((1,), (1,)), ((), ()))


def _as_bf16(u):
    return pltpu.bitcast(u, BF16)


def _as_u32(b):
    return pltpu.bitcast(b, U32)


def _layernorm(v):
    m = jnp.mean(v, axis=-1, keepdims=True)
    c = v - m
    var = jnp.mean(c * c, axis=-1, keepdims=True)
    return c * jax.lax.rsqrt(var + EPS)


def _gelu(v):
    return jax.nn.gelu(v, approximate=True)


def _mult(v, m):
    return v if isinstance(v, int) else pl.multiple_of(v, m)


def _lanes(tile):
    return pl.ds(_mult(tile * 128, 128), 128)


def _mask(qgroups, kgroups):
    shape = (8 * len(qgroups), 8 * len(kgroups))

    def table(groups, axis):
        idx = jax.lax.broadcasted_iota(jnp.int32, shape, axis)
        seg = jnp.full(shape, groups[-1][0], jnp.int32)
        pos = idx + (groups[-1][1] - 8 * (len(groups) - 1))
        for g in range(len(groups) - 2, -1, -1):
            inside = idx < 8 * (g + 1)
            seg = jnp.where(inside, groups[g][0], seg)
            pos = jnp.where(inside, idx + (groups[g][1] - 8 * g), pos)
        return seg, pos

    qseg, qpos = table(qgroups, 0)
    kseg, kpos = table(kgroups, 1)
    same = qseg == kseg
    keep = same & ((qpos < MEM) | (qpos >= kpos))
    return keep, jnp.where(same, NEG, -jnp.inf).astype(F32)


def _masks():
    own = lambda sg: [(sg, 0), (sg, 16), (sg, 24), (sg, 32)]
    k0 = [(0, 0), (0, 8), (0, 16), (0, 24), (0, 32), (1, 8)]
    k2 = own(2) + [(2, 8), (3, 8)]
    return [
        _mask(k0[:4], k0),
        _mask(own(1) + k0[4:], own(1) + k0),
        _mask(own(2), k2),
        _mask(own(3) + k2[4:], own(3) + k2),
    ]


def _fast_table(types):
    lines = {0: ((1, 0), (1, -1)), 1: ((0, 1), (1, -1)), 2: ((1, 0), (0, 1))}
    neg = lambda f: (-f[0], -f[1])

    def dual(u, v):
        det = u[0] * v[1] - u[1] * v[0]
        return (v[1] * det, -v[0] * det), (-u[1] * det, u[0] * det)

    n = len(types)
    diag = {(i, k): {(i, i): 1} for i in range(n) for k in range(2)}
    units = [[] for _ in range(n)]
    for i in range(n):
        u = lines[types[i]]
        units[i] += [('p', [(i, u[k])], diag[i, k], [(i, dual(*u)[k])]) for k in range(2)]
        for j in range(i + 1, n):
            if types[i] == types[j]:
                units[i] += [('b', i, j), ('b', j, i)]
                continue
            w = lines[types[j]]
            (ci, cj), = [(x, y) for x in range(2) for y in range(2) if u[x] == w[y]]
            (p, q), = [(x, y) for x in (u[1 - ci], neg(u[1 - ci])) for y in (w[1 - cj], neg(w[1 - cj]))
                       if (x[0] - y[0], x[1] - y[1]) == u[ci]]
            sd, td = dual(p, q)
            units[i] += [('p', [(i, p), (j, q)], {(i, j): 1, (j, i): 1}, [(i, td), (j, sd)]),
                         ('p', [(i, q), (j, q)], {(i, j): 1}, [(i, neg(td)), (j, td)]),
                         ('p', [(i, p), (j, p)], {(j, i): 1}, [(i, sd), (j, neg(sd))])]
            diag[i, ci][i, j] = 1
            diag[i, 1 - ci][j, i] = -1
            diag[j, 1 - cj][i, j] = -1
            diag[j, cj][j, i] = 1
    out = []
    for i in range(n):
        row = []
        for un in units[i]:
            if un[0] == 'p' and [c for c in un[1][0][1] if c][0] < 0:
                un = ('p', [(k, neg(f)) for k, f in un[1]], un[2], [(k, neg(f)) for k, f in un[3]])
            row.append(un)
        out.append(row)
    return out


GH = 5
NGRP = H // GH
UNITS = _fast_table((0, 1, 2, 0, 1))
SUMS = [un[2] for row in UNITS for un in row if un[0] == 'p' and len(un[2]) > 1]
NSUM = len(SUMS)


def _signed_sum(terms):
    terms = sorted(terms, key=lambda cv: -cv[0])
    acc = terms[0][1]
    for c, v in terms[1:]:
        acc = acc + v if c > 0 else acc - v
    return acc


def _lhs_operands(top, bot):
    forms = {}

    def form(i, f):
        sign = 1 if [c for c in f if c][0] > 0 else -1
        key = (i, (sign * f[0], sign * f[1]))
        if key not in forms:
            forms[key] = {(1, 0): lambda: top[i], (0, 1): lambda: bot[i],
                          (1, -1): lambda: top[i] - bot[i]}[key[1]]()
        return sign, forms[key]

    return lambda un: _signed_sum([form(i, f) for i, f in un[1]]).astype(BF16)


class _Acc:
    def __init__(self):
        self.v = {}

    def add(self, key, c, p):
        if key not in self.v:
            self.v[key] = (c, p)
        else:
            sign, v = self.v[key]
            self.v[key] = (sign, v + p if sign == c else v - p)

    def pop(self, key):
        sign, v = self.v.pop(key)
        return v if sign > 0 else -v


def _kernel(x_hbm, mem0_hbm, wq_hbm, wk_hbm, wv_hbm, wo_hbm, wint_hbm, wsp_hbm,
            bsp_hbm, wout_hbm, out_hbm,
            x_v, xn_v, xa_v, xb_v, mem0_v, bsp_v, bsp32_v, zero_v, wint_v, wsp_v, wout_v, woutc_v,
            stage_v, wqkv_v, wc_v, wo_v, woc_v, zg_v, st_v, z1t_v, za_v, ta_v, tb_v, u_v, q_v, k_v, v_v, o_v, cap_v, out_v,
            sem_x, sem_w, sem_st, sem_wo, sem_out):
    NRB = FH // RB
    NG = RB // 8
    HT = T1 // 2
    NB2 = NTILE // T2
    PPB = 48 // NB2

    x_parts = [(0, XCH), (XCH, XCH), (2 * XCH, XCH), (3 * XCH, S - 3 * XCH)]
    x_cps = [pltpu.make_async_copy(x_hbm.at[pl.ds(o, n), :], x_v.at[pl.ds(o, n), :], sem_x.at[k])
             for k, (o, n) in enumerate(x_parts)]
    wint_u = wint_hbm.bitcast(U32)
    blk_row = lambda k: (FH + k * RB) if k < NRB else (k - NRB) * RB
    wint_cps, k0 = [], 0
    for k, nb in enumerate(WIN_PIECES):
        o, n = blk_row(k0) // 2, nb * RB // 2
        wint_cps.append(pltpu.make_async_copy(wint_u.at[pl.ds(o, n), :], wint_v.at[pl.ds(o, n), :],
                                              sem_w.at[k]))
        k0 += nb
    wsp_u = wsp_hbm.bitcast(U32)
    wsp_cp = pltpu.make_async_copy(wsp_u.at[pl.ds(0, WSP_HEAD), :], wsp_v.at[pl.ds(0, WSP_HEAD), :],
                                   sem_w.at[3])
    wsp_cp2 = pltpu.make_async_copy(wsp_u.at[pl.ds(WSP_HEAD, S // 2 - WSP_HEAD), :],
                                    wsp_v.at[pl.ds(WSP_HEAD, S // 2 - WSP_HEAD), :], sem_w.at[7])
    wout_cp = pltpu.make_async_copy(wout_hbm.bitcast(U32), wout_v, sem_w.at[4])
    WOQ = H * DH // 2 // NB2

    def wo_copy(i):
        r0 = _mult(i * WOQ, WOQ)
        return pltpu.make_async_copy(wo_hbm.bitcast(U32).at[pl.ds(r0, WOQ), :],
                                     wo_v.at[pl.ds(r0, WOQ), :], sem_wo.at[i])

    mem0_cp = pltpu.make_async_copy(mem0_hbm, mem0_v, sem_w.at[5])
    bsp_cp = pltpu.make_async_copy(bsp_hbm, bsp_v, sem_w.at[6])
    w_hbms = (wq_hbm, wk_hbm, wv_hbm)

    def stage_copy(m, j):
        p = m * 16 + j
        return pltpu.make_async_copy(w_hbms[m].bitcast(U32).at[:, j, :],
                                     stage_v.at[p, pl.ds(0, DM), :], sem_st.at[p // PPB])

    x_cps[0].start()
    x_cps[1].start()
    for cp in wint_cps:
        cp.start()
    x_cps[2].start()
    x_cps[3].start()
    bsp_cp.start()
    wsp_cp.start()
    wout_cp.start()
    for p in range(48):
        stage_copy(p // 16, p % 16).start()
        if (p + 1) % PPB == 0:
            wo_copy(p // PPB).start()
        if p + 1 == 2 * PPB:
            wsp_cp2.start()
    mem0_cp.start()

    zero_v[...] = jnp.zeros((8, 128), U32)

    pending = []
    first_round = [True]

    def dep_of(v):
        return pltpu.bitcast(v[0:8, :], U32) & zero_v[...]

    def ln_rows(r0, n, dst, d0, dep=None):
        xr = x_v[pl.ds(r0, n), :].astype(F32)
        if dep is not None:
            d = jnp.concatenate([dep] * (n // 8), axis=0)
            xr = pltpu.bitcast(pltpu.bitcast(xr, U32) | jnp.concatenate([d] * (DM // 128), axis=1), F32)
        xn = _as_u32(_layernorm(xr).astype(BF16))
        xn_v[pl.ds(_mult(r0 // 2, n // 2), n // 2), :] = xn
        if dst is not None:
            dst[d0 // 2:(d0 + n) // 2, :] = xn
        if dep is not None:
            pending.append([LN_DEADLINE, xn[0:8, DM - 128:DM] & zero_v[...]])

    def win_block(nt, f0):
        if first_round[0]:
            xt = _as_bf16(xn_v[nt * 64:(nt + 1) * 64, :])
        else:
            src = xa_v if nt < HT else xb_v
            xt = _as_bf16(src[(nt % HT) * 64:(nt % HT + 1) * 64, :])
        w = wint_v[f0 // 2:(f0 + RB) // 2, :]
        due = None
        for e in pending:
            e[0] -= 1
            if e[0] == 0:
                due = e[1] if due is None else due | e[1]
        pending[:] = [e for e in pending if e[0] > 0]
        if due is not None:
            top = jnp.concatenate([w[0:8, 0:128] | due, w[0:8, 128:]], axis=1)
            w = jnp.concatenate([top, w[8:]], axis=0)
        return jax.lax.dot_general(_as_bf16(w), xt, NT, preferred_element_type=F32)

    def z2_block(nt, rb):
        z = win_block(nt, FH + rb * RB)
        g = _gelu(z)
        zg_v[nt, rb * RB:(rb + 1) * RB, :] = g
        g3 = g.reshape(NG, 8, 128)
        bm = jnp.sum(g3, axis=0) * (1.0 / NG)
        c = g3 - bm
        st_v[nt, rb * 8:(rb + 1) * 8, :] = bm
        st_v[nt, (NRB + rb) * 8:(NRB + rb + 1) * 8, :] = jnp.sum(c * c, axis=0)
        return z

    def z2_stats(nt):
        bm = st_v[nt, 0:NRB * 8, :]
        m = jnp.sum(bm, axis=0, keepdims=True) * (1.0 / (NRB * 8))
        dm = bm - m
        m2 = jnp.sum(st_v[nt, NRB * 8:2 * NRB * 8, :] + dm * dm * NG, axis=0, keepdims=True)
        r = jax.lax.rsqrt(m2 * (1.0 / FH) + EPS)
        return jnp.broadcast_to(m, (8, 128)), jnp.broadcast_to(r, (8, 128))

    def z2_norm(ne, tp, k, st, dep):
        (me, re), (mo, ro) = st
        me = pltpu.bitcast(pltpu.bitcast(me, U32) | dep, F32)
        mo = pltpu.bitcast(pltpu.bitcast(mo, U32) | dep, F32)
        nrm = lambda nt, f0, m, r: ((zg_v[nt, f0:f0 + 16, :].reshape(2, 8, 128) - m) * r).reshape(16, 128)
        a11, a21 = nrm(ne, 16 * k, me, re), nrm(ne, FH // 2 + 16 * k, me, re)
        a12, a22 = nrm(ne + 1, 16 * k, mo, ro), nrm(ne + 1, FH // 2 + 16 * k, mo, ro)
        s1 = a21 + a22
        s2 = s1 - a11
        ops = jnp.concatenate([a11, a12, a12 - s2, a22, s1, s2, a11 - a21], axis=1)
        za_v.at[tp][8 * k:8 * k + 8, :] = _as_u32(ops.astype(BF16))

    def z1_block(nt, tile, rb):
        z = win_block(nt, rb * RB)
        z1t_v[rb * RB // 2:(rb + 1) * RB // 2, _lanes(tile)] = _as_u32(_gelu(z).astype(BF16))
        return z

    def z1_pair(ne, tile, side=None):
        st = (z2_stats(ne), z2_stats(ne + 1))
        npc, nbl = FH // 32, 2 * NRB - 1
        for b in range(2 * NRB):
            z = z1_block(ne + b // NRB, tile + b // NRB, b % NRB)
            ks = range(b * npc // nbl, min((b + 1) * npc // nbl, npc))
            for q, k in enumerate(ks):
                z2_norm(ne, tile // 2, k, st, dep_of(z[q * 48:]))
            if side is not None:
                side(b, z)

    x_cps[0].wait()
    ln_rows(0, XCH, None, 0)
    x_cps[1].wait()
    ln_rows(XCH, XCH, None, 0)
    wint_cps[0].wait()
    for nt in range(T1):
        for rb in range(WIN_PIECES[0]):
            z2_block(nt, rb)
    wint_cps[1].wait()
    for nt in range(T1):
        for rb in range(WIN_PIECES[0], NRB):
            z2_block(nt, rb)
    wint_cps[2].wait()
    x_cps[2].wait()
    for ne in range(0, T1, 2):
        def side(b, z, ne=ne):
            k = ne * NRB + b
            if k < HT * 8:
                ln_rows(T1 * 128 + k * 16, 16, xa_v, k * 16, dep_of(z[RB // 2:]))
        z1_pair(ne, ne, side)
    x_cps[3].wait()
    pending.clear()
    first_round[0] = False

    def b1_body(i, carry):
        for ne in range(0, T1, 2):
            tile = i * T1 + ne
            if ne < HT:
                base, dst = (tile + HT) * 128, xb_v
            else:
                base, dst = jnp.minimum(tile + HT, NTILE - HT) * 128, xa_v

            def ln_piece(k, z):
                if k < HT * 8:
                    ln_rows(pl.multiple_of(base + k * 16, 16), 16, dst, k * 16, dep_of(z[RB // 2:]))

            for b in range(2 * NRB):
                ln_piece(b, z2_block(ne + b // NRB, b % NRB))
            z1_pair(ne, tile, lambda b, z: ln_piece(2 * NRB + b, z))
        pending.clear()
        return carry

    jax.lax.fori_loop(1, NTILE // T1, b1_body, 0)

    wsp_cp.wait()
    wout_cp.wait()
    bsp_cp.wait()
    bsp32_v[...] = bsp_v[...].astype(F32)

    def split_block(p, bi, dep):
        a = stage_v[p, pl.ds(128 * bi, 64, stride=2), :] | dep
        b = stage_v[p, pl.ds(128 * bi + 1, 64, stride=2), :] | dep
        wqkv_v[2 * p, 64 * bi:64 * bi + 64, :] = (a & jnp.uint32(0xFFFF)) | (b << 16)
        wqkv_v[2 * p + 1, 64 * bi:64 * bi + 64, :] = (a >> 16) | (b & jnp.uint32(0xFFFF0000))

    def up(u):
        return _as_bf16(u).astype(F32)

    def weight_sums(block, dst, rows, idx, dep):
        cache = {}

        def blk(ij):
            if ij not in cache:
                w = block(*ij)
                cache[ij] = up(w | dep[0:w.shape[0]])
            return cache[ij]

        mine = [un[2] for un in UNITS[idx] if un[0] == 'p' and len(un[2]) > 1]
        c0 = SUMS.index(mine[0])
        sums = jnp.concatenate([_signed_sum([(c, blk(ij)) for ij, c in r.items()]) for r in mine], axis=1)
        dst[rows, c0 * 128:(c0 + len(mine)) * 128] = _as_u32(sums.astype(BF16))

    fblocks = [(f0, min(128, FH - f0)) for f0 in range(0, FH, 128)]

    def u_transpose(tile):
        for f0, fn in fblocks:
            ut = _as_bf16(z1t_v[f0 // 2:(f0 + fn) // 2, _lanes(tile)]).astype(F32)
            u_v[:, f0:f0 + fn] = _as_u32(ut.T.astype(BF16))

    NK = NTILE // 2

    def t_piece(tp, dst, k, dep=None):
        h0 = _mult(tp * 128, 128)
        we = wsp_v[pl.ds(h0, 64), k * 256:(k + 1) * 256]
        wo = wsp_v[pl.ds(h0 + 64, 64), k * 256:(k + 1) * 256]
        if dep is not None:
            d = jnp.concatenate([dep, dep], axis=1)
            we, wo = we | d, wo | d
        we, wo = up(we), up(wo)
        b11, b21, b12, b22 = we[:, 0:128], we[:, 128:256], wo[:, 0:128], wo[:, 128:256]
        t1 = b12 - b11
        t2 = b22 - t1
        ops = jnp.concatenate([t1, t2, b22 - b12, t2 - b21], axis=1)
        dst[:, k * 512:(k + 1) * 512] = _as_u32(ops.astype(BF16))

    for k in range(NK):
        t_piece(0, ta_v, k)

    def b2_body(i, carry):
        group = stage_v.at[pl.ds(i * PPB, PPB), pl.ds(0, DM), :]
        pltpu.make_async_copy(group, group, sem_st.at[i]).wait()
        wo_copy(i).wait()

        @pl.when(i == 2)
        def _():
            wsp_cp2.wait()

        u_transpose(0)
        for lp in range(2):
            tp = i * 2 + lp
            cur, nxt = (ta_v, tb_v) if lp == 0 else (tb_v, ta_v)
            tpn = jnp.minimum(tp + 1, NK - 1)
            he = pl.multiple_of(tp * 128, 128)
            raw = lambda odd_t, odd_s: lambda k: wsp_v[
                pl.ds(he + odd_t * 64, 64), (2 * k + odd_s) * 128:(2 * k + odd_s + 1) * 128]
            tj = lambda j: lambda k: cur[:, k * 512 + j * 128:k * 512 + (j + 1) * 128]
            rhs = [raw(0, 0), raw(0, 1), raw(1, 1), tj(3), tj(0), tj(1), tj(2)]

            part = functools.partial
            full = slice(0, 64)
            kinds = [[(25, part(t_piece, tpn, nxt, k)) for k in range(NK)], []]
            if lp == 0:
                kinds[1] = [(9, part(split_block, i * PPB + pp, bi)) for pp in range(PPB) for bi in range(GH)]
            else:
                for sl in range(5):
                    gid = jnp.minimum((9 * i) // 2 + sl, (9 * i + 9) // 2 - 1)
                    f0h = (gid // NGRP) * H + (gid % NGRP) * GH
                    block = lambda bi, bj, f0h=f0h: wqkv_v[f0h + bj, 64 * bi:64 * bi + 64, :]
                    kinds[1] += [(30, part(weight_sums, block, wc_v.at[gid], full, idx)) for idx in range(GH)]
            if lp == 0:
                kinds.append([])
                for sl in range(2):
                    gid = jnp.minimum((3 * i) // 2 + sl, (3 * i + 3) // 2 - 1)
                    block = lambda bi, bj, gid=gid: wo_v[
                        pl.ds(pl.multiple_of((gid * GH + bi) * 64, 64), 64), bj * 128:(bj + 1) * 128]
                    kinds[-1] += [(30, part(weight_sums, block, woc_v.at[gid], full, idx)) for idx in range(GH)]
            r8 = pl.multiple_of(8 * (2 * i + lp), 8)
            block = lambda bi, bj, r8=r8: wout_v[pl.ds(64 * bi + r8, 8), bj * 128:(bj + 1) * 128]
            kinds.append([(4, part(weight_sums, block, woutc_v, pl.ds(r8, 8), idx)) for idx in range(GH)])
            order = sorted(((q + 0.5) / len(kd), kn, q) for kn, kd in enumerate(kinds) for q in range(len(kd)))
            tasks = [kinds[kn][q] for _, kn, q in order]
            budget = sum(c for c, _ in tasks) / (2 * 7 * len(SBLK) - SIDE_TAIL)
            state = [0.0]

            def side(p):
                state[0] += budget
                phase = 0
                while tasks and state[0] > 0:
                    c, fn = tasks.pop(0)
                    rows = p[0:128].reshape(8, 16, 128)[:, 8 * phase:8 * phase + 8, :]
                    fn((pltpu.bitcast(rows, U32) & zero_v[...]).reshape(64, 128))
                    state[0] -= c
                    phase = 1 - phase

            def prod(j, f0, fn):
                p = None
                for ks in (range(NK // 2), range(NK // 2, NK)):
                    lhs = jnp.concatenate(
                        [za_v[k, f0 // 2:(f0 + fn) // 2, j * 128:(j + 1) * 128] for k in ks], axis=1)
                    r = jnp.concatenate([rhs[j](k) for k in ks], axis=1)
                    q = jax.lax.dot_general(_as_bf16(lhs), _as_bf16(r), NT, preferred_element_type=F32)
                    side(q)
                    p = q if p is None else p + q
                return p

            def finish(c, f0, fn, odd_t):
                tile = tp * 2 + odd_t
                z1 = _as_bf16(z1t_v[f0 // 2:(f0 + fn) // 2, _lanes(tile)]).astype(F32)
                brow = bsp32_v[pl.ds(tile, 1), :]
                z1t_v[f0 // 2:(f0 + fn) // 2, _lanes(tile)] = _as_u32((z1 * (c + brow)).astype(BF16))

            f0 = 0
            for fn in SBLK:
                p1 = prod(0, f0, fn)
                finish(p1 + prod(1, f0, fn), f0, fn, 0)
                u2 = p1 + prod(5, f0, fn)
                u3 = u2 + prod(6, f0, fn)
                p5 = prod(4, f0, fn)
                finish(u3 + p5, FH // 2 + f0, fn, 1)
                u4 = u2 + p5
                finish(u3 - prod(3, f0, fn), FH // 2 + f0, fn, 0)
                finish(u4 + prod(2, f0, fn), f0, fn, 1)
                f0 += fn
            assert not tasks
        return carry

    jax.lax.fori_loop(0, NB2, b2_body, 0)
    mem0_cp.wait()

    masks = _masks()
    for n, (keep, fill) in enumerate(masks):
        cap_v[n, 0:keep.shape[0], 0:keep.shape[1]] = jnp.where(keep, 0.0, fill)
    dot = lambda l, r: jnp.dot(l, r, preferred_element_type=F32)

    def fast_units(lhs_of, both, raw, sums, acc, done):
        items = []
        for i, row in enumerate(UNITS):
            for q, un in enumerate(row):
                def fn(un=un, last=(q == len(row) - 1), i=i):
                    if un[0] == 'b':
                        p = dot(both(un[1]), raw(un[1], un[2]))
                        hr = p.shape[0] // 2
                        acc.add((0, un[2]), 1, p[0:hr])
                        acc.add((1, un[2]), 1, p[hr:])
                    else:
                        r = un[2]
                        p = dot(lhs_of(un), raw(*list(r)[0]) if len(r) == 1 else sums(SUMS.index(r)))
                        for k, f in un[3]:
                            for half in range(2):
                                if f[half]:
                                    acc.add((half, k), f[half], p)
                    if last:
                        done(i)
                items.append((16 if un[0] == 'b' else 8, fn))
        return items

    def step(n, h):
        odd = n % 2 == 1
        hb = h.astype(BF16)
        qb = 24 * n
        kb = 40 * (n // 2) + (0 if odd else 16)
        nq, nk = (24, 40) if odd else (16, 24)
        clock = [0]
        d_s, d_o, gap, lag_v = PIPE[n]
        ready, s_at, o_at, ps = {}, {}, {}, {}

        def put(buf, r0, t, v):
            buf[r0:r0 + v.shape[0] // 2, _lanes(t)] = _as_u32(v.astype(BF16))

        def put64(m, t, top, bot):
            buf = (q_v, k_v, v_v)[m]
            if m == 0:
                put(buf, 0, t, top)
                put(buf, 24 + 16, t, bot[0:16])
                put(buf, 72 + 16, t, bot[16:32])
            else:
                put(buf, 16, t, top)
                put(buf, 32, t, bot[0:16])
                put(buf, 40 + 32, t, bot[16:32])
            ready[m, t] = clock[0]

        def plain(m, t):
            r = dot(hb, _as_bf16(wqkv_v[m * H + t]))
            if n == 0:
                put64(m, t, r[0:32], r[32:64])
            else:
                put((q_v, k_v, v_v)[m], qb if m == 0 else kb, t, r)
                ready[m, t] = clock[0]

        work = []
        if n == 0:
            cols = lambda i: slice(i * 128, (i + 1) * 128)
            make = _lhs_operands([h[0:32, cols(i)] for i in range(GH)], [h[32:64, cols(i)] for i in range(GH)])
            ops = {id(un): make(un) for row in UNITS for un in row if un[0] == 'p'}
            for g in range(NGRP):
                for m in ORDER0:
                    if g == NGRP - 1 and m == 2:
                        work += [(80, functools.partial(plain, mm, t))
                                 for t in range(NGRP * GH, H) for mm in (1, 0)]
                    acc = _Acc()
                    work += fast_units(
                        lambda un: ops[id(un)], lambda i: hb[:, cols(i)],
                        lambda i, j, m=m, g=g: _as_bf16(wqkv_v[m * H + g * GH + j, 64 * i:64 * i + 64, :]),
                        lambda q, m=m, g=g: _as_bf16(wc_v[m * NGRP + g, :, q * 128:(q + 1) * 128]),
                        acc, lambda j, m=m, g=g, acc=acc: put64(m, g * GH + j, acc.pop((0, j)), acc.pop((1, j))))
            work += [(80, functools.partial(plain, 2, t)) for t in range(NGRP * GH, H)]
        else:
            for t in range(H + lag_v):
                for m, tt in ((1, t), (2, t - lag_v), (0, t)):
                    if 0 <= tt < H:
                        work.append((40, functools.partial(plain, m, tt)))
        work = [(c, fn, -1) for c, fn in work]

        res = []
        if n == 3:
            acc = _Acc()
            for g in range(NGRP):
                hc = lambda i, g=g: slice((g * GH + i) * DH, (g * GH + i + 1) * DH)
                box = []

                def lhs_of(un, box=box, hc=hc):
                    if not box:
                        box.append(_lhs_operands([up(o_v[0:16, hc(i)]) for i in range(GH)],
                                                 [up(o_v[16:32, hc(i)]) for i in range(GH)]))
                    return box[0](un)

                items = fast_units(
                    lhs_of, lambda i, hc=hc: _as_bf16(o_v[:, hc(i)]),
                    lambda i, j, g=g: _as_bf16(wo_v[(g * GH + i) * 64:(g * GH + i + 1) * 64, j * 128:(j + 1) * 128]),
                    lambda q, g=g: _as_bf16(woc_v[g, :, q * 128:(q + 1) * 128]), acc, lambda j: None)
                work += [(c, fn, g * GH + GH - 1) for c, fn in items]

            def tail():
                c0 = NGRP * GH * DH
                part = dot(_as_bf16(o_v[:, c0:]), _as_bf16(wo_v[c0 // 2:, :]))
                res.append(part + jnp.concatenate(
                    [jnp.concatenate([acc.pop((hf, j)) for j in range(GH)], axis=1) for hf in range(2)], axis=0))

            work.append((160, tail, H - 1))
        else:
            def wgroup(g):
                c0, c1 = g * WG * DH, (g + 1) * WG * DH
                part = dot(_as_bf16(o_v[0:16, c0:c1]), _as_bf16(wo_v[c0 // 2:c1 // 2, :]))
                res[:] = [part + res[0]] if res else [part]

            work += [(40 * WG, functools.partial(wgroup, g), (g + 1) * WG - 1) for g in range(H // WG)]

        def scores(t):
            sc = jax.lax.dot_general(_as_bf16(q_v[qb:qb + nq, _lanes(t)]),
                                     _as_bf16(k_v[kb:kb + nk, _lanes(t)]), NT,
                                     preferred_element_type=F32) * SCALE
            cap = cap_v[n, 0:sc.shape[0], 0:sc.shape[1]]
            sc = jnp.where(cap == 0.0, sc, cap)
            e = jnp.exp(sc - jnp.max(sc, axis=-1, keepdims=True))
            l = jnp.sum(e, axis=-1, keepdims=True)
            inv = pl.reciprocal(l, approx=True)
            inv = inv * (2.0 - l * inv)
            ps[t] = (e * inv).astype(BF16)
            s_at[t] = clock[0]
            clock[0] += nq // 2

        def values(t):
            o = dot(ps.pop(t), _as_bf16(v_v[kb:kb + nk, _lanes(t)]))
            if n == 1:
                put(o_v, 0, t, o[0:32])
                put(o_v, 24, t, o[32:48])
            else:
                put(o_v, 0, t, o)
            o_at[t] = clock[0]
            clock[0] += nq // 2

        def drain(upto):
            while True:
                to, ts = len(o_at), len(s_at)
                if to < ts and (2, to) in ready and (
                        to <= upto or clock[0] >= max(s_at[to] + d_o, ready[2, to] + d_s)):
                    values(to)
                elif ts < H and (0, ts) in ready and (1, ts) in ready and (
                        ts <= upto or clock[0] >= max(ready[0, ts] + d_s, ready[1, ts] + d_s,
                                                      s_at.get(ts - 1, -gap) + gap)):
                    scores(ts)
                else:
                    return

        for c, fn, need in work:
            drain(need)
            clock[0] += c
            fn()
        return res[0]

    def gate_work():
        acc = _Acc()
        cols = lambda i: slice(i * 128, (i + 1) * 128)
        box = []

        def lhs_of(un):
            if not box:
                box.append(_lhs_operands([up(u_v[0:32, cols(i)]) for i in range(GH)],
                                         [up(u_v[32:64, cols(i)]) for i in range(GH)]))
            return box[0](un)

        items = [(2 * c, fn) for c, fn in fast_units(
            lhs_of, lambda i: _as_bf16(u_v[:, cols(i)]),
            lambda i, j: _as_bf16(wout_v[64 * i:64 * i + 64, cols(j)]),
            lambda q: _as_bf16(woutc_v[:, cols(q)]), acc, lambda j: None)]

        def rest(j):
            p = dot(_as_bf16(u_v[:, DM:FH]), _as_bf16(wout_v[DM // 2:FH // 2, cols(j)]))
            acc.add((0, j), 1, p[0:64])
            acc.add((1, j), 1, p[64:128])

        items = [(64, functools.partial(rest, j)) for j in range(GH)] + items

        def chunk(budget):
            box.clear()
            while items and budget > 0:
                c, fn = items.pop(0)
                fn()
                budget -= c

        def result():
            hb = 0.5 * jnp.concatenate(
                [jnp.concatenate([acc.pop((hf, j)) for j in range(GH)], axis=1) for hf in range(2)], axis=0)
            return hb + hb * jnp.tanh(hb)

        return chunk, result

    def tile_body(j, mem):
        r0 = pl.multiple_of(j * 128, 128)
        xs = _as_bf16(xn_v[pl.ds(pl.multiple_of(j * 64, 64), 64), :]).astype(F32)
        chunk, gate_result = gate_work()
        chunk(FILL[0])
        a0 = step(0, jnp.concatenate([mem, xs[0:40], xs[64:72], xs[96:104]], axis=0))
        chunk(FILL[1])
        a1 = step(1, jnp.concatenate([a0[0:MEM], xs[40:64]], axis=0))
        chunk(FILL[2])
        a2 = step(2, jnp.concatenate([a1[0:MEM], xs[72:96]], axis=0))
        chunk(10 ** 6)
        gate = gate_result()
        u_transpose(jnp.minimum(j + 1, NTILE - 1))
        a3 = step(3, jnp.concatenate([a2[0:MEM], xs[104:128]], axis=0))
        s_rows = jnp.concatenate([a0[8:32], a3[48:64], a1[8:32], a3[32:40], a2[8:32], a3[40:48], a3[8:32]],
                                 axis=0)
        res = x_v[pl.ds(r0, 128), :].astype(F32) + s_rows * gate
        out_v[pl.ds(r0, 128), :] = res.astype(BF16)
        pltpu.make_async_copy(out_v.at[pl.ds(r0, 128), :],
                              out_hbm.at[pl.ds(r0, 128), :], sem_out).start()
        return a3[0:MEM]

    jax.lax.fori_loop(0, NTILE, tile_body, mem0_v[...].astype(F32))
    pltpu.make_async_copy(out_v, out_hbm, sem_out).wait()


@jax.jit
def pallas_recurrent_scan__memory_aug_recurrent_mem_tr__mixer_gmlp__prompt_kernel(
    A_x: jax.Array,
    A_mem0: jax.Array,
    A_Wq: jax.Array,
    A_Wk: jax.Array,
    A_Wv: jax.Array,
    A_Wo: jax.Array,
    A_seg_len: jax.Array,
    B_x: jax.Array,
    B_w_in: jax.Array,
    B_w_sp: jax.Array,
    B_b_sp: jax.Array,
    B_w_out: jax.Array,
):
    del A_seg_len, B_x
    hbm = pl.BlockSpec(memory_space=pl.ANY)
    out = pl.pallas_call(
        _kernel,
        out_shape=jax.ShapeDtypeStruct((S, DM), BF16),
        in_specs=[hbm] * 10,
        out_specs=hbm,
        scratch_shapes=[
            pltpu.VMEM((S, DM), BF16),
            pltpu.VMEM((S // 2, DM), U32),
            pltpu.VMEM((T1 * 32, DM), U32),
            pltpu.VMEM((T1 * 32, DM), U32),
            pltpu.VMEM((MEM, DM), BF16),
            pltpu.VMEM((16, 128), BF16),
            pltpu.VMEM((16, 128), F32),
            pltpu.VMEM((8, 128), U32),
            pltpu.VMEM((FH, DM), U32),
            pltpu.VMEM((S // 2, S), U32),
            pltpu.VMEM((FH // 2, DM), U32),
            pltpu.VMEM((64, NSUM * 128), U32),
            pltpu.VMEM((48, DM + 8, DH), U32),
            pltpu.VMEM((3 * H, DM // 2, DH), U32),
            pltpu.VMEM((3 * NGRP, 64, NSUM * 128), U32),
            pltpu.VMEM((H * DH // 2, DM), U32),
            pltpu.VMEM((NGRP, 64, NSUM * 128), U32),
            pltpu.VMEM((T1, FH, 128), F32),
            pltpu.VMEM((T1, 2 * (FH // RB) * 8, 128), F32),
            pltpu.VMEM((FH // 2, S), U32),
            pltpu.VMEM((NTILE // 2, FH // 4, 7 * 128), U32),
            pltpu.VMEM((64, 4 * S // 2), U32),
            pltpu.VMEM((64, 4 * S // 2), U32),
            pltpu.VMEM((64, FH), U32),
            pltpu.VMEM((96, H * DH), U32),
            pltpu.VMEM((80, H * DH), U32),
            pltpu.VMEM((80, H * DH), U32),
            pltpu.VMEM((32, H * DH), U32),
            pltpu.VMEM((4, 48, 80), F32),
            pltpu.VMEM((S, DM), BF16),
            pltpu.SemaphoreType.DMA((4,)),
            pltpu.SemaphoreType.DMA((8,)),
            pltpu.SemaphoreType.DMA((NTILE // T2,)),
            pltpu.SemaphoreType.DMA((NTILE // T2,)),
            pltpu.SemaphoreType.DMA,
        ],
        compiler_params=pltpu.CompilerParams(vmem_limit_bytes=112 * 1024 * 1024),
    )(
        A_x.reshape(S, DM),
        A_mem0.reshape(MEM, DM),
        A_Wq, A_Wk, A_Wv,
        A_Wo.reshape(H * DH, DM),
        B_w_in.T,
        B_w_sp,
        B_b_sp.reshape(16, 128),
        B_w_out,
    )
    return out.reshape(1, S, DM)
```

```python
import functools

import jax
import jax.numpy as jnp
import jax.experimental.pallas as pl
import jax.experimental.pallas.tpu as pltpu

F32 = jnp.float32
BF16 = jnp.bfloat16
U32 = jnp.uint32

S = 2048
DM = 640
H = 32
DH = 128
MEM = 8
SEG = 32
FH = 864
NTILE = S // 128
EPS = 1e-5
SCALE = DH ** (-0.5)
NEG = -1000000000.0

XCH = 256
T1 = 4
T2 = 4
RB = 144
WIN_PIECES = (2, 4, 6)
SBLK = (144, 144, 144)
SIDE_TAIL = 1
WSP_HEAD = 640
LN_DEADLINE = 10
LN_FIRST = 5
NORM_TAIL = 4
ORDER0 = (1, 0, 2)
PIPE = ((270, 450, 170, 0), (230, 540, 128, 2), (270, 510, 112, 4), (230, 450, 128, 1))
WG = 4
FILL = (320, 224, 224)

NT = (((1,), (1,)), ((), ()))


def _as_bf16(u):
    return pltpu.bitcast(u, BF16)


def _as_u32(b):
    return pltpu.bitcast(b, U32)


def _layernorm(v):
    m = jnp.mean(v, axis=-1, keepdims=True)
    c = v - m
    var = jnp.mean(c * c, axis=-1, keepdims=True)
    return c * jax.lax.rsqrt(var + EPS)


def _gelu2(v):
    c = 0.7978845608028654
    return v + v * jnp.tanh(v * (c + (c * 0.044715) * (v * v)))


def _mult(v, m):
    return v if isinstance(v, int) else pl.multiple_of(v, m)


def _lanes(tile):
    return pl.ds(_mult(tile * 128, 128), 128)


def _mask(qgroups, kgroups):
    shape = (8 * len(qgroups), 8 * len(kgroups))

    def table(groups, axis):
        idx = jax.lax.broadcasted_iota(jnp.int32, shape, axis)
        seg = jnp.full(shape, groups[-1][0], jnp.int32)
        pos = idx + (groups[-1][1] - 8 * (len(groups) - 1))
        for g in range(len(groups) - 2, -1, -1):
            inside = idx < 8 * (g + 1)
            seg = jnp.where(inside, groups[g][0], seg)
            pos = jnp.where(inside, idx + (groups[g][1] - 8 * g), pos)
        return seg, pos

    qseg, qpos = table(qgroups, 0)
    kseg, kpos = table(kgroups, 1)
    same = qseg == kseg
    keep = same & ((qpos < MEM) | (qpos >= kpos))
    return keep, jnp.where(same, NEG, -jnp.inf).astype(F32)


def _masks():
    own = lambda sg: [(sg, 0), (sg, 16), (sg, 24), (sg, 32)]
    k0 = [(0, 0), (0, 8), (0, 16), (0, 24), (0, 32), (1, 8)]
    k2 = own(2) + [(2, 8), (3, 8)]
    return [
        _mask(k0[:4], k0),
        _mask(own(1) + k0[4:], own(1) + k0),
        _mask(own(2), k2),
        _mask(own(3) + k2[4:], own(3) + k2),
    ]


def _fast_table(types):
    lines = {0: ((1, 0), (1, -1)), 1: ((0, 1), (1, -1)), 2: ((1, 0), (0, 1))}
    neg = lambda f: (-f[0], -f[1])

    def dual(u, v):
        det = u[0] * v[1] - u[1] * v[0]
        return (v[1] * det, -v[0] * det), (-u[1] * det, u[0] * det)

    n = len(types)
    diag = {(i, k): {(i, i): 1} for i in range(n) for k in range(2)}
    units = [[] for _ in range(n)]
    for i in range(n):
        u = lines[types[i]]
        units[i] += [('p', [(i, u[k])], diag[i, k], [(i, dual(*u)[k])]) for k in range(2)]
        for j in range(i + 1, n):
            if types[i] == types[j]:
                units[i] += [('b', i, j), ('b', j, i)]
                continue
            w = lines[types[j]]
            (ci, cj), = [(x, y) for x in range(2) for y in range(2) if u[x] == w[y]]
            (p, q), = [(x, y) for x in (u[1 - ci], neg(u[1 - ci])) for y in (w[1 - cj], neg(w[1 - cj]))
                       if (x[0] - y[0], x[1] - y[1]) == u[ci]]
            sd, td = dual(p, q)
            units[i] += [('p', [(i, p), (j, q)], {(i, j): 1, (j, i): 1}, [(i, td), (j, sd)]),
                         ('p', [(i, q), (j, q)], {(i, j): 1}, [(i, neg(td)), (j, td)]),
                         ('p', [(i, p), (j, p)], {(j, i): 1}, [(i, sd), (j, neg(sd))])]
            diag[i, ci][i, j] = 1
            diag[i, 1 - ci][j, i] = -1
            diag[j, 1 - cj][i, j] = -1
            diag[j, cj][j, i] = 1
    out = []
    for i in range(n):
        row = []
        for un in units[i]:
            if un[0] == 'p' and [c for c in un[1][0][1] if c][0] < 0:
                un = ('p', [(k, neg(f)) for k, f in un[1]], un[2], [(k, neg(f)) for k, f in un[3]])
            row.append(un)
        out.append(row)
    return out


GH = 5
NGRP = H // GH
UNITS = _fast_table((0, 1, 2, 0, 1))
SUMS = [un[2] for row in UNITS for un in row if un[0] == 'p' and len(un[2]) > 1]
NSUM = len(SUMS)


def _signed_sum(terms):
    terms = sorted(terms, key=lambda cv: -cv[0])
    acc = terms[0][1]
    for c, v in terms[1:]:
        acc = acc + v if c > 0 else acc - v
    return acc


def _lhs_operands(top, bot):
    forms = {}

    def form(i, f):
        sign = 1 if [c for c in f if c][0] > 0 else -1
        key = (i, (sign * f[0], sign * f[1]))
        if key not in forms:
            forms[key] = {(1, 0): lambda: top[i], (0, 1): lambda: bot[i],
                          (1, -1): lambda: top[i] - bot[i]}[key[1]]()
        return sign, forms[key]

    return lambda un: _signed_sum([form(i, f) for i, f in un[1]]).astype(BF16)


class _Acc:
    def __init__(self):
        self.v = {}

    def add(self, key, c, p):
        if key not in self.v:
            self.v[key] = (c, p)
        else:
            sign, v = self.v[key]
            self.v[key] = (sign, v + p if sign == c else v - p)

    def pop(self, key):
        sign, v = self.v.pop(key)
        return v if sign > 0 else -v


def _kernel(x_hbm, mem0_hbm, wq_hbm, wk_hbm, wv_hbm, wo_hbm, wint_hbm, wsp_hbm,
            bsp_hbm, wout_hbm, out_hbm,
            x_v, xn_v, xa_v, xb_v, mem0_v, bsp_v, bsp32_v, zero_v, wint_v, wins_v, wsp_v, wout_v, woutc_v,
            stage_v, wqkv_v, wc_v, wo_v, woc_v, zg_v, st_v, z1t_v, za_v, ta_v, tb_v, u_v, q_v, k_v, v_v, o_v, cap_v, out_v,
            sem_x, sem_w, sem_st, sem_wo, sem_out):
    NRB = FH // RB
    NG = RB // 8
    NB2 = NTILE // T2
    PPB = 48 // NB2

    x_parts = [(0, XCH), (XCH, XCH), (2 * XCH, XCH), (3 * XCH, S - 3 * XCH)]
    x_cps = [pltpu.make_async_copy(x_hbm.at[pl.ds(o, n), :], x_v.at[pl.ds(o, n), :], sem_x.at[k])
             for k, (o, n) in enumerate(x_parts)]
    wint_u = wint_hbm.bitcast(U32)
    blk_row = lambda k: (FH + k * RB) if k < NRB else (k - NRB) * RB
    wint_cps, k0 = [], 0
    for k, nb in enumerate(WIN_PIECES):
        o, n = blk_row(k0) // 2, nb * RB // 2
        wint_cps.append(pltpu.make_async_copy(wint_u.at[pl.ds(o, n), :], wint_v.at[pl.ds(o, n), :],
                                              sem_w.at[k]))
        k0 += nb
    wsp_u = wsp_hbm.bitcast(U32)
    wsp_cp = pltpu.make_async_copy(wsp_u.at[pl.ds(0, WSP_HEAD), :], wsp_v.at[pl.ds(0, WSP_HEAD), :],
                                   sem_w.at[3])
    wsp_cp2 = pltpu.make_async_copy(wsp_u.at[pl.ds(WSP_HEAD, S // 2 - WSP_HEAD), :],
                                    wsp_v.at[pl.ds(WSP_HEAD, S // 2 - WSP_HEAD), :], sem_w.at[7])
    wout_cp = pltpu.make_async_copy(wout_hbm.bitcast(U32), wout_v, sem_w.at[4])
    WOQ = H * DH // 2 // NB2

    def wo_copy(i):
        r0 = _mult(i * WOQ, WOQ)
        return pltpu.make_async_copy(wo_hbm.bitcast(U32).at[pl.ds(r0, WOQ), :],
                                     wo_v.at[pl.ds(r0, WOQ), :], sem_wo.at[i])

    mem0_cp = pltpu.make_async_copy(mem0_hbm, mem0_v, sem_w.at[5])
    bsp_cp = pltpu.make_async_copy(bsp_hbm, bsp_v, sem_w.at[6])
    w_hbms = (wq_hbm, wk_hbm, wv_hbm)

    def stage_copy(m, j):
        p = m * 16 + j
        return pltpu.make_async_copy(w_hbms[m].bitcast(U32).at[:, j, :],
                                     stage_v.at[p, pl.ds(0, DM), :], sem_st.at[p // PPB])

    x_cps[0].start()
    x_cps[1].start()
    for cp in wint_cps:
        cp.start()
    x_cps[2].start()
    x_cps[3].start()
    bsp_cp.start()
    wsp_cp.start()
    wout_cp.start()
    for p in range(48):
        stage_copy(p // 16, p % 16).start()
        if (p + 1) % PPB == 0:
            wo_copy(p // PPB).start()
        if p + 1 == 2 * PPB:
            wsp_cp2.start()
    mem0_cp.start()

    zero_v[...] = jnp.zeros((8, 128), U32)

    pending = []

    def dep_of(v):
        return pltpu.bitcast(v[0:8, 0:128], U32) & zero_v[...]

    def up(u):
        return _as_bf16(u).astype(F32)

    def ln_rows(r0, n, dep=None):
        xr = x_v[pl.ds(r0, n), :].astype(F32)
        if dep is not None:
            d = jnp.concatenate([dep] * (n // 8), axis=0)
            xr = pltpu.bitcast(pltpu.bitcast(xr, U32) | jnp.concatenate([d] * (DM // 128), axis=1), F32)
        xn = _layernorm(xr)
        xn_v[pl.ds(_mult(r0 // 2, n // 2), n // 2), :] = _as_u32(xn.astype(BF16))
        return xn

    def ln_pair(base, k, dst, dep):
        xe = ln_rows(_mult(base + 16 * k, 16), 16, dep)
        xo = ln_rows(_mult(base + 128 + 16 * k, 16), 16, dep)
        b11, b21, b12, b22 = xe[:, 0:256], xe[:, 256:512], xo[:, 0:256], xo[:, 256:512]
        t1 = b12 - b11
        t2 = b22 - t1
        ops = jnp.concatenate([xe, xo[:, 256:], b21 - t2, xe[:, 512:], t1, t2, b22 - b12], axis=1)
        dst[8 * k:8 * k + 8, :] = _as_u32(ops.astype(BF16))
        pending.append([LN_DEADLINE, dst[8 * k:8 * k + 8, 1024:1152] & zero_v[...]])

    def win_sums(hz, k, dep):
        d = jnp.concatenate([dep] * 4, axis=1)
        r0 = hz * (FH // 2) + 8 * k
        top, bot = up(wint_v[r0:r0 + 8, 0:512] | d), up(wint_v[r0 + FH // 4:r0 + FH // 4 + 8, 0:512] | d)
        a11, a12, a21, a22 = top[:, 0:256], top[:, 256:512], bot[:, 0:256], bot[:, 256:512]
        s1 = a21 + a22
        s2 = s1 - a11
        ops = jnp.concatenate([s1, s2, a11 - a21, a12 - s2], axis=1)
        wins_v[hz * (FH // 4) + 8 * k:hz * (FH // 4) + 8 * k + 8, :] = _as_u32(ops.astype(BF16))

    def nt_dot(w, xt):
        due = None
        for e in pending:
            e[0] -= 1
            if e[0] == 0:
                due = e[1] if due is None else due | e[1]
        pending[:] = [e for e in pending if e[0] > 0]
        if due is not None:
            top = w[0:8, 0:128] | due
            if w.shape[1] > 128:
                top = jnp.concatenate([top, w[0:8, 128:]], axis=1)
            w = jnp.concatenate([top, w[8:]], axis=0)
        return jax.lax.dot_general(_as_bf16(w), _as_bf16(xt), NT, preferred_element_type=F32)

    def win_block(nt, f0):
        return nt_dot(wint_v[f0 // 2:(f0 + RB) // 2, :], xn_v[nt * 64:(nt + 1) * 64, :])

    def win_group(src, hz, rb, emit, side, late):
        rt = (hz * FH + rb * RB) // 2
        rows = lambda r: slice(r, r + RB // 2)
        top, bot, sm = rows(rt), rows(rt + FH // 4), rows(hz * (FH // 4) + rb * RB // 2)
        ss = lambda q: wins_v[sm, q * 256:(q + 1) * 256]
        tt = lambda q: src[:, 1408 + q * 256:1408 + (q + 1) * 256]

        def prod(w, xt):
            p = nt_dot(w, xt)
            side(p)
            return p

        p1 = prod(wint_v[top, 0:256], src[:, 0:256])
        emit(0, rb, p1 + prod(wint_v[top, 256:640], src[:, 256:640]))
        u2 = p1 + prod(ss(1), tt(1))
        if late is not None:
            late()
        u3 = u2 + prod(ss(2), tt(2))
        emit(0, rb + NRB // 2, u3 + prod(wint_v[bot, 256:640], src[:, 1024:1408]))
        l22 = prod(wint_v[bot, 512:640], src[:, 896:1024])
        p5 = prod(ss(0), tt(0))
        emit(1, rb + NRB // 2, u3 + l22 + p5)
        u4 = u2 + p5
        return lambda: emit(1, rb, u4 + prod(
            jnp.concatenate([ss(3), wint_v[top, 512:640]], axis=1), src[:, 640:1024]))

    def z2_emit(nt, rb, z):
        g = _gelu2(z)
        zg_v[nt, rb * RB:(rb + 1) * RB, :] = g
        g3 = g.reshape(NG, 8, 128)
        bm = jnp.sum(g3, axis=0) * (1.0 / NG)
        c = g3 - bm
        st_v[nt, rb * 8:(rb + 1) * 8, :] = bm
        st_v[nt, (NRB + rb) * 8:(NRB + rb + 1) * 8, :] = jnp.sum(c * c, axis=0)

    def z2_stats(nt):
        bm = st_v[nt, 0:NRB * 8, :]
        m = jnp.sum(bm, axis=0, keepdims=True) * (1.0 / (NRB * 8))
        dm = bm - m
        m2 = jnp.sum(st_v[nt, NRB * 8:2 * NRB * 8, :] + dm * dm * NG, axis=0, keepdims=True)
        r = jax.lax.rsqrt(m2 * (1.0 / FH) + 4.0 * EPS)
        return jnp.broadcast_to(m, (8, 128)), jnp.broadcast_to(r, (8, 128))

    def z2_norm(ne, tp, k, st, dep):
        (me, re), (mo, ro) = st
        me = pltpu.bitcast(pltpu.bitcast(me, U32) | dep, F32)
        mo = pltpu.bitcast(pltpu.bitcast(mo, U32) | dep, F32)
        nrm = lambda nt, f0, m, r: ((zg_v[nt, f0:f0 + 16, :].reshape(2, 8, 128) - m) * r).reshape(16, 128)
        a11, a21 = nrm(ne, 16 * k, me, re), nrm(ne, FH // 2 + 16 * k, me, re)
        a12, a22 = nrm(ne + 1, 16 * k, mo, ro), nrm(ne + 1, FH // 2 + 16 * k, mo, ro)
        s1 = a21 + a22
        s2 = s1 - a11
        ops = jnp.concatenate([a11, a12, a12 - s2, a22, s1, s2, a11 - a21], axis=1)
        za_v.at[tp][8 * k:8 * k + 8, :] = _as_u32(ops.astype(BF16))

    def z1_emit(tile, rb, z):
        z1t_v[rb * RB // 2:(rb + 1) * RB // 2, _lanes(tile)] = _as_u32(_gelu2(z).astype(BF16))

    def spread(tasks, slots):
        state = [0]

        def side(p):
            n = state[0]
            mine = tasks[n * len(tasks) // slots:(n + 1) * len(tasks) // slots]
            for q, fn in enumerate(mine):
                fn(dep_of(p[8 * ((q * NG) // len(mine)):]))
            state[0] += 1

        return side

    def mix(*kinds):
        order = sorted(((q + 0.5) / len(kd), kn, q) for kn, kd in enumerate(kinds) for q in range(len(kd)))
        return [kinds[kn][q] for _, kn, q in order]

    part = functools.partial
    NSLAB = FH // 32

    x_cps[0].wait()
    ln_rows(0, XCH)
    x_cps[1].wait()
    ln_rows(XCH, XCH)
    wint_cps[0].wait()
    for nt in range(T1):
        for rb in range(WIN_PIECES[0]):
            z2_emit(nt, rb, win_block(nt, FH + rb * RB))
    wint_cps[1].wait()
    side = spread([part(win_sums, 1, k) for k in range(NSLAB)], T1 * (NRB - WIN_PIECES[0]) - 1)
    for nt in range(T1):
        for rb in range(WIN_PIECES[0], NRB):
            z = win_block(nt, FH + rb * RB)
            z2_emit(nt, rb, z)
            side(z)
    wint_cps[2].wait()
    x_cps[2].wait()
    norms = []
    for ne in range(0, T1, 2):
        st = (z2_stats(ne), z2_stats(ne + 1))
        norms += [part(z2_norm, ne, ne // 2, k, st) for k in range(NSLAB)]
    side = spread(mix(norms, [part(win_sums, 0, k) for k in range(NSLAB)],
                      [part(ln_pair, T1 * 128, k, xa_v) for k in range(8)]), T1 * NRB - 1)
    for nt in range(T1):
        for rb in range(NRB):
            z = win_block(nt, rb * RB)
            z1_emit(nt, rb, z)
            side(z)
    x_cps[3].wait()
    pending.clear()

    def b1_body(i, carry):
        for ne in range(0, T1, 2):
            tile = i * T1 + ne
            src, dst = (xa_v, xb_v) if ne == 0 else (xb_v, xa_v)
            base = jnp.minimum(tile + 2, NTILE - 2) * 128
            lns = [part(ln_pair, base, k, dst) for k in range(8)]
            side = spread(lns[:LN_FIRST], 8 * NRB // 2)
            late = None
            for rb in range(NRB // 2):
                late = win_group(src, 1, rb, lambda o, r, z: z2_emit(ne + o, r, z), side, late)
            late()
            st = (z2_stats(ne), z2_stats(ne + 1))
            norms = [part(z2_norm, ne, tile // 2, k, st) for k in range(NSLAB)]
            side = spread(mix(norms, lns[LN_FIRST:]) if LN_FIRST < 8 else norms, 8 * NRB // 2 - NORM_TAIL)
            late = None
            for rb in range(NRB // 2):
                late = win_group(src, 0, rb, lambda o, r, z: z1_emit(tile + o, r, z), side, late)
            late()
        pending.clear()
        return carry

    jax.lax.fori_loop(1, NTILE // T1, b1_body, 0)

    wsp_cp.wait()
    wout_cp.wait()
    bsp_cp.wait()
    bsp32_v[...] = 0.5 * bsp_v[...].astype(F32)

    def split_block(p, bi, dep):
        a = stage_v[p, pl.ds(128 * bi, 64, stride=2), :] | dep
        b = stage_v[p, pl.ds(128 * bi + 1, 64, stride=2), :] | dep
        wqkv_v[2 * p, 64 * bi:64 * bi + 64, :] = (a & jnp.uint32(0xFFFF)) | (b << 16)
        wqkv_v[2 * p + 1, 64 * bi:64 * bi + 64, :] = (a >> 16) | (b & jnp.uint32(0xFFFF0000))

    def weight_sums(block, dst, rows, idx, dep):
        cache = {}

        def blk(ij):
            if ij not in cache:
                w = block(*ij)
                cache[ij] = up(w | dep[0:w.shape[0]])
            return cache[ij]

        mine = [un[2] for un in UNITS[idx] if un[0] == 'p' and len(un[2]) > 1]
        c0 = SUMS.index(mine[0])
        sums = jnp.concatenate([_signed_sum([(c, blk(ij)) for ij, c in r.items()]) for r in mine], axis=1)
        dst[rows, c0 * 128:(c0 + len(mine)) * 128] = _as_u32(sums.astype(BF16))

    fblocks = [(f0, min(128, FH - f0)) for f0 in range(0, FH, 128)]

    def u_transpose(tile):
        for f0, fn in fblocks:
            ut = _as_bf16(z1t_v[f0 // 2:(f0 + fn) // 2, _lanes(tile)]).astype(F32)
            u_v[:, f0:f0 + fn] = _as_u32(ut.T.astype(BF16))

    NK = NTILE // 2

    def t_piece(tp, dst, k, dep=None):
        h0 = _mult(tp * 128, 128)
        we = wsp_v[pl.ds(h0, 64), k * 256:(k + 1) * 256]
        wo = wsp_v[pl.ds(h0 + 64, 64), k * 256:(k + 1) * 256]
        if dep is not None:
            d = jnp.concatenate([dep, dep], axis=1)
            we, wo = we | d, wo | d
        we, wo = up(we), up(wo)
        b11, b21, b12, b22 = we[:, 0:128], we[:, 128:256], wo[:, 0:128], wo[:, 128:256]
        t1 = b12 - b11
        t2 = b22 - t1
        ops = jnp.concatenate([t1, t2, b22 - b12, t2 - b21], axis=1)
        dst[:, k * 512:(k + 1) * 512] = _as_u32(ops.astype(BF16))

    for k in range(NK):
        t_piece(0, ta_v, k)

    def b2_body(i, carry):
        group = stage_v.at[pl.ds(i * PPB, PPB), pl.ds(0, DM), :]
        pltpu.make_async_copy(group, group, sem_st.at[i]).wait()
        wo_copy(i).wait()

        @pl.when(i == 2)
        def _():
            wsp_cp2.wait()

        u_transpose(0)
        for lp in range(2):
            tp = i * 2 + lp
            cur, nxt = (ta_v, tb_v) if lp == 0 else (tb_v, ta_v)
            tpn = jnp.minimum(tp + 1, NK - 1)
            he = pl.multiple_of(tp * 128, 128)
            raw = lambda odd_t, odd_s: lambda k: wsp_v[
                pl.ds(he + odd_t * 64, 64), (2 * k + odd_s) * 128:(2 * k + odd_s + 1) * 128]
            tj = lambda j: lambda k: cur[:, k * 512 + j * 128:k * 512 + (j + 1) * 128]
            rhs = [raw(0, 0), raw(0, 1), raw(1, 1), tj(3), tj(0), tj(1), tj(2)]

            part = functools.partial
            full = slice(0, 64)
            kinds = [[(25, part(t_piece, tpn, nxt, k)) for k in range(NK)], []]
            if lp == 0:
                kinds[1] = [(9, part(split_block, i * PPB + pp, bi)) for pp in range(PPB) for bi in range(GH)]
            else:
                for sl in range(5):
                    gid = jnp.minimum((9 * i) // 2 + sl, (9 * i + 9) // 2 - 1)
                    f0h = (gid // NGRP) * H + (gid % NGRP) * GH
                    block = lambda bi, bj, f0h=f0h: wqkv_v[f0h + bj, 64 * bi:64 * bi + 64, :]
                    kinds[1] += [(30, part(weight_sums, block, wc_v.at[gid], full, idx)) for idx in range(GH)]
            if lp == 0:
                kinds.append([])
                for sl in range(2):
                    gid = jnp.minimum((3 * i) // 2 + sl, (3 * i + 3) // 2 - 1)
                    block = lambda bi, bj, gid=gid: wo_v[
                        pl.ds(pl.multiple_of((gid * GH + bi) * 64, 64), 64), bj * 128:(bj + 1) * 128]
                    kinds[-1] += [(30, part(weight_sums, block, woc_v.at[gid], full, idx)) for idx in range(GH)]
            r8 = pl.multiple_of(8 * (2 * i + lp), 8)
            block = lambda bi, bj, r8=r8: wout_v[pl.ds(64 * bi + r8, 8), bj * 128:(bj + 1) * 128]
            kinds.append([(4, part(weight_sums, block, woutc_v, pl.ds(r8, 8), idx)) for idx in range(GH)])
            order = sorted(((q + 0.5) / len(kd), kn, q) for kn, kd in enumerate(kinds) for q in range(len(kd)))
            tasks = [kinds[kn][q] for _, kn, q in order]
            budget = sum(c for c, _ in tasks) / (2 * 7 * len(SBLK) - SIDE_TAIL)
            state = [0.0]

            def side(p):
                state[0] += budget
                phase = 0
                while tasks and state[0] > 0:
                    c, fn = tasks.pop(0)
                    rows = p[0:128].reshape(8, 16, 128)[:, 8 * phase:8 * phase + 8, :]
                    fn((pltpu.bitcast(rows, U32) & zero_v[...]).reshape(64, 128))
                    state[0] -= c
                    phase = 1 - phase

            def prod(j, f0, fn):
                p = None
                for ks in (range(NK // 2), range(NK // 2, NK)):
                    lhs = jnp.concatenate(
                        [za_v[k, f0 // 2:(f0 + fn) // 2, j * 128:(j + 1) * 128] for k in ks], axis=1)
                    r = jnp.concatenate([rhs[j](k) for k in ks], axis=1)
                    q = jax.lax.dot_general(_as_bf16(lhs), _as_bf16(r), NT, preferred_element_type=F32)
                    side(q)
                    p = q if p is None else p + q
                return p

            def finish(c, f0, fn, odd_t):
                tile = tp * 2 + odd_t
                z1 = _as_bf16(z1t_v[f0 // 2:(f0 + fn) // 2, _lanes(tile)]).astype(F32)
                brow = bsp32_v[pl.ds(tile, 1), :]
                z1t_v[f0 // 2:(f0 + fn) // 2, _lanes(tile)] = _as_u32((z1 * (0.5 * c + brow)).astype(BF16))

            f0 = 0
            for fn in SBLK:
                p1 = prod(0, f0, fn)
                finish(p1 + prod(1, f0, fn), f0, fn, 0)
                u2 = p1 + prod(5, f0, fn)
                u3 = u2 + prod(6, f0, fn)
                p5 = prod(4, f0, fn)
                finish(u3 + p5, FH // 2 + f0, fn, 1)
                u4 = u2 + p5
                finish(u3 - prod(3, f0, fn), FH // 2 + f0, fn, 0)
                finish(u4 + prod(2, f0, fn), f0, fn, 1)
                f0 += fn
            assert not tasks
        return carry

    jax.lax.fori_loop(0, NB2, b2_body, 0)
    mem0_cp.wait()

    masks = _masks()
    for n, (keep, fill) in enumerate(masks):
        cap_v[n, 0:keep.shape[0], 0:keep.shape[1]] = jnp.where(keep, 0.0, fill)
    dot = lambda l, r: jnp.dot(l, r, preferred_element_type=F32)

    def fast_units(lhs_of, both, raw, sums, acc, done):
        items = []
        for i, row in enumerate(UNITS):
            for q, un in enumerate(row):
                def fn(un=un, last=(q == len(row) - 1), i=i):
                    if un[0] == 'b':
                        p = dot(both(un[1]), raw(un[1], un[2]))
                        hr = p.shape[0] // 2
                        acc.add((0, un[2]), 1, p[0:hr])
                        acc.add((1, un[2]), 1, p[hr:])
                    else:
                        r = un[2]
                        p = dot(lhs_of(un), raw(*list(r)[0]) if len(r) == 1 else sums(SUMS.index(r)))
                        for k, f in un[3]:
                            for half in range(2):
                                if f[half]:
                                    acc.add((half, k), f[half], p)
                    if last:
                        done(i)
                items.append((16 if un[0] == 'b' else 8, fn))
        return items

    def step(n, h):
        odd = n % 2 == 1
        hb = h.astype(BF16)
        qb = 24 * n
        kb = 40 * (n // 2) + (0 if odd else 16)
        nq, nk = (24, 40) if odd else (16, 24)
        clock = [0]
        d_s, d_o, gap, lag_v = PIPE[n]
        ready, s_at, o_at, ps = {}, {}, {}, {}

        def put(buf, r0, t, v):
            buf[r0:r0 + v.shape[0] // 2, _lanes(t)] = _as_u32(v.astype(BF16))

        def put64(m, t, top, bot):
            buf = (q_v, k_v, v_v)[m]
            if m == 0:
                put(buf, 0, t, top)
                put(buf, 24 + 16, t, bot[0:16])
                put(buf, 72 + 16, t, bot[16:32])
            else:
                put(buf, 16, t, top)
                put(buf, 32, t, bot[0:16])
                put(buf, 40 + 32, t, bot[16:32])
            ready[m, t] = clock[0]

        def plain(m, t):
            r = dot(hb, _as_bf16(wqkv_v[m * H + t]))
            if n == 0:
                put64(m, t, r[0:32], r[32:64])
            else:
                put((q_v, k_v, v_v)[m], qb if m == 0 else kb, t, r)
                ready[m, t] = clock[0]

        work = []
        if n == 0:
            cols = lambda i: slice(i * 128, (i + 1) * 128)
            make = _lhs_operands([h[0:32, cols(i)] for i in range(GH)], [h[32:64, cols(i)] for i in range(GH)])
            ops = {id(un): make(un) for row in UNITS for un in row if un[0] == 'p'}
            for g in range(NGRP):
                for m in ORDER0:
                    if g == NGRP - 1 and m == 2:
                        work += [(80, functools.partial(plain, mm, t))
                                 for t in range(NGRP * GH, H) for mm in (1, 0)]
                    acc = _Acc()
                    work += fast_units(
                        lambda un: ops[id(un)], lambda i: hb[:, cols(i)],
                        lambda i, j, m=m, g=g: _as_bf16(wqkv_v[m * H + g * GH + j, 64 * i:64 * i + 64, :]),
                        lambda q, m=m, g=g: _as_bf16(wc_v[m * NGRP + g, :, q * 128:(q + 1) * 128]),
                        acc, lambda j, m=m, g=g, acc=acc: put64(m, g * GH + j, acc.pop((0, j)), acc.pop((1, j))))
            work += [(80, functools.partial(plain, 2, t)) for t in range(NGRP * GH, H)]
        else:
            for t in range(H + lag_v):
                for m, tt in ((1, t), (2, t - lag_v), (0, t)):
                    if 0 <= tt < H:
                        work.append((40, functools.partial(plain, m, tt)))
        work = [(c, fn, -1) for c, fn in work]

        res = []
        if n == 3:
            acc = _Acc()
            for g in range(NGRP):
                hc = lambda i, g=g: slice((g * GH + i) * DH, (g * GH + i + 1) * DH)
                box = []

                def lhs_of(un, box=box, hc=hc):
                    if not box:
                        box.append(_lhs_operands([up(o_v[0:16, hc(i)]) for i in range(GH)],
                                                 [up(o_v[16:32, hc(i)]) for i in range(GH)]))
                    return box[0](un)

                items = fast_units(
                    lhs_of, lambda i, hc=hc: _as_bf16(o_v[:, hc(i)]),
                    lambda i, j, g=g: _as_bf16(wo_v[(g * GH + i) * 64:(g * GH + i + 1) * 64, j * 128:(j + 1) * 128]),
                    lambda q, g=g: _as_bf16(woc_v[g, :, q * 128:(q + 1) * 128]), acc, lambda j: None)
                work += [(c, fn, g * GH + GH - 1) for c, fn in items]

            def tail():
                c0 = NGRP * GH * DH
                part = dot(_as_bf16(o_v[:, c0:]), _as_bf16(wo_v[c0 // 2:, :]))
                res.append(part + jnp.concatenate(
                    [jnp.concatenate([acc.pop((hf, j)) for j in range(GH)], axis=1) for hf in range(2)], axis=0))

            work.append((160, tail, H - 1))
        else:
            def wgroup(g):
                c0, c1 = g * WG * DH, (g + 1) * WG * DH
                part = dot(_as_bf16(o_v[0:16, c0:c1]), _as_bf16(wo_v[c0 // 2:c1 // 2, :]))
                res[:] = [part + res[0]] if res else [part]

            work += [(40 * WG, functools.partial(wgroup, g), (g + 1) * WG - 1) for g in range(H // WG)]

        def scores(t):
            sc = jax.lax.dot_general(_as_bf16(q_v[qb:qb + nq, _lanes(t)]),
                                     _as_bf16(k_v[kb:kb + nk, _lanes(t)]), NT,
                                     preferred_element_type=F32) * SCALE
            cap = cap_v[n, 0:sc.shape[0], 0:sc.shape[1]]
            sc = jnp.where(cap == 0.0, sc, cap)
            e = jnp.exp(sc - jnp.max(sc, axis=-1, keepdims=True))
            l = jnp.sum(e, axis=-1, keepdims=True)
            inv = pl.reciprocal(l, approx=True)
            inv = inv * (2.0 - l * inv)
            ps[t] = (e * inv).astype(BF16)
            s_at[t] = clock[0]
            clock[0] += nq // 2

        def values(t):
            o = dot(ps.pop(t), _as_bf16(v_v[kb:kb + nk, _lanes(t)]))
            if n == 1:
                put(o_v, 0, t, o[0:32])
                put(o_v, 24, t, o[32:48])
            else:
                put(o_v, 0, t, o)
            o_at[t] = clock[0]
            clock[0] += nq // 2

        def drain(upto):
            while True:
                to, ts = len(o_at), len(s_at)
                if to < ts and (2, to) in ready and (
                        to <= upto or clock[0] >= max(s_at[to] + d_o, ready[2, to] + d_s)):
                    values(to)
                elif ts < H and (0, ts) in ready and (1, ts) in ready and (
                        ts <= upto or clock[0] >= max(ready[0, ts] + d_s, ready[1, ts] + d_s,
                                                      s_at.get(ts - 1, -gap) + gap)):
                    scores(ts)
                else:
                    return

        for c, fn, need in work:
            drain(need)
            clock[0] += c
            fn()
        return res[0]

    def gate_work():
        acc = _Acc()
        cols = lambda i: slice(i * 128, (i + 1) * 128)
        box = []

        def lhs_of(un):
            if not box:
                box.append(_lhs_operands([up(u_v[0:32, cols(i)]) for i in range(GH)],
                                         [up(u_v[32:64, cols(i)]) for i in range(GH)]))
            return box[0](un)

        items = [(2 * c, fn) for c, fn in fast_units(
            lhs_of, lambda i: _as_bf16(u_v[:, cols(i)]),
            lambda i, j: _as_bf16(wout_v[64 * i:64 * i + 64, cols(j)]),
            lambda q: _as_bf16(woutc_v[:, cols(q)]), acc, lambda j: None)]

        def rest(j):
            p = dot(_as_bf16(u_v[:, DM:FH]), _as_bf16(wout_v[DM // 2:FH // 2, cols(j)]))
            acc.add((0, j), 1, p[0:64])
            acc.add((1, j), 1, p[64:128])

        items = [(64, functools.partial(rest, j)) for j in range(GH)] + items

        def chunk(budget):
            box.clear()
            while items and budget > 0:
                c, fn = items.pop(0)
                fn()
                budget -= c

        def result():
            hb = 0.5 * jnp.concatenate(
                [jnp.concatenate([acc.pop((hf, j)) for j in range(GH)], axis=1) for hf in range(2)], axis=0)
            return hb + hb * jnp.tanh(hb)

        return chunk, result

    def tile_body(j, mem):
        r0 = pl.multiple_of(j * 128, 128)
        xs = _as_bf16(xn_v[pl.ds(pl.multiple_of(j * 64, 64), 64), :]).astype(F32)
        chunk, gate_result = gate_work()
        chunk(FILL[0])
        a0 = step(0, jnp.concatenate([mem, xs[0:40], xs[64:72], xs[96:104]], axis=0))
        chunk(FILL[1])
        a1 = step(1, jnp.concatenate([a0[0:MEM], xs[40:64]], axis=0))
        chunk(FILL[2])
        a2 = step(2, jnp.concatenate([a1[0:MEM], xs[72:96]], axis=0))
        chunk(10 ** 6)
        gate = gate_result()
        u_transpose(jnp.minimum(j + 1, NTILE - 1))
        a3 = step(3, jnp.concatenate([a2[0:MEM], xs[104:128]], axis=0))
        s_rows = jnp.concatenate([a0[8:32], a3[48:64], a1[8:32], a3[32:40], a2[8:32], a3[40:48], a3[8:32]],
                                 axis=0)
        res = x_v[pl.ds(r0, 128), :].astype(F32) + s_rows * gate
        out_v[pl.ds(r0, 128), :] = res.astype(BF16)
        pltpu.make_async_copy(out_v.at[pl.ds(r0, 128), :],
                              out_hbm.at[pl.ds(r0, 128), :], sem_out).start()
        return a3[0:MEM]

    jax.lax.fori_loop(0, NTILE, tile_body, mem0_v[...].astype(F32))
    pltpu.make_async_copy(out_v, out_hbm, sem_out).wait()


@jax.jit
def pallas_recurrent_scan__memory_aug_recurrent_mem_tr__mixer_gmlp__prompt_kernel(
    A_x: jax.Array,
    A_mem0: jax.Array,
    A_Wq: jax.Array,
    A_Wk: jax.Array,
    A_Wv: jax.Array,
    A_Wo: jax.Array,
    A_seg_len: jax.Array,
    B_x: jax.Array,
    B_w_in: jax.Array,
    B_w_sp: jax.Array,
    B_b_sp: jax.Array,
    B_w_out: jax.Array,
):
    del A_seg_len, B_x
    hbm = pl.BlockSpec(memory_space=pl.ANY)
    out = pl.pallas_call(
        _kernel,
        out_shape=jax.ShapeDtypeStruct((S, DM), BF16),
        in_specs=[hbm] * 10,
        out_specs=hbm,
        scratch_shapes=[
            pltpu.VMEM((S, DM), BF16),
            pltpu.VMEM((S // 2, DM), U32),
            pltpu.VMEM((64, 2176), U32),
            pltpu.VMEM((64, 2176), U32),
            pltpu.VMEM((MEM, DM), BF16),
            pltpu.VMEM((16, 128), BF16),
            pltpu.VMEM((16, 128), F32),
            pltpu.VMEM((8, 128), U32),
            pltpu.VMEM((FH, DM), U32),
            pltpu.VMEM((FH // 2, 1024), U32),
            pltpu.VMEM((S // 2, S), U32),
            pltpu.VMEM((FH // 2, DM), U32),
            pltpu.VMEM((64, NSUM * 128), U32),
            pltpu.VMEM((48, DM + 8, DH), U32),
            pltpu.VMEM((3 * H, DM // 2, DH), U32),
            pltpu.VMEM((3 * NGRP, 64, NSUM * 128), U32),
            pltpu.VMEM((H * DH // 2, DM), U32),
            pltpu.VMEM((NGRP, 64, NSUM * 128), U32),
            pltpu.VMEM((T1, FH, 128), F32),
            pltpu.VMEM((T1, 2 * (FH // RB) * 8, 128), F32),
            pltpu.VMEM((FH // 2, S), U32),
            pltpu.VMEM((NTILE // 2, FH // 4, 7 * 128), U32),
            pltpu.VMEM((64, 4 * S // 2), U32),
            pltpu.VMEM((64, 4 * S // 2), U32),
            pltpu.VMEM((64, FH), U32),
            pltpu.VMEM((96, H * DH), U32),
            pltpu.VMEM((80, H * DH), U32),
            pltpu.VMEM((80, H * DH), U32),
            pltpu.VMEM((32, H * DH), U32),
            pltpu.VMEM((4, 48, 80), F32),
            pltpu.VMEM((S, DM), BF16),
            pltpu.SemaphoreType.DMA((4,)),
            pltpu.SemaphoreType.DMA((8,)),
            pltpu.SemaphoreType.DMA((NTILE // T2,)),
            pltpu.SemaphoreType.DMA((NTILE // T2,)),
            pltpu.SemaphoreType.DMA,
        ],
        compiler_params=pltpu.CompilerParams(vmem_limit_bytes=112 * 1024 * 1024),
    )(
        A_x.reshape(S, DM),
        A_mem0.reshape(MEM, DM),
        A_Wq, A_Wk, A_Wv,
        A_Wo.reshape(H * DH, DM),
        B_w_in.T,
        B_w_sp,
        B_b_sp.reshape(16, 128),
        B_w_out,
    )
    return out.reshape(1, S, DM)
```

```python
import functools

import jax
import jax.numpy as jnp
import jax.experimental.pallas as pl
import jax.experimental.pallas.tpu as pltpu

F32 = jnp.float32
BF16 = jnp.bfloat16
U32 = jnp.uint32

S = 2048
DM = 640
H = 32
DH = 128
MEM = 8
SEG = 32
FH = 864
NTILE = S // 128
EPS = 1e-5
SCALE = DH ** (-0.5)
NEG = -1000000000.0

XCH = 256
T1 = 4
T2 = 4
RB = 144
WIN_PIECES = (2, 4, 6)
SBLK = (144, 144, 144)
SIDE_TAIL = 1
WSP_HEAD = 640
LN_DEADLINE = 10
LN_FIRST = 4
NORM_TAIL = 4
ORDER0 = (1, 0, 2)
PIPE = ((270, 450, 170, 0), (230, 540, 128, 2), (270, 510, 112, 4), (230, 450, 128, 1))
WG = 4
FILL = (320, 224, 224)

NT = (((1,), (1,)), ((), ()))


def _as_bf16(u):
    return pltpu.bitcast(u, BF16)


def _as_u32(b):
    return pltpu.bitcast(b, U32)


def _layernorm(v):
    m = jnp.mean(v, axis=-1, keepdims=True)
    c = v - m
    var = jnp.mean(c * c, axis=-1, keepdims=True)
    return c * jax.lax.rsqrt(var + EPS)


def _gelu2(v):
    c = 0.7978845608028654
    return v + v * jnp.tanh(v * (c + (c * 0.044715) * (v * v)))


def _mult(v, m):
    return v if isinstance(v, int) else pl.multiple_of(v, m)


def _lanes(tile):
    return pl.ds(_mult(tile * 128, 128), 128)


def _mask(qgroups, kgroups):
    shape = (8 * len(qgroups), 8 * len(kgroups))

    def table(groups, axis):
        idx = jax.lax.broadcasted_iota(jnp.int32, shape, axis)
        seg = jnp.full(shape, groups[-1][0], jnp.int32)
        pos = idx + (groups[-1][1] - 8 * (len(groups) - 1))
        for g in range(len(groups) - 2, -1, -1):
            inside = idx < 8 * (g + 1)
            seg = jnp.where(inside, groups[g][0], seg)
            pos = jnp.where(inside, idx + (groups[g][1] - 8 * g), pos)
        return seg, pos

    qseg, qpos = table(qgroups, 0)
    kseg, kpos = table(kgroups, 1)
    same = qseg == kseg
    keep = same & ((qpos < MEM) | (qpos >= kpos))
    return keep, jnp.where(same, NEG, -jnp.inf).astype(F32)


def _masks():
    own = lambda sg: [(sg, 0), (sg, 16), (sg, 24), (sg, 32)]
    k0 = [(0, 0), (0, 8), (0, 16), (0, 24), (0, 32), (1, 8)]
    k2 = own(2) + [(2, 8), (3, 8)]
    return [
        _mask(k0[:4], k0),
        _mask(own(1) + k0[4:], own(1) + k0),
        _mask(own(2), k2),
        _mask(own(3) + k2[4:], own(3) + k2),
    ]


def _fast_table(types):
    lines = {0: ((1, 0), (1, -1)), 1: ((0, 1), (1, -1)), 2: ((1, 0), (0, 1))}
    neg = lambda f: (-f[0], -f[1])

    def dual(u, v):
        det = u[0] * v[1] - u[1] * v[0]
        return (v[1] * det, -v[0] * det), (-u[1] * det, u[0] * det)

    n = len(types)
    diag = {(i, k): {(i, i): 1} for i in range(n) for k in range(2)}
    units = [[] for _ in range(n)]
    for i in range(n):
        u = lines[types[i]]
        units[i] += [('p', [(i, u[k])], diag[i, k], [(i, dual(*u)[k])]) for k in range(2)]
        for j in range(i + 1, n):
            if types[i] == types[j]:
                units[i] += [('b', i, j), ('b', j, i)]
                continue
            w = lines[types[j]]
            (ci, cj), = [(x, y) for x in range(2) for y in range(2) if u[x] == w[y]]
            (p, q), = [(x, y) for x in (u[1 - ci], neg(u[1 - ci])) for y in (w[1 - cj], neg(w[1 - cj]))
                       if (x[0] - y[0], x[1] - y[1]) == u[ci]]
            sd, td = dual(p, q)
            units[i] += [('p', [(i, p), (j, q)], {(i, j): 1, (j, i): 1}, [(i, td), (j, sd)]),
                         ('p', [(i, q), (j, q)], {(i, j): 1}, [(i, neg(td)), (j, td)]),
                         ('p', [(i, p), (j, p)], {(j, i): 1}, [(i, sd), (j, neg(sd))])]
            diag[i, ci][i, j] = 1
            diag[i, 1 - ci][j, i] = -1
            diag[j, 1 - cj][i, j] = -1
            diag[j, cj][j, i] = 1
    out = []
    for i in range(n):
        row = []
        for un in units[i]:
            if un[0] == 'p' and [c for c in un[1][0][1] if c][0] < 0:
                un = ('p', [(k, neg(f)) for k, f in un[1]], un[2], [(k, neg(f)) for k, f in un[3]])
            row.append(un)
        out.append(row)
    return out


GH = 5
NGRP = H // GH
UNITS = _fast_table((0, 1, 2, 0, 1))
SUMS = [un[2] for row in UNITS for un in row if un[0] == 'p' and len(un[2]) > 1]
NSUM = len(SUMS)


def _signed_sum(terms):
    terms = sorted(terms, key=lambda cv: -cv[0])
    acc = terms[0][1]
    for c, v in terms[1:]:
        acc = acc + v if c > 0 else acc - v
    return acc


def _lhs_operands(top, bot):
    forms = {}

    def form(i, f):
        sign = 1 if [c for c in f if c][0] > 0 else -1
        key = (i, (sign * f[0], sign * f[1]))
        if key not in forms:
            forms[key] = {(1, 0): lambda: top[i], (0, 1): lambda: bot[i],
                          (1, -1): lambda: top[i] - bot[i]}[key[1]]()
        return sign, forms[key]

    return lambda un: _signed_sum([form(i, f) for i, f in un[1]]).astype(BF16)


class _Acc:
    def __init__(self):
        self.v = {}

    def add(self, key, c, p):
        if key not in self.v:
            self.v[key] = (c, p)
        else:
            sign, v = self.v[key]
            self.v[key] = (sign, v + p if sign == c else v - p)

    def pop(self, key):
        sign, v = self.v.pop(key)
        return v if sign > 0 else -v


def _kernel(x_hbm, mem0_hbm, wq_hbm, wk_hbm, wv_hbm, wo_hbm, wint_hbm, wsp_hbm,
            bsp_hbm, wout_hbm, out_hbm,
            x_v, xn_v, xa_v, xb_v, mem0_v, bsp_v, bsp32_v, zero_v, wint_v, wins_v, wsp_v, wout_v, woutc_v,
            stage_v, wqkv_v, wc_v, wo_v, woc_v, zg_v, st_v, z1t_v, za_v, ta_v, tb_v, u_v, q_v, k_v, v_v, o_v, cap_v, out_v,
            sem_x, sem_w, sem_st, sem_wo, sem_out):
    NRB = FH // RB
    NG = RB // 8
    NB2 = NTILE // T2
    PPB = 48 // NB2

    x_parts = [(0, XCH), (XCH, XCH), (2 * XCH, XCH), (3 * XCH, S - 3 * XCH)]
    x_cps = [pltpu.make_async_copy(x_hbm.at[pl.ds(o, n), :], x_v.at[pl.ds(o, n), :], sem_x.at[k])
             for k, (o, n) in enumerate(x_parts)]
    wint_u = wint_hbm.bitcast(U32)
    blk_row = lambda k: (FH + k * RB) if k < NRB else (k - NRB) * RB
    wint_cps, k0 = [], 0
    for k, nb in enumerate(WIN_PIECES):
        o, n = blk_row(k0) // 2, nb * RB // 2
        wint_cps.append(pltpu.make_async_copy(wint_u.at[pl.ds(o, n), :], wint_v.at[pl.ds(o, n), :],
                                              sem_w.at[k]))
        k0 += nb
    wsp_u = wsp_hbm.bitcast(U32)
    wsp_cp = pltpu.make_async_copy(wsp_u.at[pl.ds(0, WSP_HEAD), :], wsp_v.at[pl.ds(0, WSP_HEAD), :],
                                   sem_w.at[3])
    wsp_cp2 = pltpu.make_async_copy(wsp_u.at[pl.ds(WSP_HEAD, S // 2 - WSP_HEAD), :],
                                    wsp_v.at[pl.ds(WSP_HEAD, S // 2 - WSP_HEAD), :], sem_w.at[7])
    wout_cp = pltpu.make_async_copy(wout_hbm.bitcast(U32), wout_v, sem_w.at[4])
    WOQ = H * DH // 2 // NB2

    def wo_copy(i):
        r0 = _mult(i * WOQ, WOQ)
        return pltpu.make_async_copy(wo_hbm.bitcast(U32).at[pl.ds(r0, WOQ), :],
                                     wo_v.at[pl.ds(r0, WOQ), :], sem_wo.at[i])

    mem0_cp = pltpu.make_async_copy(mem0_hbm, mem0_v, sem_w.at[5])
    bsp_cp = pltpu.make_async_copy(bsp_hbm, bsp_v, sem_w.at[6])
    w_hbms = (wq_hbm, wk_hbm, wv_hbm)

    def stage_copy(m, j):
        p = m * 16 + j
        return pltpu.make_async_copy(w_hbms[m].bitcast(U32).at[:, j, :],
                                     stage_v.at[p, pl.ds(0, DM), :], sem_st.at[p // PPB])

    x_cps[0].start()
    x_cps[1].start()
    for cp in wint_cps:
        cp.start()
    x_cps[2].start()
    x_cps[3].start()
    bsp_cp.start()
    wsp_cp.start()
    wout_cp.start()
    for p in range(48):
        stage_copy(p // 16, p % 16).start()
        if (p + 1) % PPB == 0:
            wo_copy(p // PPB).start()
        if p + 1 == 2 * PPB:
            wsp_cp2.start()
    mem0_cp.start()

    zero_v[...] = jnp.zeros((8, 128), U32)

    pending = []

    def dep_of(v):
        return pltpu.bitcast(v[0:8, 0:128], U32) & zero_v[...]

    def up(u):
        return _as_bf16(u).astype(F32)

    def ln_rows(r0, n, dep=None):
        xr = x_v[pl.ds(r0, n), :].astype(F32)
        if dep is not None:
            d = jnp.concatenate([dep] * (n // 8), axis=0)
            xr = pltpu.bitcast(pltpu.bitcast(xr, U32) | jnp.concatenate([d] * (DM // 128), axis=1), F32)
        xn = _layernorm(xr)
        xn_v[pl.ds(_mult(r0 // 2, n // 2), n // 2), :] = _as_u32(xn.astype(BF16))
        return xn

    def ln_pair(base, k, dst, dep):
        xe = ln_rows(_mult(base + 16 * k, 16), 16, dep)
        xo = ln_rows(_mult(base + 128 + 16 * k, 16), 16, dep)
        b11, b21, b12, b22 = xe[:, 0:256], xe[:, 256:512], xo[:, 0:256], xo[:, 256:512]
        ops = jnp.concatenate([b11 + b22, b11, b12 - b22, b21 - b11, b22,
                               b11 + b12, xo[:, 512:], b21 + b22, xe[:, 512:]], axis=1)
        dst[8 * k:8 * k + 8, :] = _as_u32(ops.astype(BF16))
        pending.append([LN_DEADLINE, dst[8 * k:8 * k + 8, 0:128] & zero_v[...]])

    def win_sums(hz, k, dep):
        d = jnp.concatenate([dep] * 4, axis=1)
        r0 = hz * (FH // 2) + 8 * k
        top, bot = up(wint_v[r0:r0 + 8, 0:512] | d), up(wint_v[r0 + FH // 4:r0 + FH // 4 + 8, 0:512] | d)
        a11, a12, a21, a22 = top[:, 0:256], top[:, 256:512], bot[:, 0:256], bot[:, 256:512]
        ops = jnp.concatenate([a11 + a22, a21 + a22, a11 + a12, a21 - a11, a12 - a22], axis=1)
        wins_v[hz * (FH // 4) + 8 * k:hz * (FH // 4) + 8 * k + 8, :] = _as_u32(ops.astype(BF16))

    def nt_dot(w, xt):
        due = None
        for e in pending:
            e[0] -= 1
            if e[0] == 0:
                due = e[1] if due is None else due | e[1]
        pending[:] = [e for e in pending if e[0] > 0]
        if due is not None:
            top = w[0:8, 0:128] | due
            if w.shape[1] > 128:
                top = jnp.concatenate([top, w[0:8, 128:]], axis=1)
            w = jnp.concatenate([top, w[8:]], axis=0)
        return jax.lax.dot_general(_as_bf16(w), _as_bf16(xt), NT, preferred_element_type=F32)

    def win_block(nt, f0):
        return nt_dot(wint_v[f0 // 2:(f0 + RB) // 2, :], xn_v[nt * 64:(nt + 1) * 64, :])

    def win_group(src, hz, rb, emit, side):
        rt = (hz * FH + rb * RB) // 2
        rows = lambda r: slice(r, r + RB // 2)
        top, bot, sm = rows(rt), rows(rt + FH // 4), rows(hz * (FH // 4) + rb * RB // 2)
        ss = lambda q: wins_v[sm, q * 256:(q + 1) * 256]
        tt = lambda q: src[:, q * 256:(q + 1) * 256]
        rest = lambda r: wint_v[r, 512:640]

        def prod(w, xt):
            p = nt_dot(w, xt)
            side(p)
            return p

        m2 = prod(ss(1), tt(1))
        m4 = prod(wint_v[bot, 256:512], tt(3))
        emit(0, rb + NRB // 2, m2 + m4 + prod(rest(bot), src[:, 1920:2048]))
        m3 = prod(wint_v[top, 0:256], tt(2))
        m5 = prod(ss(2), tt(4))
        emit(1, rb, m3 + m5 + prod(rest(top), src[:, 1536:1664]))
        c11, c22 = m4 - m5, m3 - m2
        m1 = prod(ss(0), tt(0))
        emit(0, rb, c11 + m1 + prod(jnp.concatenate([ss(4), rest(top)], axis=1), src[:, 1664:2048]))
        emit(1, rb + NRB // 2,
             c22 + m1 + prod(jnp.concatenate([ss(3), rest(bot)], axis=1), src[:, 1280:1664]))

    def z2_emit(nt, rb, z):
        g = _gelu2(z)
        zg_v[nt, rb * RB:(rb + 1) * RB, :] = g
        g3 = g.reshape(NG, 8, 128)
        bm = jnp.sum(g3, axis=0) * (1.0 / NG)
        c = g3 - bm
        st_v[nt, rb * 8:(rb + 1) * 8, :] = bm
        st_v[nt, (NRB + rb) * 8:(NRB + rb + 1) * 8, :] = jnp.sum(c * c, axis=0)

    def z2_stats(nt):
        bm = st_v[nt, 0:NRB * 8, :]
        m = jnp.sum(bm, axis=0, keepdims=True) * (1.0 / (NRB * 8))
        dm = bm - m
        m2 = jnp.sum(st_v[nt, NRB * 8:2 * NRB * 8, :] + dm * dm * NG, axis=0, keepdims=True)
        r = jax.lax.rsqrt(m2 * (1.0 / FH) + 4.0 * EPS)
        return jnp.broadcast_to(m, (8, 128)), jnp.broadcast_to(r, (8, 128))

    def z2_norm(ne, tp, k, st, dep):
        (me, re), (mo, ro) = st
        me = pltpu.bitcast(pltpu.bitcast(me, U32) | dep, F32)
        mo = pltpu.bitcast(pltpu.bitcast(mo, U32) | dep, F32)
        nrm = lambda nt, f0, m, r: ((zg_v[nt, f0:f0 + 16, :].reshape(2, 8, 128) - m) * r).reshape(16, 128)
        a11, a21 = nrm(ne, 16 * k, me, re), nrm(ne, FH // 2 + 16 * k, me, re)
        a12, a22 = nrm(ne + 1, 16 * k, mo, ro), nrm(ne + 1, FH // 2 + 16 * k, mo, ro)
        ops = jnp.concatenate([a11 + a22, a21 + a22, a11, a22, a11 + a12, a21 - a11, a12 - a22], axis=1)
        za_v.at[tp][8 * k:8 * k + 8, :] = _as_u32(ops.astype(BF16))

    def z1_emit(tile, rb, z):
        z1t_v[rb * RB // 2:(rb + 1) * RB // 2, _lanes(tile)] = _as_u32(_gelu2(z).astype(BF16))

    def spread(tasks, slots):
        state = [0]

        def side(p):
            n = state[0]
            mine = tasks[n * len(tasks) // slots:(n + 1) * len(tasks) // slots]
            for q, fn in enumerate(mine):
                fn(dep_of(p[8 * ((q * NG) // len(mine)):]))
            state[0] += 1

        return side

    def mix(*kinds):
        order = sorted(((q + 0.5) / len(kd), kn, q) for kn, kd in enumerate(kinds) for q in range(len(kd)))
        return [kinds[kn][q] for _, kn, q in order]

    part = functools.partial
    NSLAB = FH // 32

    x_cps[0].wait()
    ln_rows(0, XCH)
    x_cps[1].wait()
    ln_rows(XCH, XCH)
    wint_cps[0].wait()
    for nt in range(T1):
        for rb in range(WIN_PIECES[0]):
            z2_emit(nt, rb, win_block(nt, FH + rb * RB))
    wint_cps[1].wait()
    side = spread([part(win_sums, 1, k) for k in range(NSLAB)], T1 * (NRB - WIN_PIECES[0]) - 1)
    for nt in range(T1):
        for rb in range(WIN_PIECES[0], NRB):
            z = win_block(nt, FH + rb * RB)
            z2_emit(nt, rb, z)
            side(z)
    wint_cps[2].wait()
    x_cps[2].wait()
    norms = []
    for ne in range(0, T1, 2):
        st = (z2_stats(ne), z2_stats(ne + 1))
        norms += [part(z2_norm, ne, ne // 2, k, st) for k in range(NSLAB)]
    side = spread(mix(norms, [part(win_sums, 0, k) for k in range(NSLAB)],
                      [part(ln_pair, T1 * 128, k, xa_v) for k in range(8)]), T1 * NRB - 1)
    for nt in range(T1):
        for rb in range(NRB):
            z = win_block(nt, rb * RB)
            z1_emit(nt, rb, z)
            side(z)
    x_cps[3].wait()
    pending.clear()

    def b1_body(i, carry):
        for ne in range(0, T1, 2):
            tile = i * T1 + ne
            src, dst = (xa_v, xb_v) if ne == 0 else (xb_v, xa_v)
            base = jnp.minimum(tile + 2, NTILE - 2) * 128
            lns = [part(ln_pair, base, k, dst) for k in range(8)]
            side = spread(lns[:LN_FIRST], 9 * NRB // 2)
            for rb in range(NRB // 2):
                win_group(src, 1, rb, lambda o, r, z: z2_emit(ne + o, r, z), side)
            st = (z2_stats(ne), z2_stats(ne + 1))
            norms = [part(z2_norm, ne, tile // 2, k, st) for k in range(NSLAB)]
            side = spread(mix(norms, lns[LN_FIRST:]) if LN_FIRST < 8 else norms, 9 * NRB // 2 - NORM_TAIL)
            for rb in range(NRB // 2):
                win_group(src, 0, rb, lambda o, r, z: z1_emit(tile + o, r, z), side)
        pending.clear()
        return carry

    jax.lax.fori_loop(1, NTILE // T1, b1_body, 0)

    wsp_cp.wait()
    wout_cp.wait()
    bsp_cp.wait()
    bsp32_v[...] = 0.5 * bsp_v[...].astype(F32)

    def split_block(p, bi, dep):
        a = stage_v[p, pl.ds(128 * bi, 64, stride=2), :] | dep
        b = stage_v[p, pl.ds(128 * bi + 1, 64, stride=2), :] | dep
        wqkv_v[2 * p, 64 * bi:64 * bi + 64, :] = (a & jnp.uint32(0xFFFF)) | (b << 16)
        wqkv_v[2 * p + 1, 64 * bi:64 * bi + 64, :] = (a >> 16) | (b & jnp.uint32(0xFFFF0000))

    def weight_sums(block, dst, rows, idx, dep):
        cache = {}

        def blk(ij):
            if ij not in cache:
                w = block(*ij)
                cache[ij] = up(w | dep[0:w.shape[0]])
            return cache[ij]

        mine = [un[2] for un in UNITS[idx] if un[0] == 'p' and len(un[2]) > 1]
        c0 = SUMS.index(mine[0])
        sums = jnp.concatenate([_signed_sum([(c, blk(ij)) for ij, c in r.items()]) for r in mine], axis=1)
        dst[rows, c0 * 128:(c0 + len(mine)) * 128] = _as_u32(sums.astype(BF16))

    fblocks = [(f0, min(128, FH - f0)) for f0 in range(0, FH, 128)]

    def u_transpose(tile):
        for f0, fn in fblocks:
            ut = _as_bf16(z1t_v[f0 // 2:(f0 + fn) // 2, _lanes(tile)]).astype(F32)
            u_v[:, f0:f0 + fn] = _as_u32(ut.T.astype(BF16))

    NK = NTILE // 2

    def t_piece(tp, dst, k, dep=None):
        h0 = _mult(tp * 128, 128)
        we = wsp_v[pl.ds(h0, 64), k * 256:(k + 1) * 256]
        wo = wsp_v[pl.ds(h0 + 64, 64), k * 256:(k + 1) * 256]
        if dep is not None:
            d = jnp.concatenate([dep, dep], axis=1)
            we, wo = we | d, wo | d
        we, wo = up(we), up(wo)
        b11, b21, b12, b22 = we[:, 0:128], we[:, 128:256], wo[:, 0:128], wo[:, 128:256]
        ops = jnp.concatenate([b11 + b22, b12 - b22, b21 - b11, b11 + b12, b21 + b22], axis=1)
        dst[:, k * 640:(k + 1) * 640] = _as_u32(ops.astype(BF16))

    for k in range(NK):
        t_piece(0, ta_v, k)

    def b2_body(i, carry):
        group = stage_v.at[pl.ds(i * PPB, PPB), pl.ds(0, DM), :]
        pltpu.make_async_copy(group, group, sem_st.at[i]).wait()
        wo_copy(i).wait()

        @pl.when(i == 2)
        def _():
            wsp_cp2.wait()

        u_transpose(0)
        for lp in range(2):
            tp = i * 2 + lp
            cur, nxt = (ta_v, tb_v) if lp == 0 else (tb_v, ta_v)
            tpn = jnp.minimum(tp + 1, NK - 1)
            he = pl.multiple_of(tp * 128, 128)
            raw = lambda odd_t, odd_s: lambda k: wsp_v[
                pl.ds(he + odd_t * 64, 64), (2 * k + odd_s) * 128:(2 * k + odd_s + 1) * 128]
            tj = lambda j: lambda k: cur[:, k * 640 + j * 128:k * 640 + (j + 1) * 128]
            rhs = [tj(0), raw(0, 0), tj(1), tj(2), raw(1, 1), tj(3), tj(4)]

            part = functools.partial
            full = slice(0, 64)
            kinds = [[(28, part(t_piece, tpn, nxt, k)) for k in range(NK)], []]
            if lp == 0:
                kinds[1] = [(9, part(split_block, i * PPB + pp, bi)) for pp in range(PPB) for bi in range(GH)]
            else:
                for sl in range(5):
                    gid = jnp.minimum((9 * i) // 2 + sl, (9 * i + 9) // 2 - 1)
                    f0h = (gid // NGRP) * H + (gid % NGRP) * GH
                    block = lambda bi, bj, f0h=f0h: wqkv_v[f0h + bj, 64 * bi:64 * bi + 64, :]
                    kinds[1] += [(30, part(weight_sums, block, wc_v.at[gid], full, idx)) for idx in range(GH)]
            if lp == 0:
                kinds.append([])
                for sl in range(2):
                    gid = jnp.minimum((3 * i) // 2 + sl, (3 * i + 3) // 2 - 1)
                    block = lambda bi, bj, gid=gid: wo_v[
                        pl.ds(pl.multiple_of((gid * GH + bi) * 64, 64), 64), bj * 128:(bj + 1) * 128]
                    kinds[-1] += [(30, part(weight_sums, block, woc_v.at[gid], full, idx)) for idx in range(GH)]
            r8 = pl.multiple_of(8 * (2 * i + lp), 8)
            block = lambda bi, bj, r8=r8: wout_v[pl.ds(64 * bi + r8, 8), bj * 128:(bj + 1) * 128]
            kinds.append([(4, part(weight_sums, block, woutc_v, pl.ds(r8, 8), idx)) for idx in range(GH)])
            order = sorted(((q + 0.5) / len(kd), kn, q) for kn, kd in enumerate(kinds) for q in range(len(kd)))
            tasks = [kinds[kn][q] for _, kn, q in order]
            budget = sum(c for c, _ in tasks) / (2 * 7 * len(SBLK) - SIDE_TAIL)
            state = [0.0]

            def side(p):
                state[0] += budget
                phase = 0
                while tasks and state[0] > 0:
                    c, fn = tasks.pop(0)
                    rows = p[0:128].reshape(8, 16, 128)[:, 8 * phase:8 * phase + 8, :]
                    fn((pltpu.bitcast(rows, U32) & zero_v[...]).reshape(64, 128))
                    state[0] -= c
                    phase = 1 - phase

            def prod(j, f0, fn):
                p = None
                for ks in (range(NK // 2), range(NK // 2, NK)):
                    lhs = jnp.concatenate(
                        [za_v[k, f0 // 2:(f0 + fn) // 2, j * 128:(j + 1) * 128] for k in ks], axis=1)
                    r = jnp.concatenate([rhs[j](k) for k in ks], axis=1)
                    q = jax.lax.dot_general(_as_bf16(lhs), _as_bf16(r), NT, preferred_element_type=F32)
                    side(q)
                    p = q if p is None else p + q
                return p

            def finish(c, f0, fn, odd_t):
                tile = tp * 2 + odd_t
                z1 = _as_bf16(z1t_v[f0 // 2:(f0 + fn) // 2, _lanes(tile)]).astype(F32)
                brow = bsp32_v[pl.ds(tile, 1), :]
                z1t_v[f0 // 2:(f0 + fn) // 2, _lanes(tile)] = _as_u32((z1 * (0.5 * c + brow)).astype(BF16))

            f0 = 0
            for fn in SBLK:
                m2, m4 = prod(1, f0, fn), prod(3, f0, fn)
                finish(m2 + m4, FH // 2 + f0, fn, 0)
                m5, m3 = prod(4, f0, fn), prod(2, f0, fn)
                finish(m3 + m5, f0, fn, 1)
                c11, c22 = m4 - m5, m3 - m2
                m1 = prod(0, f0, fn)
                finish(c11 + m1 + prod(6, f0, fn), f0, fn, 0)
                finish(c22 + m1 + prod(5, f0, fn), FH // 2 + f0, fn, 1)
                f0 += fn
            assert not tasks
        return carry

    jax.lax.fori_loop(0, NB2, b2_body, 0)
    mem0_cp.wait()

    masks = _masks()
    for n, (keep, fill) in enumerate(masks):
        cap_v[n, 0:keep.shape[0], 0:keep.shape[1]] = jnp.where(keep, 0.0, fill)
    dot = lambda l, r: jnp.dot(l, r, preferred_element_type=F32)

    def fast_units(lhs_of, both, raw, sums, acc, done):
        items = []
        for i, row in enumerate(UNITS):
            for q, un in enumerate(row):
                def fn(un=un, last=(q == len(row) - 1), i=i):
                    if un[0] == 'b':
                        p = dot(both(un[1]), raw(un[1], un[2]))
                        hr = p.shape[0] // 2
                        acc.add((0, un[2]), 1, p[0:hr])
                        acc.add((1, un[2]), 1, p[hr:])
                    else:
                        r = un[2]
                        p = dot(lhs_of(un), raw(*list(r)[0]) if len(r) == 1 else sums(SUMS.index(r)))
                        for k, f in un[3]:
                            for half in range(2):
                                if f[half]:
                                    acc.add((half, k), f[half], p)
                    if last:
                        done(i)
                items.append((16 if un[0] == 'b' else 8, fn))
        return items

    def step(n, h):
        odd = n % 2 == 1
        hb = h.astype(BF16)
        qb = 24 * n
        kb = 40 * (n // 2) + (0 if odd else 16)
        nq, nk = (24, 40) if odd else (16, 24)
        clock = [0]
        d_s, d_o, gap, lag_v = PIPE[n]
        ready, s_at, o_at, ps = {}, {}, {}, {}

        def put(buf, r0, t, v):
            buf[r0:r0 + v.shape[0] // 2, _lanes(t)] = _as_u32(v.astype(BF16))

        def put64(m, t, top, bot):
            buf = (q_v, k_v, v_v)[m]
            if m == 0:
                put(buf, 0, t, top)
                put(buf, 24 + 16, t, bot[0:16])
                put(buf, 72 + 16, t, bot[16:32])
            else:
                put(buf, 16, t, top)
                put(buf, 32, t, bot[0:16])
                put(buf, 40 + 32, t, bot[16:32])
            ready[m, t] = clock[0]

        def plain(m, t):
            r = dot(hb, _as_bf16(wqkv_v[m * H + t]))
            if n == 0:
                put64(m, t, r[0:32], r[32:64])
            else:
                put((q_v, k_v, v_v)[m], qb if m == 0 else kb, t, r)
                ready[m, t] = clock[0]

        work = []
        if n == 0:
            cols = lambda i: slice(i * 128, (i + 1) * 128)
            make = _lhs_operands([h[0:32, cols(i)] for i in range(GH)], [h[32:64, cols(i)] for i in range(GH)])
            ops = {id(un): make(un) for row in UNITS for un in row if un[0] == 'p'}
            for g in range(NGRP):
                for m in ORDER0:
                    if g == NGRP - 1 and m == 2:
                        work += [(80, functools.partial(plain, mm, t))
                                 for t in range(NGRP * GH, H) for mm in (1, 0)]
                    acc = _Acc()
                    work += fast_units(
                        lambda un: ops[id(un)], lambda i: hb[:, cols(i)],
                        lambda i, j, m=m, g=g: _as_bf16(wqkv_v[m * H + g * GH + j, 64 * i:64 * i + 64, :]),
                        lambda q, m=m, g=g: _as_bf16(wc_v[m * NGRP + g, :, q * 128:(q + 1) * 128]),
                        acc, lambda j, m=m, g=g, acc=acc: put64(m, g * GH + j, acc.pop((0, j)), acc.pop((1, j))))
            work += [(80, functools.partial(plain, 2, t)) for t in range(NGRP * GH, H)]
        else:
            for t in range(H + lag_v):
                for m, tt in ((1, t), (2, t - lag_v), (0, t)):
                    if 0 <= tt < H:
                        work.append((40, functools.partial(plain, m, tt)))
        work = [(c, fn, -1) for c, fn in work]

        res = []
        if n == 3:
            acc = _Acc()
            for g in range(NGRP):
                hc = lambda i, g=g: slice((g * GH + i) * DH, (g * GH + i + 1) * DH)
                box = []

                def lhs_of(un, box=box, hc=hc):
                    if not box:
                        box.append(_lhs_operands([up(o_v[0:16, hc(i)]) for i in range(GH)],
                                                 [up(o_v[16:32, hc(i)]) for i in range(GH)]))
                    return box[0](un)

                items = fast_units(
                    lhs_of, lambda i, hc=hc: _as_bf16(o_v[:, hc(i)]),
                    lambda i, j, g=g: _as_bf16(wo_v[(g * GH + i) * 64:(g * GH + i + 1) * 64, j * 128:(j + 1) * 128]),
                    lambda q, g=g: _as_bf16(woc_v[g, :, q * 128:(q + 1) * 128]), acc, lambda j: None)
                work += [(c, fn, g * GH + GH - 1) for c, fn in items]

            def tail():
                c0 = NGRP * GH * DH
                part = dot(_as_bf16(o_v[:, c0:]), _as_bf16(wo_v[c0 // 2:, :]))
                res.append(part + jnp.concatenate(
                    [jnp.concatenate([acc.pop((hf, j)) for j in range(GH)], axis=1) for hf in range(2)], axis=0))

            work.append((160, tail, H - 1))
        else:
            def wgroup(g):
                c0, c1 = g * WG * DH, (g + 1) * WG * DH
                part = dot(_as_bf16(o_v[0:16, c0:c1]), _as_bf16(wo_v[c0 // 2:c1 // 2, :]))
                res[:] = [part + res[0]] if res else [part]

            work += [(40 * WG, functools.partial(wgroup, g), (g + 1) * WG - 1) for g in range(H // WG)]

        def scores(t):
            sc = jax.lax.dot_general(_as_bf16(q_v[qb:qb + nq, _lanes(t)]),
                                     _as_bf16(k_v[kb:kb + nk, _lanes(t)]), NT,
                                     preferred_element_type=F32) * SCALE
            cap = cap_v[n, 0:sc.shape[0], 0:sc.shape[1]]
            sc = jnp.where(cap == 0.0, sc, cap)
            e = jnp.exp(sc - jnp.max(sc, axis=-1, keepdims=True))
            l = jnp.sum(e, axis=-1, keepdims=True)
            inv = pl.reciprocal(l, approx=True)
            inv = inv * (2.0 - l * inv)
            ps[t] = (e * inv).astype(BF16)
            s_at[t] = clock[0]
            clock[0] += nq // 2

        def values(t):
            o = dot(ps.pop(t), _as_bf16(v_v[kb:kb + nk, _lanes(t)]))
            if n == 1:
                put(o_v, 0, t, o[0:32])
                put(o_v, 24, t, o[32:48])
            else:
                put(o_v, 0, t, o)
            o_at[t] = clock[0]
            clock[0] += nq // 2

        def drain(upto):
            while True:
                to, ts = len(o_at), len(s_at)
                if to < ts and (2, to) in ready and (
                        to <= upto or clock[0] >= max(s_at[to] + d_o, ready[2, to] + d_s)):
                    values(to)
                elif ts < H and (0, ts) in ready and (1, ts) in ready and (
                        ts <= upto or clock[0] >= max(ready[0, ts] + d_s, ready[1, ts] + d_s,
                                                      s_at.get(ts - 1, -gap) + gap)):
                    scores(ts)
                else:
                    return

        for c, fn, need in work:
            drain(need)
            clock[0] += c
            fn()
        return res[0]

    def gate_work():
        acc = _Acc()
        cols = lambda i: slice(i * 128, (i + 1) * 128)
        box = []

        def lhs_of(un):
            if not box:
                box.append(_lhs_operands([up(u_v[0:32, cols(i)]) for i in range(GH)],
                                         [up(u_v[32:64, cols(i)]) for i in range(GH)]))
            return box[0](un)

        items = [(2 * c, fn) for c, fn in fast_units(
            lhs_of, lambda i: _as_bf16(u_v[:, cols(i)]),
            lambda i, j: _as_bf16(wout_v[64 * i:64 * i + 64, cols(j)]),
            lambda q: _as_bf16(woutc_v[:, cols(q)]), acc, lambda j: None)]

        def rest(j):
            p = dot(_as_bf16(u_v[:, DM:FH]), _as_bf16(wout_v[DM // 2:FH // 2, cols(j)]))
            acc.add((0, j), 1, p[0:64])
            acc.add((1, j), 1, p[64:128])

        items = [(64, functools.partial(rest, j)) for j in range(GH)] + items

        def chunk(budget):
            box.clear()
            while items and budget > 0:
                c, fn = items.pop(0)
                fn()
                budget -= c

        def result():
            hb = 0.5 * jnp.concatenate(
                [jnp.concatenate([acc.pop((hf, j)) for j in range(GH)], axis=1) for hf in range(2)], axis=0)
            return hb + hb * jnp.tanh(hb)

        return chunk, result

    def tile_body(j, mem):
        r0 = pl.multiple_of(j * 128, 128)
        xs = _as_bf16(xn_v[pl.ds(pl.multiple_of(j * 64, 64), 64), :]).astype(F32)
        chunk, gate_result = gate_work()
        chunk(FILL[0])
        a0 = step(0, jnp.concatenate([mem, xs[0:40], xs[64:72], xs[96:104]], axis=0))
        chunk(FILL[1])
        a1 = step(1, jnp.concatenate([a0[0:MEM], xs[40:64]], axis=0))
        chunk(FILL[2])
        a2 = step(2, jnp.concatenate([a1[0:MEM], xs[72:96]], axis=0))
        chunk(10 ** 6)
        gate = gate_result()
        u_transpose(jnp.minimum(j + 1, NTILE - 1))
        a3 = step(3, jnp.concatenate([a2[0:MEM], xs[104:128]], axis=0))
        s_rows = jnp.concatenate([a0[8:32], a3[48:64], a1[8:32], a3[32:40], a2[8:32], a3[40:48], a3[8:32]],
                                 axis=0)
        res = x_v[pl.ds(r0, 128), :].astype(F32) + s_rows * gate
        out_v[pl.ds(r0, 128), :] = res.astype(BF16)
        pltpu.make_async_copy(out_v.at[pl.ds(r0, 128), :],
                              out_hbm.at[pl.ds(r0, 128), :], sem_out).start()
        return a3[0:MEM]

    jax.lax.fori_loop(0, NTILE, tile_body, mem0_v[...].astype(F32))
    pltpu.make_async_copy(out_v, out_hbm, sem_out).wait()


@jax.jit
def pallas_recurrent_scan__memory_aug_recurrent_mem_tr__mixer_gmlp__prompt_kernel(
    A_x: jax.Array,
    A_mem0: jax.Array,
    A_Wq: jax.Array,
    A_Wk: jax.Array,
    A_Wv: jax.Array,
    A_Wo: jax.Array,
    A_seg_len: jax.Array,
    B_x: jax.Array,
    B_w_in: jax.Array,
    B_w_sp: jax.Array,
    B_b_sp: jax.Array,
    B_w_out: jax.Array,
):
    del A_seg_len, B_x
    hbm = pl.BlockSpec(memory_space=pl.ANY)
    out = pl.pallas_call(
        _kernel,
        out_shape=jax.ShapeDtypeStruct((S, DM), BF16),
        in_specs=[hbm] * 10,
        out_specs=hbm,
        scratch_shapes=[
            pltpu.VMEM((S, DM), BF16),
            pltpu.VMEM((S // 2, DM), U32),
            pltpu.VMEM((64, 2048), U32),
            pltpu.VMEM((64, 2048), U32),
            pltpu.VMEM((MEM, DM), BF16),
            pltpu.VMEM((16, 128), BF16),
            pltpu.VMEM((16, 128), F32),
            pltpu.VMEM((8, 128), U32),
            pltpu.VMEM((FH, DM), U32),
            pltpu.VMEM((FH // 2, 1280), U32),
            pltpu.VMEM((S // 2, S), U32),
            pltpu.VMEM((FH // 2, DM), U32),
            pltpu.VMEM((64, NSUM * 128), U32),
            pltpu.VMEM((48, DM + 8, DH), U32),
            pltpu.VMEM((3 * H, DM // 2, DH), U32),
            pltpu.VMEM((3 * NGRP, 64, NSUM * 128), U32),
            pltpu.VMEM((H * DH // 2, DM), U32),
            pltpu.VMEM((NGRP, 64, NSUM * 128), U32),
            pltpu.VMEM((T1, FH, 128), F32),
            pltpu.VMEM((T1, 2 * (FH // RB) * 8, 128), F32),
            pltpu.VMEM((FH // 2, S), U32),
            pltpu.VMEM((NTILE // 2, FH // 4, 7 * 128), U32),
            pltpu.VMEM((64, 5 * S // 2), U32),
            pltpu.VMEM((64, 5 * S // 2), U32),
            pltpu.VMEM((64, FH), U32),
            pltpu.VMEM((96, H * DH), U32),
            pltpu.VMEM((80, H * DH), U32),
            pltpu.VMEM((80, H * DH), U32),
            pltpu.VMEM((32, H * DH), U32),
            pltpu.VMEM((4, 48, 80), F32),
            pltpu.VMEM((S, DM), BF16),
            pltpu.SemaphoreType.DMA((4,)),
            pltpu.SemaphoreType.DMA((8,)),
            pltpu.SemaphoreType.DMA((NTILE // T2,)),
            pltpu.SemaphoreType.DMA((NTILE // T2,)),
            pltpu.SemaphoreType.DMA,
        ],
        compiler_params=pltpu.CompilerParams(vmem_limit_bytes=112 * 1024 * 1024),
    )(
        A_x.reshape(S, DM),
        A_mem0.reshape(MEM, DM),
        A_Wq, A_Wk, A_Wv,
        A_Wo.reshape(H * DH, DM),
        B_w_in.T,
        B_w_sp,
        B_b_sp.reshape(16, 128),
        B_w_out,
    )
    return out.reshape(1, S, DM)
```

```python
import functools

import jax
import jax.numpy as jnp
import jax.experimental.pallas as pl
import jax.experimental.pallas.tpu as pltpu

F32 = jnp.float32
BF16 = jnp.bfloat16
U32 = jnp.uint32

S = 2048
DM = 640
H = 32
DH = 128
MEM = 8
SEG = 32
FH = 864
NTILE = S // 128
EPS = 1e-5
SCALE = DH ** (-0.5)
NEG = -1000000000.0

XCH = 256
T1 = 4
T2 = 4
RB = 144
WIN_PIECES = (2, 4, 6)
SBLK = (144, 144, 144)
SIDE_TAIL = 1
WSP_HEAD = 512
LN_DEADLINE = 10
LN_FIRST = 4
NORM_TAIL = 4
ORDER0 = (1, 0, 2)
PIPE = ((270, 450, 170, 0), (230, 540, 128, 2), (270, 510, 112, 4), (230, 450, 128, 1))
WG = 4
FILL = (320, 224, 224)

NT = (((1,), (1,)), ((), ()))


def _as_bf16(u):
    return pltpu.bitcast(u, BF16)


def _as_u32(b):
    return pltpu.bitcast(b, U32)


def _layernorm(v):
    m = jnp.mean(v, axis=-1, keepdims=True)
    c = v - m
    var = jnp.mean(c * c, axis=-1, keepdims=True)
    return c * jax.lax.rsqrt(var + EPS)


def _gelu2(v):
    c = 0.7978845608028654
    return v + v * jnp.tanh(v * (c + (c * 0.044715) * (v * v)))


def _mult(v, m):
    return v if isinstance(v, int) else pl.multiple_of(v, m)


def _lanes(tile):
    return pl.ds(_mult(tile * 128, 128), 128)


def _mask(qgroups, kgroups):
    shape = (8 * len(qgroups), 8 * len(kgroups))

    def table(groups, axis):
        idx = jax.lax.broadcasted_iota(jnp.int32, shape, axis)
        seg = jnp.full(shape, groups[-1][0], jnp.int32)
        pos = idx + (groups[-1][1] - 8 * (len(groups) - 1))
        for g in range(len(groups) - 2, -1, -1):
            inside = idx < 8 * (g + 1)
            seg = jnp.where(inside, groups[g][0], seg)
            pos = jnp.where(inside, idx + (groups[g][1] - 8 * g), pos)
        return seg, pos

    qseg, qpos = table(qgroups, 0)
    kseg, kpos = table(kgroups, 1)
    same = qseg == kseg
    keep = same & ((qpos < MEM) | (qpos >= kpos))
    return keep, jnp.where(same, NEG, -jnp.inf).astype(F32)


def _masks():
    own = lambda sg: [(sg, 0), (sg, 16), (sg, 24), (sg, 32)]
    k0 = [(0, 0), (0, 8), (0, 16), (0, 24), (0, 32), (1, 8)]
    k2 = own(2) + [(2, 8), (3, 8)]
    return [
        _mask(k0[:4], k0),
        _mask(own(1) + k0[4:], own(1) + k0),
        _mask(own(2), k2),
        _mask(own(3) + k2[4:], own(3) + k2),
    ]


def _fast_table(types):
    lines = {0: ((1, 0), (1, -1)), 1: ((0, 1), (1, -1)), 2: ((1, 0), (0, 1))}
    neg = lambda f: (-f[0], -f[1])

    def dual(u, v):
        det = u[0] * v[1] - u[1] * v[0]
        return (v[1] * det, -v[0] * det), (-u[1] * det, u[0] * det)

    n = len(types)
    diag = {(i, k): {(i, i): 1} for i in range(n) for k in range(2)}
    units = [[] for _ in range(n)]
    for i in range(n):
        u = lines[types[i]]
        units[i] += [('p', [(i, u[k])], diag[i, k], [(i, dual(*u)[k])]) for k in range(2)]
        for j in range(i + 1, n):
            if types[i] == types[j]:
                units[i] += [('b', i, j), ('b', j, i)]
                continue
            w = lines[types[j]]
            (ci, cj), = [(x, y) for x in range(2) for y in range(2) if u[x] == w[y]]
            (p, q), = [(x, y) for x in (u[1 - ci], neg(u[1 - ci])) for y in (w[1 - cj], neg(w[1 - cj]))
                       if (x[0] - y[0], x[1] - y[1]) == u[ci]]
            sd, td = dual(p, q)
            units[i] += [('p', [(i, p), (j, q)], {(i, j): 1, (j, i): 1}, [(i, td), (j, sd)]),
                         ('p', [(i, q), (j, q)], {(i, j): 1}, [(i, neg(td)), (j, td)]),
                         ('p', [(i, p), (j, p)], {(j, i): 1}, [(i, sd), (j, neg(sd))])]
            diag[i, ci][i, j] = 1
            diag[i, 1 - ci][j, i] = -1
            diag[j, 1 - cj][i, j] = -1
            diag[j, cj][j, i] = 1
    out = []
    for i in range(n):
        row = []
        for un in units[i]:
            if un[0] == 'p' and [c for c in un[1][0][1] if c][0] < 0:
                un = ('p', [(k, neg(f)) for k, f in un[1]], un[2], [(k, neg(f)) for k, f in un[3]])
            row.append(un)
        out.append(row)
    return out


GH = 5
NGRP = H // GH
UNITS = _fast_table((0, 1, 2, 0, 1))
SUMS = [un[2] for row in UNITS for un in row if un[0] == 'p' and len(un[2]) > 1]
NSUM = len(SUMS)


def _signed_sum(terms):
    terms = sorted(terms, key=lambda cv: -cv[0])
    acc = terms[0][1]
    for c, v in terms[1:]:
        acc = acc + v if c > 0 else acc - v
    return acc


def _lhs_operands(top, bot):
    forms = {}

    def form(i, f):
        sign = 1 if [c for c in f if c][0] > 0 else -1
        key = (i, (sign * f[0], sign * f[1]))
        if key not in forms:
            forms[key] = {(1, 0): lambda: top[i], (0, 1): lambda: bot[i],
                          (1, -1): lambda: top[i] - bot[i]}[key[1]]()
        return sign, forms[key]

    return lambda un: _signed_sum([form(i, f) for i, f in un[1]]).astype(BF16)


class _Acc:
    def __init__(self):
        self.v = {}

    def add(self, key, c, p):
        if key not in self.v:
            self.v[key] = (c, p)
        else:
            sign, v = self.v[key]
            self.v[key] = (sign, v + p if sign == c else v - p)

    def pop(self, key):
        sign, v = self.v.pop(key)
        return v if sign > 0 else -v


def _kernel(x_hbm, mem0_hbm, wq_hbm, wk_hbm, wv_hbm, wo_hbm, wint_hbm, wsp_hbm,
            bsp_hbm, wout_hbm, out_hbm,
            x_v, xn_v, xa_v, xb_v, mem0_v, bsp_v, bsp32_v, zero_v, wint_v, wins_v, wsp_v, wout_v, woutc_v,
            stage_v, wqkv_v, wc_v, wo_v, woc_v, zg_v, st_v, z1t_v, za_v, ts_v, u_v, q_v, k_v, v_v, o_v, cap_v, out_v,
            sem_x, sem_w, sem_st, sem_wo, sem_out):
    NRB = FH // RB
    NG = RB // 8
    NB2 = NTILE // T2
    PPB = 48 // NB2

    x_parts = [(0, XCH), (XCH, XCH), (2 * XCH, XCH), (3 * XCH, S - 3 * XCH)]
    x_cps = [pltpu.make_async_copy(x_hbm.at[pl.ds(o, n), :], x_v.at[pl.ds(o, n), :], sem_x.at[k])
             for k, (o, n) in enumerate(x_parts)]
    wint_u = wint_hbm.bitcast(U32)
    blk_row = lambda k: (FH + k * RB) if k < NRB else (k - NRB) * RB
    wint_cps, k0 = [], 0
    for k, nb in enumerate(WIN_PIECES):
        o, n = blk_row(k0) // 2, nb * RB // 2
        wint_cps.append(pltpu.make_async_copy(wint_u.at[pl.ds(o, n), :], wint_v.at[pl.ds(o, n), :],
                                              sem_w.at[k]))
        k0 += nb
    wsp_u = wsp_hbm.bitcast(U32)
    wsp_cp = pltpu.make_async_copy(wsp_u.at[pl.ds(0, WSP_HEAD), :], wsp_v.at[pl.ds(0, WSP_HEAD), :],
                                   sem_w.at[3])
    wsp_cp2 = pltpu.make_async_copy(wsp_u.at[pl.ds(WSP_HEAD, S // 2 - WSP_HEAD), :],
                                    wsp_v.at[pl.ds(WSP_HEAD, S // 2 - WSP_HEAD), :], sem_w.at[7])
    wout_cp = pltpu.make_async_copy(wout_hbm.bitcast(U32), wout_v, sem_w.at[4])
    WOQ = H * DH // 2 // NB2

    def wo_copy(i):
        r0 = _mult(i * WOQ, WOQ)
        return pltpu.make_async_copy(wo_hbm.bitcast(U32).at[pl.ds(r0, WOQ), :],
                                     wo_v.at[pl.ds(r0, WOQ), :], sem_wo.at[i])

    mem0_cp = pltpu.make_async_copy(mem0_hbm, mem0_v, sem_w.at[5])
    bsp_cp = pltpu.make_async_copy(bsp_hbm, bsp_v, sem_w.at[6])
    w_hbms = (wq_hbm, wk_hbm, wv_hbm)

    def stage_copy(m, j):
        p = m * 16 + j
        return pltpu.make_async_copy(w_hbms[m].bitcast(U32).at[:, j, :],
                                     stage_v.at[p, pl.ds(0, DM), :], sem_st.at[p // PPB])

    x_cps[0].start()
    x_cps[1].start()
    for cp in wint_cps:
        cp.start()
    x_cps[2].start()
    x_cps[3].start()
    bsp_cp.start()
    wsp_cp.start()
    wout_cp.start()
    for p in range(48):
        stage_copy(p // 16, p % 16).start()
        if (p + 1) % PPB == 0:
            wo_copy(p // PPB).start()
        if p + 1 == 2 * PPB:
            wsp_cp2.start()
    mem0_cp.start()

    zero_v[...] = jnp.zeros((8, 128), U32)

    pending = []

    def dep_of(v):
        return pltpu.bitcast(v[0:8, 0:128], U32) & zero_v[...]

    def up(u):
        return _as_bf16(u).astype(F32)

    def ln_rows(r0, n, dep=None):
        xr = x_v[pl.ds(r0, n), :].astype(F32)
        if dep is not None:
            d = jnp.concatenate([dep] * (n // 8), axis=0)
            xr = pltpu.bitcast(pltpu.bitcast(xr, U32) | jnp.concatenate([d] * (DM // 128), axis=1), F32)
        xn = _layernorm(xr)
        xn_v[pl.ds(_mult(r0 // 2, n // 2), n // 2), :] = _as_u32(xn.astype(BF16))
        return xn

    def ln_pair(base, k, dst, dep):
        xe = ln_rows(_mult(base + 16 * k, 16), 16, dep)
        xo = ln_rows(_mult(base + 128 + 16 * k, 16), 16, dep)
        b11, b21, b12, b22 = xe[:, 0:256], xe[:, 256:512], xo[:, 0:256], xo[:, 256:512]
        ops = jnp.concatenate([b11 + b22, b11, b12 - b22, b21 - b11, b22,
                               b11 + b12, xo[:, 512:], b21 + b22, xe[:, 512:]], axis=1)
        dst[8 * k:8 * k + 8, :] = _as_u32(ops.astype(BF16))
        pending.append([LN_DEADLINE, dst[8 * k:8 * k + 8, 0:128] & zero_v[...]])

    def win_sums(hz, k, dep):
        d = jnp.concatenate([dep] * 4, axis=1)
        r0 = hz * (FH // 2) + 8 * k
        top, bot = up(wint_v[r0:r0 + 8, 0:512] | d), up(wint_v[r0 + FH // 4:r0 + FH // 4 + 8, 0:512] | d)
        a11, a12, a21, a22 = top[:, 0:256], top[:, 256:512], bot[:, 0:256], bot[:, 256:512]
        ops = jnp.concatenate([a11 + a22, a21 + a22, a11 + a12, a21 - a11, a12 - a22], axis=1)
        wins_v[hz * (FH // 4) + 8 * k:hz * (FH // 4) + 8 * k + 8, :] = _as_u32(ops.astype(BF16))

    def nt_dot(w, xt):
        due = None
        for e in pending:
            e[0] -= 1
            if e[0] == 0:
                due = e[1] if due is None else due | e[1]
        pending[:] = [e for e in pending if e[0] > 0]
        if due is not None:
            top = w[0:8, 0:128] | due
            if w.shape[1] > 128:
                top = jnp.concatenate([top, w[0:8, 128:]], axis=1)
            w = jnp.concatenate([top, w[8:]], axis=0)
        return jax.lax.dot_general(_as_bf16(w), _as_bf16(xt), NT, preferred_element_type=F32)

    def win_block(nt, f0):
        return nt_dot(wint_v[f0 // 2:(f0 + RB) // 2, :], xn_v[nt * 64:(nt + 1) * 64, :])

    def win_group(src, hz, rb, emit, side):
        rt = (hz * FH + rb * RB) // 2
        rows = lambda r: slice(r, r + RB // 2)
        top, bot, sm = rows(rt), rows(rt + FH // 4), rows(hz * (FH // 4) + rb * RB // 2)
        ss = lambda q: wins_v[sm, q * 256:(q + 1) * 256]
        tt = lambda q: src[:, q * 256:(q + 1) * 256]
        rest = lambda r: wint_v[r, 512:640]

        def prod(w, xt):
            p = nt_dot(w, xt)
            side(p)
            return p

        m2 = prod(ss(1), tt(1))
        m4 = prod(wint_v[bot, 256:512], tt(3))
        emit(0, rb + NRB // 2, m2 + m4 + prod(rest(bot), src[:, 1920:2048]))
        m3 = prod(wint_v[top, 0:256], tt(2))
        m5 = prod(ss(2), tt(4))
        emit(1, rb, m3 + m5 + prod(rest(top), src[:, 1536:1664]))
        c11, c22 = m4 - m5, m3 - m2
        m1 = prod(ss(0), tt(0))
        emit(0, rb, c11 + m1 + prod(jnp.concatenate([ss(4), rest(top)], axis=1), src[:, 1664:2048]))
        emit(1, rb + NRB // 2,
             c22 + m1 + prod(jnp.concatenate([ss(3), rest(bot)], axis=1), src[:, 1280:1664]))

    def z2_emit(nt, rb, z):
        g = _gelu2(z)
        zg_v[nt, rb * RB:(rb + 1) * RB, :] = g
        g3 = g.reshape(NG, 8, 128)
        bm = jnp.sum(g3, axis=0) * (1.0 / NG)
        c = g3 - bm
        st_v[nt, rb * 8:(rb + 1) * 8, :] = bm
        st_v[nt, (NRB + rb) * 8:(NRB + rb + 1) * 8, :] = jnp.sum(c * c, axis=0)

    def z2_stats(nt):
        bm = st_v[nt, 0:NRB * 8, :]
        m = jnp.sum(bm, axis=0, keepdims=True) * (1.0 / (NRB * 8))
        dm = bm - m
        m2 = jnp.sum(st_v[nt, NRB * 8:2 * NRB * 8, :] + dm * dm * NG, axis=0, keepdims=True)
        r = jax.lax.rsqrt(m2 * (1.0 / FH) + 4.0 * EPS)
        return jnp.broadcast_to(m, (8, 128)), jnp.broadcast_to(r, (8, 128))

    def z2_norm(ne, tp, k, st, dep):
        (me, re), (mo, ro) = st
        me = pltpu.bitcast(pltpu.bitcast(me, U32) | dep, F32)
        mo = pltpu.bitcast(pltpu.bitcast(mo, U32) | dep, F32)
        nrm = lambda nt, f0, m, r: ((zg_v[nt, f0:f0 + 16, :].reshape(2, 8, 128) - m) * r).reshape(16, 128)
        a11, a21 = nrm(ne, 16 * k, me, re), nrm(ne, FH // 2 + 16 * k, me, re)
        a12, a22 = nrm(ne + 1, 16 * k, mo, ro), nrm(ne + 1, FH // 2 + 16 * k, mo, ro)
        ops = jnp.concatenate([a11 + a22, a21 + a22, a11, a22, a11 + a12, a21 - a11, a12 - a22], axis=1)
        za_v.at[tp][8 * k:8 * k + 8, :] = _as_u32(ops.astype(BF16))

    def z1_emit(tile, rb, z):
        z1t_v[rb * RB // 2:(rb + 1) * RB // 2, _lanes(tile)] = _as_u32(_gelu2(z).astype(BF16))

    def spread(tasks, slots):
        state = [0]

        def side(p):
            n = state[0]
            mine = tasks[n * len(tasks) // slots:(n + 1) * len(tasks) // slots]
            for q, fn in enumerate(mine):
                fn(dep_of(p[8 * ((q * NG) // len(mine)):]))
            state[0] += 1

        return side

    def mix(*kinds):
        order = sorted(((q + 0.5) / len(kd), kn, q) for kn, kd in enumerate(kinds) for q in range(len(kd)))
        return [kinds[kn][q] for _, kn, q in order]

    part = functools.partial
    NSLAB = FH // 32

    x_cps[0].wait()
    ln_rows(0, XCH)
    x_cps[1].wait()
    ln_rows(XCH, XCH)
    wint_cps[0].wait()
    for nt in range(T1):
        for rb in range(WIN_PIECES[0]):
            z2_emit(nt, rb, win_block(nt, FH + rb * RB))
    wint_cps[1].wait()
    side = spread([part(win_sums, 1, k) for k in range(NSLAB)], T1 * (NRB - WIN_PIECES[0]) - 1)
    for nt in range(T1):
        for rb in range(WIN_PIECES[0], NRB):
            z = win_block(nt, FH + rb * RB)
            z2_emit(nt, rb, z)
            side(z)
    wint_cps[2].wait()
    x_cps[2].wait()
    norms = []
    for ne in range(0, T1, 2):
        st = (z2_stats(ne), z2_stats(ne + 1))
        norms += [part(z2_norm, ne, ne // 2, k, st) for k in range(NSLAB)]
    side = spread(mix(norms, [part(win_sums, 0, k) for k in range(NSLAB)],
                      [part(ln_pair, T1 * 128, k, xa_v) for k in range(8)]), T1 * NRB - 1)
    for nt in range(T1):
        for rb in range(NRB):
            z = win_block(nt, rb * RB)
            z1_emit(nt, rb, z)
            side(z)
    x_cps[3].wait()
    pending.clear()

    def b1_body(i, carry):
        for ne in range(0, T1, 2):
            tile = i * T1 + ne
            src, dst = (xa_v, xb_v) if ne == 0 else (xb_v, xa_v)
            base = jnp.minimum(tile + 2, NTILE - 2) * 128
            lns = [part(ln_pair, base, k, dst) for k in range(8)]
            side = spread(lns[:LN_FIRST], 9 * NRB // 2)
            for rb in range(NRB // 2):
                win_group(src, 1, rb, lambda o, r, z: z2_emit(ne + o, r, z), side)
            st = (z2_stats(ne), z2_stats(ne + 1))
            norms = [part(z2_norm, ne, tile // 2, k, st) for k in range(NSLAB)]
            side = spread(mix(norms, lns[LN_FIRST:]) if LN_FIRST < 8 else norms, 9 * NRB // 2 - NORM_TAIL)
            for rb in range(NRB // 2):
                win_group(src, 0, rb, lambda o, r, z: z1_emit(tile + o, r, z), side)
        pending.clear()
        return carry

    jax.lax.fori_loop(1, NTILE // T1, b1_body, 0)

    wsp_cp.wait()
    wout_cp.wait()
    bsp_cp.wait()
    bsp32_v[...] = 0.5 * bsp_v[...].astype(F32)

    def split_block(p, bi, dep):
        a = stage_v[p, pl.ds(128 * bi, 64, stride=2), :] | dep
        b = stage_v[p, pl.ds(128 * bi + 1, 64, stride=2), :] | dep
        wqkv_v[2 * p, 64 * bi:64 * bi + 64, :] = (a & jnp.uint32(0xFFFF)) | (b << 16)
        wqkv_v[2 * p + 1, 64 * bi:64 * bi + 64, :] = (a >> 16) | (b & jnp.uint32(0xFFFF0000))

    def weight_sums(block, dst, rows, idx, dep):
        cache = {}

        def blk(ij):
            if ij not in cache:
                w = block(*ij)
                cache[ij] = up(w | dep[0:w.shape[0]])
            return cache[ij]

        mine = [un[2] for un in UNITS[idx] if un[0] == 'p' and len(un[2]) > 1]
        c0 = SUMS.index(mine[0])
        sums = jnp.concatenate([_signed_sum([(c, blk(ij)) for ij, c in r.items()]) for r in mine], axis=1)
        dst[rows, c0 * 128:(c0 + len(mine)) * 128] = _as_u32(sums.astype(BF16))

    fblocks = [(f0, min(128, FH - f0)) for f0 in range(0, FH, 128)]

    def u_transpose(tile):
        for f0, fn in fblocks:
            ut = _as_bf16(z1t_v[f0 // 2:(f0 + fn) // 2, _lanes(tile)]).astype(F32)
            u_v[:, f0:f0 + fn] = _as_u32(ut.T.astype(BF16))

    NK = NTILE // 2

    def t_piece(tp, k, dep):
        h0 = _mult(tp * 128, 128)
        we = wsp_v[pl.ds(h0, 64), k * 256:(k + 1) * 256]
        wo = wsp_v[pl.ds(h0 + 64, 64), k * 256:(k + 1) * 256]
        d = jnp.concatenate([dep, dep], axis=1)
        we, wo = up(we | d), up(wo | d)
        b11, b21, b12, b22 = we[:, 0:128], we[:, 128:256], wo[:, 0:128], wo[:, 128:256]
        ops = jnp.concatenate([b11 + b22, b12 - b22, b21 - b11, b11 + b12, b21 + b22], axis=1)
        z0 = pl.multiple_of(jnp.minimum(tp, 0) * 64, 64)
        ts_v[pl.ds(z0, 64), k * 640:(k + 1) * 640] = _as_u32(ops.astype(BF16))

    def b2_body(i, carry):
        group = stage_v.at[pl.ds(i * PPB, PPB), pl.ds(0, DM), :]
        pltpu.make_async_copy(group, group, sem_st.at[i]).wait()
        wo_copy(i).wait()

        @pl.when(i == 2)
        def _():
            wsp_cp2.wait()

        u_transpose(0)
        for lp in range(2):
            tp = i * 2 + lp
            he = pl.multiple_of(tp * 128, 128)
            raw = lambda odd_t, odd_s: lambda k: wsp_v[
                pl.ds(he + odd_t * 64, 64), (2 * k + odd_s) * 128:(2 * k + odd_s + 1) * 128]
            tj = lambda j: lambda k: ts_v[:, k * 640 + j * 128:k * 640 + (j + 1) * 128]
            rhs = [tj(0), raw(0, 0), tj(1), tj(2), raw(1, 1), tj(3), tj(4)]

            part = functools.partial
            full = slice(0, 64)
            kinds = [[], []]
            if lp == 0:
                kinds[1] = [(9, part(split_block, i * PPB + pp, bi)) for pp in range(PPB) for bi in range(GH)]
            else:
                for sl in range(5):
                    gid = jnp.minimum((9 * i) // 2 + sl, (9 * i + 9) // 2 - 1)
                    f0h = (gid // NGRP) * H + (gid % NGRP) * GH
                    block = lambda bi, bj, f0h=f0h: wqkv_v[f0h + bj, 64 * bi:64 * bi + 64, :]
                    kinds[1] += [(30, part(weight_sums, block, wc_v.at[gid], full, idx)) for idx in range(GH)]
            if lp == 0:
                kinds.append([])
                for sl in range(2):
                    gid = jnp.minimum((3 * i) // 2 + sl, (3 * i + 3) // 2 - 1)
                    block = lambda bi, bj, gid=gid: wo_v[
                        pl.ds(pl.multiple_of((gid * GH + bi) * 64, 64), 64), bj * 128:(bj + 1) * 128]
                    kinds[-1] += [(30, part(weight_sums, block, woc_v.at[gid], full, idx)) for idx in range(GH)]
            r8 = pl.multiple_of(8 * (2 * i + lp), 8)
            block = lambda bi, bj, r8=r8: wout_v[pl.ds(64 * bi + r8, 8), bj * 128:(bj + 1) * 128]
            kinds.append([(4, part(weight_sums, block, woutc_v, pl.ds(r8, 8), idx)) for idx in range(GH)])
            order = sorted(((q + 0.5) / len(kd), kn, q) for kn, kd in enumerate(kinds) for q in range(len(kd)))
            tasks = ([(28, part(t_piece, tp, k)) for k in range(NK)]
                     + [kinds[kn][q] for _, kn, q in order])
            budget = sum(c for c, _ in tasks) / (2 * 7 * len(SBLK) - SIDE_TAIL)
            state = [0.0]

            def side(p):
                state[0] += budget
                phase = 0
                while tasks and state[0] > 0:
                    c, fn = tasks.pop(0)
                    rows = p[0:128].reshape(8, 16, 128)[:, 8 * phase:8 * phase + 8, :]
                    fn((pltpu.bitcast(rows, U32) & zero_v[...]).reshape(64, 128))
                    state[0] -= c
                    phase = 1 - phase

            def prod(j, f0, fn):
                p = None
                for ks in (range(NK // 2), range(NK // 2, NK)):
                    lhs = jnp.concatenate(
                        [za_v[k, f0 // 2:(f0 + fn) // 2, j * 128:(j + 1) * 128] for k in ks], axis=1)
                    r = jnp.concatenate([rhs[j](k) for k in ks], axis=1)
                    q = jax.lax.dot_general(_as_bf16(lhs), _as_bf16(r), NT, preferred_element_type=F32)
                    side(q)
                    p = q if p is None else p + q
                return p

            def finish(c, f0, fn, odd_t):
                tile = tp * 2 + odd_t
                z1 = _as_bf16(z1t_v[f0 // 2:(f0 + fn) // 2, _lanes(tile)]).astype(F32)
                brow = bsp32_v[pl.ds(tile, 1), :]
                z1t_v[f0 // 2:(f0 + fn) // 2, _lanes(tile)] = _as_u32((z1 * (0.5 * c + brow)).astype(BF16))

            blocks = [(sum(SBLK[:q]), fn) for q, fn in enumerate(SBLK)]
            early = [(prod(1, f0, fn), prod(4, f0, fn)) for f0, fn in blocks]
            for (f0, fn), (m2, m5) in zip(blocks, early):
                m4 = prod(3, f0, fn)
                finish(m2 + m4, FH // 2 + f0, fn, 0)
                m1 = prod(0, f0, fn)
                finish(m4 - m5 + m1 + prod(6, f0, fn), f0, fn, 0)
                m3 = prod(2, f0, fn)
                finish(m3 + m5, f0, fn, 1)
                finish(m3 - m2 + m1 + prod(5, f0, fn), FH // 2 + f0, fn, 1)
            assert not tasks
        return carry

    jax.lax.fori_loop(0, NB2, b2_body, 0)
    mem0_cp.wait()

    masks = _masks()
    for n, (keep, fill) in enumerate(masks):
        cap_v[n, 0:keep.shape[0], 0:keep.shape[1]] = jnp.where(keep, 0.0, fill)
    dot = lambda l, r: jnp.dot(l, r, preferred_element_type=F32)

    def fast_units(lhs_of, both, raw, sums, acc, done):
        items = []
        for i, row in enumerate(UNITS):
            for q, un in enumerate(row):
                def fn(un=un, last=(q == len(row) - 1), i=i):
                    if un[0] == 'b':
                        p = dot(both(un[1]), raw(un[1], un[2]))
                        hr = p.shape[0] // 2
                        acc.add((0, un[2]), 1, p[0:hr])
                        acc.add((1, un[2]), 1, p[hr:])
                    else:
                        r = un[2]
                        p = dot(lhs_of(un), raw(*list(r)[0]) if len(r) == 1 else sums(SUMS.index(r)))
                        for k, f in un[3]:
                            for half in range(2):
                                if f[half]:
                                    acc.add((half, k), f[half], p)
                    if last:
                        done(i)
                items.append((16 if un[0] == 'b' else 8, fn))
        return items

    def step(n, h):
        odd = n % 2 == 1
        hb = h.astype(BF16)
        qb = 24 * n
        kb = 40 * (n // 2) + (0 if odd else 16)
        nq, nk = (24, 40) if odd else (16, 24)
        clock = [0]
        d_s, d_o, gap, lag_v = PIPE[n]
        ready, s_at, o_at, ps = {}, {}, {}, {}

        def put(buf, r0, t, v):
            buf[r0:r0 + v.shape[0] // 2, _lanes(t)] = _as_u32(v.astype(BF16))

        def put64(m, t, top, bot):
            buf = (q_v, k_v, v_v)[m]
            if m == 0:
                put(buf, 0, t, top)
                put(buf, 24 + 16, t, bot[0:16])
                put(buf, 72 + 16, t, bot[16:32])
            else:
                put(buf, 16, t, top)
                put(buf, 32, t, bot[0:16])
                put(buf, 40 + 32, t, bot[16:32])
            ready[m, t] = clock[0]

        def plain(m, t):
            r = dot(hb, _as_bf16(wqkv_v[m * H + t]))
            if n == 0:
                put64(m, t, r[0:32], r[32:64])
            else:
                put((q_v, k_v, v_v)[m], qb if m == 0 else kb, t, r)
                ready[m, t] = clock[0]

        work = []
        if n == 0:
            cols = lambda i: slice(i * 128, (i + 1) * 128)
            make = _lhs_operands([h[0:32, cols(i)] for i in range(GH)], [h[32:64, cols(i)] for i in range(GH)])
            ops = {id(un): make(un) for row in UNITS for un in row if un[0] == 'p'}
            for g in range(NGRP):
                for m in ORDER0:
                    if g == NGRP - 1 and m == 2:
                        work += [(80, functools.partial(plain, mm, t))
                                 for t in range(NGRP * GH, H) for mm in (1, 0)]
                    acc = _Acc()
                    work += fast_units(
                        lambda un: ops[id(un)], lambda i: hb[:, cols(i)],
                        lambda i, j, m=m, g=g: _as_bf16(wqkv_v[m * H + g * GH + j, 64 * i:64 * i + 64, :]),
                        lambda q, m=m, g=g: _as_bf16(wc_v[m * NGRP + g, :, q * 128:(q + 1) * 128]),
                        acc, lambda j, m=m, g=g, acc=acc: put64(m, g * GH + j, acc.pop((0, j)), acc.pop((1, j))))
            work += [(80, functools.partial(plain, 2, t)) for t in range(NGRP * GH, H)]
        else:
            for t in range(H + lag_v):
                for m, tt in ((1, t), (2, t - lag_v), (0, t)):
                    if 0 <= tt < H:
                        work.append((40, functools.partial(plain, m, tt)))
        work = [(c, fn, -1) for c, fn in work]

        res = []
        if n == 3:
            acc = _Acc()
            for g in range(NGRP):
                hc = lambda i, g=g: slice((g * GH + i) * DH, (g * GH + i + 1) * DH)
                box = []

                def lhs_of(un, box=box, hc=hc):
                    if not box:
                        box.append(_lhs_operands([up(o_v[0:16, hc(i)]) for i in range(GH)],
                                                 [up(o_v[16:32, hc(i)]) for i in range(GH)]))
                    return box[0](un)

                items = fast_units(
                    lhs_of, lambda i, hc=hc: _as_bf16(o_v[:, hc(i)]),
                    lambda i, j, g=g: _as_bf16(wo_v[(g * GH + i) * 64:(g * GH + i + 1) * 64, j * 128:(j + 1) * 128]),
                    lambda q, g=g: _as_bf16(woc_v[g, :, q * 128:(q + 1) * 128]), acc, lambda j: None)
                work += [(c, fn, g * GH + GH - 1) for c, fn in items]

            def tail():
                c0 = NGRP * GH * DH
                part = dot(_as_bf16(o_v[:, c0:]), _as_bf16(wo_v[c0 // 2:, :]))
                res.append(part + jnp.concatenate(
                    [jnp.concatenate([acc.pop((hf, j)) for j in range(GH)], axis=1) for hf in range(2)], axis=0))

            work.append((160, tail, H - 1))
        else:
            def wgroup(g):
                c0, c1 = g * WG * DH, (g + 1) * WG * DH
                part = dot(_as_bf16(o_v[0:16, c0:c1]), _as_bf16(wo_v[c0 // 2:c1 // 2, :]))
                res[:] = [part + res[0]] if res else [part]

            work += [(40 * WG, functools.partial(wgroup, g), (g + 1) * WG - 1) for g in range(H // WG)]

        def scores(t):
            sc = jax.lax.dot_general(_as_bf16(q_v[qb:qb + nq, _lanes(t)]),
                                     _as_bf16(k_v[kb:kb + nk, _lanes(t)]), NT,
                                     preferred_element_type=F32) * SCALE
            cap = cap_v[n, 0:sc.shape[0], 0:sc.shape[1]]
            sc = jnp.where(cap == 0.0, sc, cap)
            e = jnp.exp(sc - jnp.max(sc, axis=-1, keepdims=True))
            l = jnp.sum(e, axis=-1, keepdims=True)
            inv = pl.reciprocal(l, approx=True)
            inv = inv * (2.0 - l * inv)
            ps[t] = (e * inv).astype(BF16)
            s_at[t] = clock[0]
            clock[0] += nq // 2

        def values(t):
            o = dot(ps.pop(t), _as_bf16(v_v[kb:kb + nk, _lanes(t)]))
            if n == 1:
                put(o_v, 0, t, o[0:32])
                put(o_v, 24, t, o[32:48])
            else:
                put(o_v, 0, t, o)
            o_at[t] = clock[0]
            clock[0] += nq // 2

        def drain(upto):
            while True:
                to, ts = len(o_at), len(s_at)
                if to < ts and (2, to) in ready and (
                        to <= upto or clock[0] >= max(s_at[to] + d_o, ready[2, to] + d_s)):
                    values(to)
                elif ts < H and (0, ts) in ready and (1, ts) in ready and (
                        ts <= upto or clock[0] >= max(ready[0, ts] + d_s, ready[1, ts] + d_s,
                                                      s_at.get(ts - 1, -gap) + gap)):
                    scores(ts)
                else:
                    return

        for c, fn, need in work:
            drain(need)
            clock[0] += c
            fn()
        return res[0]

    def gate_work():
        acc = _Acc()
        cols = lambda i: slice(i * 128, (i + 1) * 128)
        box = []

        def lhs_of(un):
            if not box:
                box.append(_lhs_operands([up(u_v[0:32, cols(i)]) for i in range(GH)],
                                         [up(u_v[32:64, cols(i)]) for i in range(GH)]))
            return box[0](un)

        items = [(2 * c, fn) for c, fn in fast_units(
            lhs_of, lambda i: _as_bf16(u_v[:, cols(i)]),
            lambda i, j: _as_bf16(wout_v[64 * i:64 * i + 64, cols(j)]),
            lambda q: _as_bf16(woutc_v[:, cols(q)]), acc, lambda j: None)]

        def rest(j):
            p = dot(_as_bf16(u_v[:, DM:FH]), _as_bf16(wout_v[DM // 2:FH // 2, cols(j)]))
            acc.add((0, j), 1, p[0:64])
            acc.add((1, j), 1, p[64:128])

        items = [(64, functools.partial(rest, j)) for j in range(GH)] + items

        def chunk(budget):
            box.clear()
            while items and budget > 0:
                c, fn = items.pop(0)
                fn()
                budget -= c

        def result():
            hb = 0.5 * jnp.concatenate(
                [jnp.concatenate([acc.pop((hf, j)) for j in range(GH)], axis=1) for hf in range(2)], axis=0)
            return hb + hb * jnp.tanh(hb)

        return chunk, result

    def tile_body(j, mem):
        r0 = pl.multiple_of(j * 128, 128)
        xs = _as_bf16(xn_v[pl.ds(pl.multiple_of(j * 64, 64), 64), :]).astype(F32)
        chunk, gate_result = gate_work()
        chunk(FILL[0])
        a0 = step(0, jnp.concatenate([mem, xs[0:40], xs[64:72], xs[96:104]], axis=0))
        chunk(FILL[1])
        a1 = step(1, jnp.concatenate([a0[0:MEM], xs[40:64]], axis=0))
        chunk(FILL[2])
        a2 = step(2, jnp.concatenate([a1[0:MEM], xs[72:96]], axis=0))
        chunk(10 ** 6)
        gate = gate_result()
        u_transpose(jnp.minimum(j + 1, NTILE - 1))
        a3 = step(3, jnp.concatenate([a2[0:MEM], xs[104:128]], axis=0))
        s_rows = jnp.concatenate([a0[8:32], a3[48:64], a1[8:32], a3[32:40], a2[8:32], a3[40:48], a3[8:32]],
                                 axis=0)
        res = x_v[pl.ds(r0, 128), :].astype(F32) + s_rows * gate
        out_v[pl.ds(r0, 128), :] = res.astype(BF16)
        pltpu.make_async_copy(out_v.at[pl.ds(r0, 128), :],
                              out_hbm.at[pl.ds(r0, 128), :], sem_out).start()
        return a3[0:MEM]

    jax.lax.fori_loop(0, NTILE, tile_body, mem0_v[...].astype(F32))
    pltpu.make_async_copy(out_v, out_hbm, sem_out).wait()


@jax.jit
def pallas_recurrent_scan__memory_aug_recurrent_mem_tr__mixer_gmlp__prompt_kernel(
    A_x: jax.Array,
    A_mem0: jax.Array,
    A_Wq: jax.Array,
    A_Wk: jax.Array,
    A_Wv: jax.Array,
    A_Wo: jax.Array,
    A_seg_len: jax.Array,
    B_x: jax.Array,
    B_w_in: jax.Array,
    B_w_sp: jax.Array,
    B_b_sp: jax.Array,
    B_w_out: jax.Array,
):
    del A_seg_len, B_x
    hbm = pl.BlockSpec(memory_space=pl.ANY)
    out = pl.pallas_call(
        _kernel,
        out_shape=jax.ShapeDtypeStruct((S, DM), BF16),
        in_specs=[hbm] * 10,
        out_specs=hbm,
        scratch_shapes=[
            pltpu.VMEM((S, DM), BF16),
            pltpu.VMEM((S // 2, DM), U32),
            pltpu.VMEM((64, 2048), U32),
            pltpu.VMEM((64, 2048), U32),
            pltpu.VMEM((MEM, DM), BF16),
            pltpu.VMEM((16, 128), BF16),
            pltpu.VMEM((16, 128), F32),
            pltpu.VMEM((8, 128), U32),
            pltpu.VMEM((FH, DM), U32),
            pltpu.VMEM((FH // 2, 1280), U32),
            pltpu.VMEM((S // 2, S), U32),
            pltpu.VMEM((FH // 2, DM), U32),
            pltpu.VMEM((64, NSUM * 128), U32),
            pltpu.VMEM((48, DM + 8, DH), U32),
            pltpu.VMEM((3 * H, DM // 2, DH), U32),
            pltpu.VMEM((3 * NGRP, 64, NSUM * 128), U32),
            pltpu.VMEM((H * DH // 2, DM), U32),
            pltpu.VMEM((NGRP, 64, NSUM * 128), U32),
            pltpu.VMEM((T1, FH, 128), F32),
            pltpu.VMEM((T1, 2 * (FH // RB) * 8, 128), F32),
            pltpu.VMEM((FH // 2, S), U32),
            pltpu.VMEM((NTILE // 2, FH // 4, 7 * 128), U32),
            pltpu.VMEM((64, 5 * S // 2), U32),
            pltpu.VMEM((64, FH), U32),
            pltpu.VMEM((96, H * DH), U32),
            pltpu.VMEM((80, H * DH), U32),
            pltpu.VMEM((80, H * DH), U32),
            pltpu.VMEM((32, H * DH), U32),
            pltpu.VMEM((4, 48, 80), F32),
            pltpu.VMEM((S, DM), BF16),
            pltpu.SemaphoreType.DMA((4,)),
            pltpu.SemaphoreType.DMA((8,)),
            pltpu.SemaphoreType.DMA((NTILE // T2,)),
            pltpu.SemaphoreType.DMA((NTILE // T2,)),
            pltpu.SemaphoreType.DMA,
        ],
        compiler_params=pltpu.CompilerParams(vmem_limit_bytes=112 * 1024 * 1024),
    )(
        A_x.reshape(S, DM),
        A_mem0.reshape(MEM, DM),
        A_Wq, A_Wk, A_Wv,
        A_Wo.reshape(H * DH, DM),
        B_w_in.T,
        B_w_sp,
        B_b_sp.reshape(16, 128),
        B_w_out,
    )
    return out.reshape(1, S, DM)
```

```python
import functools

import jax
import jax.numpy as jnp
import jax.experimental.pallas as pl
import jax.experimental.pallas.tpu as pltpu

F32 = jnp.float32
BF16 = jnp.bfloat16
U32 = jnp.uint32

S = 2048
DM = 640
H = 32
DH = 128
MEM = 8
SEG = 32
FH = 864
NTILE = S // 128
EPS = 1e-5
SCALE = DH ** (-0.5)
NEG = -1000000000.0

XCH = 256
T1 = 4
T2 = 4
RB = 144
WIN_PIECES = (2, 4, 6)
SBLK = (144, 144, 144)
SIDE_TAIL = 1
WSP_HEAD = 512
LN_DEADLINE = 10
LN_FIRST = 4
NORM_TAIL = 4
ORDER0 = (1, 0, 2)
PIPE = ((270, 450, 170, 0), (230, 540, 128, 1), (210, 600, 100, 0), (230, 470, 112, 4))
WG = 4
FILL = (320, 224, 224)

NT = (((1,), (1,)), ((), ()))


def _as_bf16(u):
    return pltpu.bitcast(u, BF16)


def _as_u32(b):
    return pltpu.bitcast(b, U32)


def _layernorm(v):
    m = jnp.mean(v, axis=-1, keepdims=True)
    c = v - m
    var = jnp.mean(c * c, axis=-1, keepdims=True)
    return c * jax.lax.rsqrt(var + EPS)


def _gelu2(v):
    c = 0.7978845608028654
    return v + v * jnp.tanh(v * (c + (c * 0.044715) * (v * v)))


def _mult(v, m):
    return v if isinstance(v, int) else pl.multiple_of(v, m)


def _lanes(tile):
    return pl.ds(_mult(tile * 128, 128), 128)


def _mask(qgroups, kgroups):
    shape = (8 * len(qgroups), 8 * len(kgroups))

    def table(groups, axis):
        idx = jax.lax.broadcasted_iota(jnp.int32, shape, axis)
        seg = jnp.full(shape, groups[-1][0], jnp.int32)
        pos = idx + (groups[-1][1] - 8 * (len(groups) - 1))
        for g in range(len(groups) - 2, -1, -1):
            inside = idx < 8 * (g + 1)
            seg = jnp.where(inside, groups[g][0], seg)
            pos = jnp.where(inside, idx + (groups[g][1] - 8 * g), pos)
        return seg, pos

    qseg, qpos = table(qgroups, 0)
    kseg, kpos = table(kgroups, 1)
    same = qseg == kseg
    keep = same & ((qpos < MEM) | (qpos >= kpos))
    return keep, jnp.where(same, NEG, -jnp.inf).astype(F32)


def _masks():
    own = lambda sg: [(sg, 0), (sg, 16), (sg, 24), (sg, 32)]
    k0 = [(0, 0), (0, 8), (0, 16), (0, 24), (0, 32), (1, 8)]
    k2 = own(2) + [(2, 8), (3, 8)]
    return [
        _mask(k0[:4], k0),
        _mask(own(1) + k0[4:], own(1) + k0),
        _mask(own(2), k2),
        _mask(own(3) + k2[4:], own(3) + k2),
    ]


def _fast_table(types):
    lines = {0: ((1, 0), (1, -1)), 1: ((0, 1), (1, -1)), 2: ((1, 0), (0, 1))}
    neg = lambda f: (-f[0], -f[1])

    def dual(u, v):
        det = u[0] * v[1] - u[1] * v[0]
        return (v[1] * det, -v[0] * det), (-u[1] * det, u[0] * det)

    n = len(types)
    diag = {(i, k): {(i, i): 1} for i in range(n) for k in range(2)}
    units = [[] for _ in range(n)]
    for i in range(n):
        u = lines[types[i]]
        units[i] += [('p', [(i, u[k])], diag[i, k], [(i, dual(*u)[k])]) for k in range(2)]
        for j in range(i + 1, n):
            if types[i] == types[j]:
                units[i] += [('b', i, j), ('b', j, i)]
                continue
            w = lines[types[j]]
            (ci, cj), = [(x, y) for x in range(2) for y in range(2) if u[x] == w[y]]
            (p, q), = [(x, y) for x in (u[1 - ci], neg(u[1 - ci])) for y in (w[1 - cj], neg(w[1 - cj]))
                       if (x[0] - y[0], x[1] - y[1]) == u[ci]]
            sd, td = dual(p, q)
            units[i] += [('p', [(i, p), (j, q)], {(i, j): 1, (j, i): 1}, [(i, td), (j, sd)]),
                         ('p', [(i, q), (j, q)], {(i, j): 1}, [(i, neg(td)), (j, td)]),
                         ('p', [(i, p), (j, p)], {(j, i): 1}, [(i, sd), (j, neg(sd))])]
            diag[i, ci][i, j] = 1
            diag[i, 1 - ci][j, i] = -1
            diag[j, 1 - cj][i, j] = -1
            diag[j, cj][j, i] = 1
    out = []
    for i in range(n):
        row = []
        for un in units[i]:
            if un[0] == 'p' and [c for c in un[1][0][1] if c][0] < 0:
                un = ('p', [(k, neg(f)) for k, f in un[1]], un[2], [(k, neg(f)) for k, f in un[3]])
            row.append(un)
        out.append(row)
    return out


GH = 5
NGRP = H // GH
WOFF = H - NGRP * GH
UNITS = _fast_table((0, 1, 2, 0, 1))
SUMS = [un[2] for row in UNITS for un in row if un[0] == 'p' and len(un[2]) > 1]
NSUM = len(SUMS)


def _signed_sum(terms):
    terms = sorted(terms, key=lambda cv: -cv[0])
    acc = terms[0][1]
    for c, v in terms[1:]:
        acc = acc + v if c > 0 else acc - v
    return acc


def _lhs_operands(top, bot):
    forms = {}

    def form(i, f):
        sign = 1 if [c for c in f if c][0] > 0 else -1
        key = (i, (sign * f[0], sign * f[1]))
        if key not in forms:
            forms[key] = {(1, 0): lambda: top[i], (0, 1): lambda: bot[i],
                          (1, -1): lambda: top[i] - bot[i]}[key[1]]()
        return sign, forms[key]

    return lambda un: _signed_sum([form(i, f) for i, f in un[1]]).astype(BF16)


class _Acc:
    def __init__(self):
        self.v = {}

    def add(self, key, c, p):
        if key not in self.v:
            self.v[key] = (c, p)
        else:
            sign, v = self.v[key]
            self.v[key] = (sign, v + p if sign == c else v - p)

    def pop(self, key):
        sign, v = self.v.pop(key)
        return v if sign > 0 else -v


def _kernel(x_hbm, mem0_hbm, wq_hbm, wk_hbm, wv_hbm, wo_hbm, wint_hbm, wsp_hbm,
            bsp_hbm, wout_hbm, out_hbm,
            x_v, xn_v, xa_v, xb_v, mem0_v, bsp_v, bsp32_v, zero_v, wint_v, wins_v, wsp_v, wout_v, woutc_v,
            stage_v, wqkv_v, wc_v, wo_v, woc_v, zg_v, st_v, z1t_v, za_v, ts_v, u_v, q_v, k_v, v_v, o_v, cap_v, out_v,
            sem_x, sem_w, sem_st, sem_wo, sem_out):
    NRB = FH // RB
    NG = RB // 8
    NB2 = NTILE // T2
    PPB = 48 // NB2

    x_parts = [(0, XCH), (XCH, XCH), (2 * XCH, XCH), (3 * XCH, S - 3 * XCH)]
    x_cps = [pltpu.make_async_copy(x_hbm.at[pl.ds(o, n), :], x_v.at[pl.ds(o, n), :], sem_x.at[k])
             for k, (o, n) in enumerate(x_parts)]
    wint_u = wint_hbm.bitcast(U32)
    blk_row = lambda k: (FH + k * RB) if k < NRB else (k - NRB) * RB
    wint_cps, k0 = [], 0
    for k, nb in enumerate(WIN_PIECES):
        o, n = blk_row(k0) // 2, nb * RB // 2
        wint_cps.append(pltpu.make_async_copy(wint_u.at[pl.ds(o, n), :], wint_v.at[pl.ds(o, n), :],
                                              sem_w.at[k]))
        k0 += nb
    wsp_u = wsp_hbm.bitcast(U32)
    wsp_cp = pltpu.make_async_copy(wsp_u.at[pl.ds(0, WSP_HEAD), :], wsp_v.at[pl.ds(0, WSP_HEAD), :],
                                   sem_w.at[3])
    wsp_cp2 = pltpu.make_async_copy(wsp_u.at[pl.ds(WSP_HEAD, S // 2 - WSP_HEAD), :],
                                    wsp_v.at[pl.ds(WSP_HEAD, S // 2 - WSP_HEAD), :], sem_w.at[7])
    wout_cp = pltpu.make_async_copy(wout_hbm.bitcast(U32), wout_v, sem_w.at[4])
    WOQ = H * DH // 2 // NB2

    def wo_copy(i):
        r0 = _mult(i * WOQ, WOQ)
        return pltpu.make_async_copy(wo_hbm.bitcast(U32).at[pl.ds(r0, WOQ), :],
                                     wo_v.at[pl.ds(r0, WOQ), :], sem_wo.at[i])

    mem0_cp = pltpu.make_async_copy(mem0_hbm, mem0_v, sem_w.at[5])
    bsp_cp = pltpu.make_async_copy(bsp_hbm, bsp_v, sem_w.at[6])
    w_hbms = (wq_hbm, wk_hbm, wv_hbm)

    def stage_copy(m, j):
        p = m * 16 + j
        return pltpu.make_async_copy(w_hbms[m].bitcast(U32).at[:, j, :],
                                     stage_v.at[p, pl.ds(0, DM), :], sem_st.at[p // PPB])

    x_cps[0].start()
    x_cps[1].start()
    for cp in wint_cps:
        cp.start()
    x_cps[2].start()
    x_cps[3].start()
    bsp_cp.start()
    wsp_cp.start()
    wout_cp.start()
    for p in range(48):
        stage_copy(p // 16, p % 16).start()
        if (p + 1) % PPB == 0:
            wo_copy(p // PPB).start()
        if p + 1 == 2 * PPB:
            wsp_cp2.start()
    mem0_cp.start()

    zero_v[...] = jnp.zeros((8, 128), U32)

    pending = []

    def dep_of(v):
        return pltpu.bitcast(v[0:8, 0:128], U32) & zero_v[...]

    def up(u):
        return _as_bf16(u).astype(F32)

    def ln_rows(r0, n, dep=None):
        xr = x_v[pl.ds(r0, n), :].astype(F32)
        if dep is not None:
            d = jnp.concatenate([dep] * (n // 8), axis=0)
            xr = pltpu.bitcast(pltpu.bitcast(xr, U32) | jnp.concatenate([d] * (DM // 128), axis=1), F32)
        xn = _layernorm(xr)
        xn_v[pl.ds(_mult(r0 // 2, n // 2), n // 2), :] = _as_u32(xn.astype(BF16))
        return xn

    def ln_pair(base, k, dst, dep):
        xe = ln_rows(_mult(base + 16 * k, 16), 16, dep)
        xo = ln_rows(_mult(base + 128 + 16 * k, 16), 16, dep)
        b11, b21, b12, b22 = xe[:, 0:256], xe[:, 256:512], xo[:, 0:256], xo[:, 256:512]
        ops = jnp.concatenate([b11 + b22, b11, b12 - b22, b21 - b11, b22,
                               b11 + b12, xo[:, 512:], b21 + b22, xe[:, 512:]], axis=1)
        dst[8 * k:8 * k + 8, :] = _as_u32(ops.astype(BF16))
        pending.append([LN_DEADLINE, dst[8 * k:8 * k + 8, 0:128] & zero_v[...]])

    def win_sums(hz, k, dep):
        d = jnp.concatenate([dep] * 4, axis=1)
        r0 = hz * (FH // 2) + 8 * k
        top, bot = up(wint_v[r0:r0 + 8, 0:512] | d), up(wint_v[r0 + FH // 4:r0 + FH // 4 + 8, 0:512] | d)
        a11, a12, a21, a22 = top[:, 0:256], top[:, 256:512], bot[:, 0:256], bot[:, 256:512]
        ops = jnp.concatenate([a11 + a22, a21 + a22, a11 + a12, a21 - a11, a12 - a22], axis=1)
        wins_v[hz * (FH // 4) + 8 * k:hz * (FH // 4) + 8 * k + 8, :] = _as_u32(ops.astype(BF16))

    def nt_dot(w, xt):
        due = None
        for e in pending:
            e[0] -= 1
            if e[0] == 0:
                due = e[1] if due is None else due | e[1]
        pending[:] = [e for e in pending if e[0] > 0]
        if due is not None:
            top = w[0:8, 0:128] | due
            if w.shape[1] > 128:
                top = jnp.concatenate([top, w[0:8, 128:]], axis=1)
            w = jnp.concatenate([top, w[8:]], axis=0)
        return jax.lax.dot_general(_as_bf16(w), _as_bf16(xt), NT, preferred_element_type=F32)

    def win_block(nt, f0):
        return nt_dot(wint_v[f0 // 2:(f0 + RB) // 2, :], xn_v[nt * 64:(nt + 1) * 64, :])

    def win_group(src, hz, rb, emit, side):
        rt = (hz * FH + rb * RB) // 2
        rows = lambda r: slice(r, r + RB // 2)
        top, bot, sm = rows(rt), rows(rt + FH // 4), rows(hz * (FH // 4) + rb * RB // 2)
        ss = lambda q: wins_v[sm, q * 256:(q + 1) * 256]
        tt = lambda q: src[:, q * 256:(q + 1) * 256]
        rest = lambda r: wint_v[r, 512:640]

        def prod(w, xt):
            p = nt_dot(w, xt)
            side(p)
            return p

        m2 = prod(ss(1), tt(1))
        m4 = prod(wint_v[bot, 256:512], tt(3))
        emit(0, rb + NRB // 2, m2 + m4 + prod(rest(bot), src[:, 1920:2048]))
        m3 = prod(wint_v[top, 0:256], tt(2))
        m5 = prod(ss(2), tt(4))
        emit(1, rb, m3 + m5 + prod(rest(top), src[:, 1536:1664]))
        c11, c22 = m4 - m5, m3 - m2
        m1 = prod(ss(0), tt(0))
        emit(0, rb, c11 + m1 + prod(jnp.concatenate([ss(4), rest(top)], axis=1), src[:, 1664:2048]))
        emit(1, rb + NRB // 2,
             c22 + m1 + prod(jnp.concatenate([ss(3), rest(bot)], axis=1), src[:, 1280:1664]))

    def z2_emit(nt, rb, z):
        g = _gelu2(z)
        zg_v[nt, rb * RB:(rb + 1) * RB, :] = g
        g3 = g.reshape(NG, 8, 128)
        bm = jnp.sum(g3, axis=0) * (1.0 / NG)
        c = g3 - bm
        st_v[nt, rb * 8:(rb + 1) * 8, :] = bm
        st_v[nt, (NRB + rb) * 8:(NRB + rb + 1) * 8, :] = jnp.sum(c * c, axis=0)

    def z2_stats(nt):
        bm = st_v[nt, 0:NRB * 8, :]
        m = jnp.sum(bm, axis=0, keepdims=True) * (1.0 / (NRB * 8))
        dm = bm - m
        m2 = jnp.sum(st_v[nt, NRB * 8:2 * NRB * 8, :] + dm * dm * NG, axis=0, keepdims=True)
        r = jax.lax.rsqrt(m2 * (1.0 / FH) + 4.0 * EPS)
        return jnp.broadcast_to(m, (8, 128)), jnp.broadcast_to(r, (8, 128))

    def z2_norm(ne, tp, k, st, dep):
        (me, re), (mo, ro) = st
        me = pltpu.bitcast(pltpu.bitcast(me, U32) | dep, F32)
        mo = pltpu.bitcast(pltpu.bitcast(mo, U32) | dep, F32)
        nrm = lambda nt, f0, m, r: ((zg_v[nt, f0:f0 + 16, :].reshape(2, 8, 128) - m) * r).reshape(16, 128)
        a11, a21 = nrm(ne, 16 * k, me, re), nrm(ne, FH // 2 + 16 * k, me, re)
        a12, a22 = nrm(ne + 1, 16 * k, mo, ro), nrm(ne + 1, FH // 2 + 16 * k, mo, ro)
        ops = jnp.concatenate([a11 + a22, a21 + a22, a11, a22, a11 + a12, a21 - a11, a12 - a22], axis=1)
        za_v.at[tp][8 * k:8 * k + 8, :] = _as_u32(ops.astype(BF16))

    def z1_emit(tile, rb, z):
        z1t_v[rb * RB // 2:(rb + 1) * RB // 2, _lanes(tile)] = _as_u32(_gelu2(z).astype(BF16))

    def spread(tasks, slots):
        state = [0]

        def side(p):
            n = state[0]
            mine = tasks[n * len(tasks) // slots:(n + 1) * len(tasks) // slots]
            for q, fn in enumerate(mine):
                fn(dep_of(p[8 * ((q * NG) // len(mine)):]))
            state[0] += 1

        return side

    def mix(*kinds):
        order = sorted(((q + 0.5) / len(kd), kn, q) for kn, kd in enumerate(kinds) for q in range(len(kd)))
        return [kinds[kn][q] for _, kn, q in order]

    part = functools.partial
    NSLAB = FH // 32

    x_cps[0].wait()
    ln_rows(0, XCH)
    x_cps[1].wait()
    ln_rows(XCH, XCH)
    wint_cps[0].wait()
    for nt in range(T1):
        for rb in range(WIN_PIECES[0]):
            z2_emit(nt, rb, win_block(nt, FH + rb * RB))
    wint_cps[1].wait()
    side = spread([part(win_sums, 1, k) for k in range(NSLAB)], T1 * (NRB - WIN_PIECES[0]) - 1)
    for nt in range(T1):
        for rb in range(WIN_PIECES[0], NRB):
            z = win_block(nt, FH + rb * RB)
            z2_emit(nt, rb, z)
            side(z)
    wint_cps[2].wait()
    x_cps[2].wait()
    norms = []
    for ne in range(0, T1, 2):
        st = (z2_stats(ne), z2_stats(ne + 1))
        norms += [part(z2_norm, ne, ne // 2, k, st) for k in range(NSLAB)]
    side = spread(mix(norms, [part(win_sums, 0, k) for k in range(NSLAB)],
                      [part(ln_pair, T1 * 128, k, xa_v) for k in range(8)]), T1 * NRB - 1)
    for nt in range(T1):
        for rb in range(NRB):
            z = win_block(nt, rb * RB)
            z1_emit(nt, rb, z)
            side(z)
    x_cps[3].wait()
    pending.clear()

    def b1_body(i, carry):
        for ne in range(0, T1, 2):
            tile = i * T1 + ne
            src, dst = (xa_v, xb_v) if ne == 0 else (xb_v, xa_v)
            base = jnp.minimum(tile + 2, NTILE - 2) * 128
            lns = [part(ln_pair, base, k, dst) for k in range(8)]
            side = spread(lns[:LN_FIRST], 9 * NRB // 2)
            for rb in range(NRB // 2):
                win_group(src, 1, rb, lambda o, r, z: z2_emit(ne + o, r, z), side)
            st = (z2_stats(ne), z2_stats(ne + 1))
            norms = [part(z2_norm, ne, tile // 2, k, st) for k in range(NSLAB)]
            side = spread(mix(norms, lns[LN_FIRST:]) if LN_FIRST < 8 else norms, 9 * NRB // 2 - NORM_TAIL)
            for rb in range(NRB // 2):
                win_group(src, 0, rb, lambda o, r, z: z1_emit(tile + o, r, z), side)
        pending.clear()
        return carry

    jax.lax.fori_loop(1, NTILE // T1, b1_body, 0)

    wsp_cp.wait()
    wout_cp.wait()
    bsp_cp.wait()
    bsp32_v[...] = 0.5 * bsp_v[...].astype(F32)

    def split_block(p, bi, dep):
        a = stage_v[p, pl.ds(128 * bi, 64, stride=2), :] | dep
        b = stage_v[p, pl.ds(128 * bi + 1, 64, stride=2), :] | dep
        wqkv_v[2 * p, 64 * bi:64 * bi + 64, :] = (a & jnp.uint32(0xFFFF)) | (b << 16)
        wqkv_v[2 * p + 1, 64 * bi:64 * bi + 64, :] = (a >> 16) | (b & jnp.uint32(0xFFFF0000))

    def weight_sums(block, dst, rows, idx, dep):
        cache = {}

        def blk(ij):
            if ij not in cache:
                w = block(*ij)
                cache[ij] = up(w | dep[0:w.shape[0]])
            return cache[ij]

        mine = [un[2] for un in UNITS[idx] if un[0] == 'p' and len(un[2]) > 1]
        c0 = SUMS.index(mine[0])
        sums = jnp.concatenate([_signed_sum([(c, blk(ij)) for ij, c in r.items()]) for r in mine], axis=1)
        dst[rows, c0 * 128:(c0 + len(mine)) * 128] = _as_u32(sums.astype(BF16))

    fblocks = [(f0, min(128, FH - f0)) for f0 in range(0, FH, 128)]

    def u_transpose(tile):
        for f0, fn in fblocks:
            ut = _as_bf16(z1t_v[f0 // 2:(f0 + fn) // 2, _lanes(tile)]).astype(F32)
            u_v[:, f0:f0 + fn] = _as_u32(ut.T.astype(BF16))

    NK = NTILE // 2

    def t_piece(tp, k, dep):
        h0 = _mult(tp * 128, 128)
        we = wsp_v[pl.ds(h0, 64), k * 256:(k + 1) * 256]
        wo = wsp_v[pl.ds(h0 + 64, 64), k * 256:(k + 1) * 256]
        d = jnp.concatenate([dep, dep], axis=1)
        we, wo = up(we | d), up(wo | d)
        b11, b21, b12, b22 = we[:, 0:128], we[:, 128:256], wo[:, 0:128], wo[:, 128:256]
        ops = jnp.concatenate([b11 + b22, b12 - b22, b21 - b11, b11 + b12, b21 + b22], axis=1)
        z0 = pl.multiple_of(jnp.minimum(tp, 0) * 64, 64)
        ts_v[pl.ds(z0, 64), k * 640:(k + 1) * 640] = _as_u32(ops.astype(BF16))

    def b2_body(i, carry):
        group = stage_v.at[pl.ds(i * PPB, PPB), pl.ds(0, DM), :]
        pltpu.make_async_copy(group, group, sem_st.at[i]).wait()
        wo_copy(i).wait()

        @pl.when(i == 2)
        def _():
            wsp_cp2.wait()

        u_transpose(0)
        for lp in range(2):
            tp = i * 2 + lp
            he = pl.multiple_of(tp * 128, 128)
            raw = lambda odd_t, odd_s: lambda k: wsp_v[
                pl.ds(he + odd_t * 64, 64), (2 * k + odd_s) * 128:(2 * k + odd_s + 1) * 128]
            tj = lambda j: lambda k: ts_v[:, k * 640 + j * 128:k * 640 + (j + 1) * 128]
            rhs = [tj(0), raw(0, 0), tj(1), tj(2), raw(1, 1), tj(3), tj(4)]

            part = functools.partial
            full = slice(0, 64)
            kinds = [[], []]
            if lp == 0:
                kinds[1] = [(9, part(split_block, i * PPB + pp, bi)) for pp in range(PPB) for bi in range(GH)]
            else:
                for sl in range(5):
                    gid = jnp.minimum((9 * i) // 2 + sl, (9 * i + 9) // 2 - 1)
                    f0h = (gid // NGRP) * H + (gid % NGRP) * GH
                    block = lambda bi, bj, f0h=f0h: wqkv_v[f0h + bj, 64 * bi:64 * bi + 64, :]
                    kinds[1] += [(30, part(weight_sums, block, wc_v.at[gid], full, idx)) for idx in range(GH)]
            if lp == 0:
                kinds.append([])
                for sl in range(2):
                    gid = jnp.maximum(i, 2 * i - 2 + sl)
                    block = lambda bi, bj, gid=gid: wo_v[
                        pl.ds(pl.multiple_of((WOFF + gid * GH + bi) * 64, 64), 64), bj * 128:(bj + 1) * 128]
                    kinds[-1] += [(30, part(weight_sums, block, woc_v.at[gid], full, idx)) for idx in range(GH)]
            r8 = pl.multiple_of(8 * (2 * i + lp), 8)
            block = lambda bi, bj, r8=r8: wout_v[pl.ds(64 * bi + r8, 8), bj * 128:(bj + 1) * 128]
            kinds.append([(4, part(weight_sums, block, woutc_v, pl.ds(r8, 8), idx)) for idx in range(GH)])
            order = sorted(((q + 0.5) / len(kd), kn, q) for kn, kd in enumerate(kinds) for q in range(len(kd)))
            tasks = ([(28, part(t_piece, tp, k)) for k in range(NK)]
                     + [kinds[kn][q] for _, kn, q in order])
            budget = sum(c for c, _ in tasks) / (2 * 7 * len(SBLK) - SIDE_TAIL)
            state = [0.0]

            def side(p):
                state[0] += budget
                phase = 0
                while tasks and state[0] > 0:
                    c, fn = tasks.pop(0)
                    rows = p[0:128].reshape(8, 16, 128)[:, 8 * phase:8 * phase + 8, :]
                    fn((pltpu.bitcast(rows, U32) & zero_v[...]).reshape(64, 128))
                    state[0] -= c
                    phase = 1 - phase

            def prod(j, f0, fn):
                p = None
                for ks in (range(NK // 2), range(NK // 2, NK)):
                    lhs = jnp.concatenate(
                        [za_v[k, f0 // 2:(f0 + fn) // 2, j * 128:(j + 1) * 128] for k in ks], axis=1)
                    r = jnp.concatenate([rhs[j](k) for k in ks], axis=1)
                    q = jax.lax.dot_general(_as_bf16(lhs), _as_bf16(r), NT, preferred_element_type=F32)
                    side(q)
                    p = q if p is None else p + q
                return p

            def finish(c, f0, fn, odd_t):
                tile = tp * 2 + odd_t
                z1 = _as_bf16(z1t_v[f0 // 2:(f0 + fn) // 2, _lanes(tile)]).astype(F32)
                brow = bsp32_v[pl.ds(tile, 1), :]
                z1t_v[f0 // 2:(f0 + fn) // 2, _lanes(tile)] = _as_u32((z1 * (0.5 * c + brow)).astype(BF16))

            blocks = [(sum(SBLK[:q]), fn) for q, fn in enumerate(SBLK)]
            early = [(prod(1, f0, fn), prod(4, f0, fn)) for f0, fn in blocks]
            for (f0, fn), (m2, m5) in zip(blocks, early):
                m4 = prod(3, f0, fn)
                finish(m2 + m4, FH // 2 + f0, fn, 0)
                m1 = prod(0, f0, fn)
                finish(m4 - m5 + m1 + prod(6, f0, fn), f0, fn, 0)
                m3 = prod(2, f0, fn)
                finish(m3 + m5, f0, fn, 1)
                finish(m3 - m2 + m1 + prod(5, f0, fn), FH // 2 + f0, fn, 1)
            assert not tasks
        return carry

    jax.lax.fori_loop(0, NB2, b2_body, 0)
    mem0_cp.wait()

    masks = _masks()
    for n, (keep, fill) in enumerate(masks):
        cap_v[n, 0:keep.shape[0], 0:keep.shape[1]] = jnp.where(keep, 0.0, fill)
    dot = lambda l, r: jnp.dot(l, r, preferred_element_type=F32)

    def fast_units(lhs_of, both, raw, sums, acc, done):
        items = []
        for i, row in enumerate(UNITS):
            for q, un in enumerate(row):
                def fn(un=un, last=(q == len(row) - 1), i=i):
                    if un[0] == 'b':
                        p = dot(both(un[1]), raw(un[1], un[2]))
                        hr = p.shape[0] // 2
                        acc.add((0, un[2]), 1, p[0:hr])
                        acc.add((1, un[2]), 1, p[hr:])
                    else:
                        r = un[2]
                        p = dot(lhs_of(un), raw(*list(r)[0]) if len(r) == 1 else sums(SUMS.index(r)))
                        for k, f in un[3]:
                            for half in range(2):
                                if f[half]:
                                    acc.add((half, k), f[half], p)
                    if last:
                        done(i)
                items.append((16 if un[0] == 'b' else 8, fn))
        return items

    def step(n, h):
        odd = n % 2 == 1
        hb = h.astype(BF16)
        qb = 24 * n
        kb = 40 * (n // 2) + (0 if odd else 16)
        nq, nk = (24, 40) if odd else (16, 24)
        clock = [0]
        d_s, d_o, gap, lag_v = PIPE[n]
        ready, s_at, o_at, ps = {}, {}, {}, {}

        def put(buf, r0, t, v):
            buf[r0:r0 + v.shape[0] // 2, _lanes(t)] = _as_u32(v.astype(BF16))

        def put64(m, t, top, bot):
            buf = (q_v, k_v, v_v)[m]
            if m == 0:
                put(buf, 0, t, top)
                put(buf, 24 + 16, t, bot[0:16])
                put(buf, 72 + 16, t, bot[16:32])
            else:
                put(buf, 16, t, top)
                put(buf, 32, t, bot[0:16])
                put(buf, 40 + 32, t, bot[16:32])
            ready[m, t] = clock[0]

        def plain(m, t):
            r = dot(hb, _as_bf16(wqkv_v[m * H + t]))
            if n == 0:
                put64(m, t, r[0:32], r[32:64])
            else:
                put((q_v, k_v, v_v)[m], qb if m == 0 else kb, t, r)
                ready[m, t] = clock[0]

        work = []
        if n == 0:
            cols = lambda i: slice(i * 128, (i + 1) * 128)
            make = _lhs_operands([h[0:32, cols(i)] for i in range(GH)], [h[32:64, cols(i)] for i in range(GH)])
            ops = {id(un): make(un) for row in UNITS for un in row if un[0] == 'p'}
            for g in range(NGRP):
                for m in ORDER0:
                    if g == NGRP - 1 and m == 2:
                        work += [(80, functools.partial(plain, mm, t))
                                 for t in range(NGRP * GH, H) for mm in (1, 0)]
                    acc = _Acc()
                    work += fast_units(
                        lambda un: ops[id(un)], lambda i: hb[:, cols(i)],
                        lambda i, j, m=m, g=g: _as_bf16(wqkv_v[m * H + g * GH + j, 64 * i:64 * i + 64, :]),
                        lambda q, m=m, g=g: _as_bf16(wc_v[m * NGRP + g, :, q * 128:(q + 1) * 128]),
                        acc, lambda j, m=m, g=g, acc=acc: put64(m, g * GH + j, acc.pop((0, j)), acc.pop((1, j))))
            work += [(80, functools.partial(plain, 2, t)) for t in range(NGRP * GH, H)]
        else:
            for t in range(H + lag_v):
                for m, tt in ((1, t), (2, t - lag_v), (0, t)):
                    if 0 <= tt < H:
                        work.append((40, functools.partial(plain, m, tt)))
        work = [(c, fn, -1) for c, fn in work]

        res = []
        if n == 3:
            acc = _Acc()

            def head():
                part = dot(_as_bf16(o_v[:, 0:WOFF * DH]), _as_bf16(wo_v[0:WOFF * DH // 2, :]))
                for hf in range(2):
                    for j in range(GH):
                        acc.add((hf, j), 1, part[32 * hf:32 * hf + 32, j * 128:(j + 1) * 128])

            work.append((80 * WOFF, head, WOFF - 1))
            for g in range(NGRP):
                h0 = WOFF + g * GH
                hc = lambda i, h0=h0: slice((h0 + i) * DH, (h0 + i + 1) * DH)
                box = []

                def lhs_of(un, box=box, hc=hc):
                    if not box:
                        box.append(_lhs_operands([up(o_v[0:16, hc(i)]) for i in range(GH)],
                                                 [up(o_v[16:32, hc(i)]) for i in range(GH)]))
                    return box[0](un)

                items = fast_units(
                    lhs_of, lambda i, hc=hc: _as_bf16(o_v[:, hc(i)]),
                    lambda i, j, h0=h0: _as_bf16(wo_v[(h0 + i) * 64:(h0 + i + 1) * 64, j * 128:(j + 1) * 128]),
                    lambda q, g=g: _as_bf16(woc_v[g, :, q * 128:(q + 1) * 128]), acc, lambda j: None)
                work += [(c, fn, h0 + GH - 1) for c, fn in items]
            work.append((0, lambda: res.append(jnp.concatenate(
                [jnp.concatenate([acc.pop((hf, j)) for j in range(GH)], axis=1) for hf in range(2)],
                axis=0)), H - 1))
        else:
            def wgroup(g):
                c0, c1 = g * WG * DH, (g + 1) * WG * DH
                part = dot(_as_bf16(o_v[0:16, c0:c1]), _as_bf16(wo_v[c0 // 2:c1 // 2, :]))
                res[:] = [part + res[0]] if res else [part]

            work += [(40 * WG, functools.partial(wgroup, g), (g + 1) * WG - 1) for g in range(H // WG)]

        def scores(t):
            sc = jax.lax.dot_general(_as_bf16(q_v[qb:qb + nq, _lanes(t)]),
                                     _as_bf16(k_v[kb:kb + nk, _lanes(t)]), NT,
                                     preferred_element_type=F32) * SCALE
            cap = cap_v[n, 0:sc.shape[0], 0:sc.shape[1]]
            sc = jnp.where(cap == 0.0, sc, cap)
            e = jnp.exp(sc - jnp.max(sc, axis=-1, keepdims=True))
            l = jnp.sum(e, axis=-1, keepdims=True)
            inv = pl.reciprocal(l, approx=True)
            inv = inv * (2.0 - l * inv)
            ps[t] = (e * inv).astype(BF16)
            s_at[t] = clock[0]
            clock[0] += nq // 2

        def values(t):
            o = dot(ps.pop(t), _as_bf16(v_v[kb:kb + nk, _lanes(t)]))
            if n == 1:
                put(o_v, 0, t, o[0:32])
                put(o_v, 24, t, o[32:48])
            else:
                put(o_v, 0, t, o)
            o_at[t] = clock[0]
            clock[0] += nq // 2

        def drain(upto):
            while True:
                to, ts = len(o_at), len(s_at)
                if to < ts and (2, to) in ready and (
                        to <= upto or clock[0] >= max(s_at[to] + d_o, ready[2, to] + d_s)):
                    values(to)
                elif ts < H and (0, ts) in ready and (1, ts) in ready and (
                        ts <= upto or clock[0] >= max(ready[0, ts] + d_s, ready[1, ts] + d_s,
                                                      s_at.get(ts - 1, -gap) + gap)):
                    scores(ts)
                else:
                    return

        for c, fn, need in work:
            drain(need)
            clock[0] += c
            fn()
        return res[0]

    def gate_work():
        acc = _Acc()
        cols = lambda i: slice(i * 128, (i + 1) * 128)
        box = []

        def lhs_of(un):
            if not box:
                box.append(_lhs_operands([up(u_v[0:32, cols(i)]) for i in range(GH)],
                                         [up(u_v[32:64, cols(i)]) for i in range(GH)]))
            return box[0](un)

        items = [(2 * c, fn) for c, fn in fast_units(
            lhs_of, lambda i: _as_bf16(u_v[:, cols(i)]),
            lambda i, j: _as_bf16(wout_v[64 * i:64 * i + 64, cols(j)]),
            lambda q: _as_bf16(woutc_v[:, cols(q)]), acc, lambda j: None)]

        def rest(j):
            p = dot(_as_bf16(u_v[:, DM:FH]), _as_bf16(wout_v[DM // 2:FH // 2, cols(j)]))
            acc.add((0, j), 1, p[0:64])
            acc.add((1, j), 1, p[64:128])

        items = [(64, functools.partial(rest, j)) for j in range(GH)] + items

        def chunk(budget):
            box.clear()
            while items and budget > 0:
                c, fn = items.pop(0)
                fn()
                budget -= c

        def result():
            hb = 0.5 * jnp.concatenate(
                [jnp.concatenate([acc.pop((hf, j)) for j in range(GH)], axis=1) for hf in range(2)], axis=0)
            return hb + hb * jnp.tanh(hb)

        return chunk, result

    def tile_body(j, mem):
        r0 = pl.multiple_of(j * 128, 128)
        xs = _as_bf16(xn_v[pl.ds(pl.multiple_of(j * 64, 64), 64), :]).astype(F32)
        chunk, gate_result = gate_work()
        chunk(FILL[0])
        a0 = step(0, jnp.concatenate([mem, xs[0:40], xs[64:72], xs[96:104]], axis=0))
        chunk(FILL[1])
        a1 = step(1, jnp.concatenate([a0[0:MEM], xs[40:64]], axis=0))
        chunk(FILL[2])
        a2 = step(2, jnp.concatenate([a1[0:MEM], xs[72:96]], axis=0))
        chunk(10 ** 6)
        gate = gate_result()
        u_transpose(jnp.minimum(j + 1, NTILE - 1))
        a3 = step(3, jnp.concatenate([a2[0:MEM], xs[104:128]], axis=0))
        s_rows = jnp.concatenate([a0[8:32], a3[48:64], a1[8:32], a3[32:40], a2[8:32], a3[40:48], a3[8:32]],
                                 axis=0)
        res = x_v[pl.ds(r0, 128), :].astype(F32) + s_rows * gate
        out_v[pl.ds(r0, 128), :] = res.astype(BF16)
        pltpu.make_async_copy(out_v.at[pl.ds(r0, 128), :],
                              out_hbm.at[pl.ds(r0, 128), :], sem_out).start()
        return a3[0:MEM]

    jax.lax.fori_loop(0, NTILE, tile_body, mem0_v[...].astype(F32))
    pltpu.make_async_copy(out_v, out_hbm, sem_out).wait()


@jax.jit
def pallas_recurrent_scan__memory_aug_recurrent_mem_tr__mixer_gmlp__prompt_kernel(
    A_x: jax.Array,
    A_mem0: jax.Array,
    A_Wq: jax.Array,
    A_Wk: jax.Array,
    A_Wv: jax.Array,
    A_Wo: jax.Array,
    A_seg_len: jax.Array,
    B_x: jax.Array,
    B_w_in: jax.Array,
    B_w_sp: jax.Array,
    B_b_sp: jax.Array,
    B_w_out: jax.Array,
):
    del A_seg_len, B_x
    hbm = pl.BlockSpec(memory_space=pl.ANY)
    out = pl.pallas_call(
        _kernel,
        out_shape=jax.ShapeDtypeStruct((S, DM), BF16),
        in_specs=[hbm] * 10,
        out_specs=hbm,
        scratch_shapes=[
            pltpu.VMEM((S, DM), BF16),
            pltpu.VMEM((S // 2, DM), U32),
            pltpu.VMEM((64, 2048), U32),
            pltpu.VMEM((64, 2048), U32),
            pltpu.VMEM((MEM, DM), BF16),
            pltpu.VMEM((16, 128), BF16),
            pltpu.VMEM((16, 128), F32),
            pltpu.VMEM((8, 128), U32),
            pltpu.VMEM((FH, DM), U32),
            pltpu.VMEM((FH // 2, 1280), U32),
            pltpu.VMEM((S // 2, S), U32),
            pltpu.VMEM((FH // 2, DM), U32),
            pltpu.VMEM((64, NSUM * 128), U32),
            pltpu.VMEM((48, DM + 8, DH), U32),
            pltpu.VMEM((3 * H, DM // 2, DH), U32),
            pltpu.VMEM((3 * NGRP, 64, NSUM * 128), U32),
            pltpu.VMEM((H * DH // 2, DM), U32),
            pltpu.VMEM((NGRP, 64, NSUM * 128), U32),
            pltpu.VMEM((T1, FH, 128), F32),
            pltpu.VMEM((T1, 2 * (FH // RB) * 8, 128), F32),
            pltpu.VMEM((FH // 2, S), U32),
            pltpu.VMEM((NTILE // 2, FH // 4, 7 * 128), U32),
            pltpu.VMEM((64, 5 * S // 2), U32),
            pltpu.VMEM((64, FH), U32),
            pltpu.VMEM((96, H * DH), U32),
            pltpu.VMEM((80, H * DH), U32),
            pltpu.VMEM((80, H * DH), U32),
            pltpu.VMEM((32, H * DH), U32),
            pltpu.VMEM((4, 48, 80), F32),
            pltpu.VMEM((S, DM), BF16),
            pltpu.SemaphoreType.DMA((4,)),
            pltpu.SemaphoreType.DMA((8,)),
            pltpu.SemaphoreType.DMA((NTILE // T2,)),
            pltpu.SemaphoreType.DMA((NTILE // T2,)),
            pltpu.SemaphoreType.DMA,
        ],
        compiler_params=pltpu.CompilerParams(vmem_limit_bytes=112 * 1024 * 1024),
    )(
        A_x.reshape(S, DM),
        A_mem0.reshape(MEM, DM),
        A_Wq, A_Wk, A_Wv,
        A_Wo.reshape(H * DH, DM),
        B_w_in.T,
        B_w_sp,
        B_b_sp.reshape(16, 128),
        B_w_out,
    )
    return out.reshape(1, S, DM)
```

```python
import functools

import jax
import jax.numpy as jnp
import jax.experimental.pallas as pl
import jax.experimental.pallas.tpu as pltpu

F32 = jnp.float32
BF16 = jnp.bfloat16
U32 = jnp.uint32

S = 2048
DM = 640
H = 32
DH = 128
MEM = 8
SEG = 32
FH = 864
NTILE = S // 128
EPS = 1e-5
SCALE = DH ** (-0.5)
NEG = -1000000000.0

XCH = 256
T1 = 4
T2 = 4
RB = 144
WIN_PIECES = (2, 4, 6)
SBLK = (144, 144, 144)
SIDE_TAIL = 1
WSP_HEAD = 512
LN_DEADLINE = 10
LN_FIRST = 4
NORM_TAIL = 4
ORDER0 = (1, 0, 2)
PIPE = ((270, 450, 170, 0), (230, 540, 128, 1), (210, 600, 100, 0), (230, 470, 112, 4))
WG = 4
FILL = (320, 224, 224)

NT = (((1,), (1,)), ((), ()))


def _as_bf16(u):
    return pltpu.bitcast(u, BF16)


def _as_u32(b):
    return pltpu.bitcast(b, U32)


def _layernorm(v):
    m = jnp.mean(v, axis=-1, keepdims=True)
    c = v - m
    var = jnp.mean(c * c, axis=-1, keepdims=True)
    return c * jax.lax.rsqrt(var + EPS)


def _gelu2(v):
    c = 0.7978845608028654
    return v + v * jnp.tanh(v * (c + (c * 0.044715) * (v * v)))


def _mult(v, m):
    return v if isinstance(v, int) else pl.multiple_of(v, m)


def _lanes(tile):
    return pl.ds(_mult(tile * 128, 128), 128)


def _mask(qgroups, kgroups):
    shape = (8 * len(qgroups), 8 * len(kgroups))

    def table(groups, axis):
        idx = jax.lax.broadcasted_iota(jnp.int32, shape, axis)
        seg = jnp.full(shape, groups[-1][0], jnp.int32)
        pos = idx + (groups[-1][1] - 8 * (len(groups) - 1))
        for g in range(len(groups) - 2, -1, -1):
            inside = idx < 8 * (g + 1)
            seg = jnp.where(inside, groups[g][0], seg)
            pos = jnp.where(inside, idx + (groups[g][1] - 8 * g), pos)
        return seg, pos

    qseg, qpos = table(qgroups, 0)
    kseg, kpos = table(kgroups, 1)
    same = qseg == kseg
    keep = same & ((qpos < MEM) | (qpos >= kpos))
    return keep, jnp.where(same, NEG, -jnp.inf).astype(F32)


def _masks():
    own = lambda sg: [(sg, 0), (sg, 16), (sg, 24), (sg, 32)]
    k0 = [(0, 0), (0, 8), (0, 16), (0, 24), (0, 32), (1, 8)]
    k2 = own(2) + [(2, 8), (3, 8)]
    return [
        _mask(k0[:4], k0),
        _mask(own(1) + k0[4:], own(1) + k0),
        _mask(own(2), k2),
        _mask(own(3) + k2[4:], own(3) + k2),
    ]


def _fast_table(types):
    lines = {0: ((1, 0), (1, -1)), 1: ((0, 1), (1, -1)), 2: ((1, 0), (0, 1))}
    neg = lambda f: (-f[0], -f[1])

    def dual(u, v):
        det = u[0] * v[1] - u[1] * v[0]
        return (v[1] * det, -v[0] * det), (-u[1] * det, u[0] * det)

    n = len(types)
    diag = {(i, k): {(i, i): 1} for i in range(n) for k in range(2)}
    units = [[] for _ in range(n)]
    for i in range(n):
        u = lines[types[i]]
        units[i] += [('p', [(i, u[k])], diag[i, k], [(i, dual(*u)[k])]) for k in range(2)]
        for j in range(i + 1, n):
            if types[i] == types[j]:
                units[i] += [('b', i, j), ('b', j, i)]
                continue
            w = lines[types[j]]
            (ci, cj), = [(x, y) for x in range(2) for y in range(2) if u[x] == w[y]]
            (p, q), = [(x, y) for x in (u[1 - ci], neg(u[1 - ci])) for y in (w[1 - cj], neg(w[1 - cj]))
                       if (x[0] - y[0], x[1] - y[1]) == u[ci]]
            sd, td = dual(p, q)
            units[i] += [('p', [(i, p), (j, q)], {(i, j): 1, (j, i): 1}, [(i, td), (j, sd)]),
                         ('p', [(i, q), (j, q)], {(i, j): 1}, [(i, neg(td)), (j, td)]),
                         ('p', [(i, p), (j, p)], {(j, i): 1}, [(i, sd), (j, neg(sd))])]
            diag[i, ci][i, j] = 1
            diag[i, 1 - ci][j, i] = -1
            diag[j, 1 - cj][i, j] = -1
            diag[j, cj][j, i] = 1
    out = []
    for i in range(n):
        row = []
        for un in units[i]:
            if un[0] == 'p' and [c for c in un[1][0][1] if c][0] < 0:
                un = ('p', [(k, neg(f)) for k, f in un[1]], un[2], [(k, neg(f)) for k, f in un[3]])
            row.append(un)
        out.append(row)
    return out


GH = 5
NGRP = H // GH
WOFF = H - NGRP * GH
UNITS = _fast_table((0, 1, 2, 0, 1))
SUMS = [un[2] for row in UNITS for un in row if un[0] == 'p' and len(un[2]) > 1]
NSUM = len(SUMS)


def _signed_sum(terms):
    terms = sorted(terms, key=lambda cv: -cv[0])
    acc = terms[0][1]
    for c, v in terms[1:]:
        acc = acc + v if c > 0 else acc - v
    return acc


def _lhs_operands(top, bot):
    forms = {}

    def form(i, f):
        sign = 1 if [c for c in f if c][0] > 0 else -1
        key = (i, (sign * f[0], sign * f[1]))
        if key not in forms:
            forms[key] = {(1, 0): lambda: top[i], (0, 1): lambda: bot[i],
                          (1, -1): lambda: top[i] - bot[i]}[key[1]]()
        return sign, forms[key]

    return lambda un: _signed_sum([form(i, f) for i, f in un[1]]).astype(BF16)


class _Acc:
    def __init__(self):
        self.v = {}

    def add(self, key, c, p):
        if key not in self.v:
            self.v[key] = (c, p)
        else:
            sign, v = self.v[key]
            self.v[key] = (sign, v + p if sign == c else v - p)

    def pop(self, key):
        sign, v = self.v.pop(key)
        return v if sign > 0 else -v


def _kernel(x_hbm, mem0_hbm, wq_hbm, wk_hbm, wv_hbm, wo_hbm, wint_hbm, wsp_hbm,
            bsp_hbm, wout_hbm, out_hbm,
            x_v, xn_v, xa_v, xb_v, mem0_v, bsp_v, bsp32_v, zero_v, wint_v, wins_v, wsp_v, wout_v, woutc_v,
            stage_v, wqkv_v, wc_v, wo_v, woc_v, zg_v, st_v, z1t_v, za_v, ts_v, u_v, q_v, k_v, v_v, o_v, cap_v, out_v,
            sem_x, sem_w, sem_st, sem_wo, sem_out):
    NRB = FH // RB
    NG = RB // 8
    NB2 = NTILE // T2
    PPB = 48 // NB2

    x_parts = [(0, XCH), (XCH, XCH), (2 * XCH, XCH), (3 * XCH, S - 3 * XCH)]
    x_cps = [pltpu.make_async_copy(x_hbm.at[pl.ds(o, n), :], x_v.at[pl.ds(o, n), :], sem_x.at[k])
             for k, (o, n) in enumerate(x_parts)]
    wint_u = wint_hbm.bitcast(U32)
    blk_row = lambda k: (FH + k * RB) if k < NRB else (k - NRB) * RB
    wint_cps, k0 = [], 0
    for k, nb in enumerate(WIN_PIECES):
        o, n = blk_row(k0) // 2, nb * RB // 2
        wint_cps.append(pltpu.make_async_copy(wint_u.at[pl.ds(o, n), :], wint_v.at[pl.ds(o, n), :],
                                              sem_w.at[k]))
        k0 += nb
    wsp_u = wsp_hbm.bitcast(U32)
    wsp_cp = pltpu.make_async_copy(wsp_u.at[pl.ds(0, WSP_HEAD), :], wsp_v.at[pl.ds(0, WSP_HEAD), :],
                                   sem_w.at[3])
    wsp_cp2 = pltpu.make_async_copy(wsp_u.at[pl.ds(WSP_HEAD, S // 2 - WSP_HEAD), :],
                                    wsp_v.at[pl.ds(WSP_HEAD, S // 2 - WSP_HEAD), :], sem_w.at[7])
    wout_cp = pltpu.make_async_copy(wout_hbm.bitcast(U32), wout_v, sem_w.at[4])
    WOQ = H * DH // 2 // NB2

    def wo_copy(i):
        r0 = _mult(i * WOQ, WOQ)
        return pltpu.make_async_copy(wo_hbm.bitcast(U32).at[pl.ds(r0, WOQ), :],
                                     wo_v.at[pl.ds(r0, WOQ), :], sem_wo.at[i])

    mem0_cp = pltpu.make_async_copy(mem0_hbm, mem0_v, sem_w.at[5])
    bsp_cp = pltpu.make_async_copy(bsp_hbm, bsp_v, sem_w.at[6])
    w_hbms = (wq_hbm, wk_hbm, wv_hbm)

    def stage_copy(m, j):
        p = m * 16 + j
        return pltpu.make_async_copy(w_hbms[m].bitcast(U32).at[:, j, :],
                                     stage_v.at[p, pl.ds(0, DM), :], sem_st.at[p // PPB])

    x_cps[0].start()
    x_cps[1].start()
    for cp in wint_cps:
        cp.start()
    x_cps[2].start()
    x_cps[3].start()
    bsp_cp.start()
    mem0_cp.start()
    wsp_cp.start()
    wout_cp.start()
    for p in range(48):
        stage_copy(p // 16, p % 16).start()
        if (p + 1) % PPB == 0:
            wo_copy(p // PPB).start()
        if p + 1 == 2 * PPB:
            wsp_cp2.start()

    zero_v[...] = jnp.zeros((8, 128), U32)
    for n, (keep, fill) in enumerate(_masks()):
        cap_v[n, 0:keep.shape[0], 0:keep.shape[1]] = jnp.where(keep, 0.0, fill)

    pending = []

    def dep_of(v):
        return pltpu.bitcast(v[0:8, 0:128], U32) & zero_v[...]

    def up(u):
        return _as_bf16(u).astype(F32)

    def ln_rows(r0, n, dep=None):
        xr = x_v[pl.ds(r0, n), :].astype(F32)
        if dep is not None:
            d = jnp.concatenate([dep] * (n // 8), axis=0)
            xr = pltpu.bitcast(pltpu.bitcast(xr, U32) | jnp.concatenate([d] * (DM // 128), axis=1), F32)
        xn = _layernorm(xr)
        xn_v[pl.ds(_mult(r0 // 2, n // 2), n // 2), :] = _as_u32(xn.astype(BF16))
        return xn

    def ln_pair(base, k, dst, dep):
        xe = ln_rows(_mult(base + 16 * k, 16), 16, dep)
        xo = ln_rows(_mult(base + 128 + 16 * k, 16), 16, dep)
        b11, b21, b12, b22 = xe[:, 0:256], xe[:, 256:512], xo[:, 0:256], xo[:, 256:512]
        ops = jnp.concatenate([b11 + b22, b11, b12 - b22, b21 - b11, b22,
                               b11 + b12, xo[:, 512:], b21 + b22, xe[:, 512:]], axis=1)
        dst[8 * k:8 * k + 8, :] = _as_u32(ops.astype(BF16))
        pending.append([LN_DEADLINE, dst[8 * k:8 * k + 8, 0:128] & zero_v[...]])

    def win_sums(hz, k, dep):
        d = jnp.concatenate([dep] * 4, axis=1)
        r0 = hz * (FH // 2) + 8 * k
        top, bot = up(wint_v[r0:r0 + 8, 0:512] | d), up(wint_v[r0 + FH // 4:r0 + FH // 4 + 8, 0:512] | d)
        a11, a12, a21, a22 = top[:, 0:256], top[:, 256:512], bot[:, 0:256], bot[:, 256:512]
        ops = jnp.concatenate([a11 + a22, a21 + a22, a11 + a12, a21 - a11, a12 - a22], axis=1)
        wins_v[hz * (FH // 4) + 8 * k:hz * (FH // 4) + 8 * k + 8, :] = _as_u32(ops.astype(BF16))

    def nt_dot(w, xt):
        due = None
        for e in pending:
            e[0] -= 1
            if e[0] == 0:
                due = e[1] if due is None else due | e[1]
        pending[:] = [e for e in pending if e[0] > 0]
        if due is not None:
            top = w[0:8, 0:128] | due
            if w.shape[1] > 128:
                top = jnp.concatenate([top, w[0:8, 128:]], axis=1)
            w = jnp.concatenate([top, w[8:]], axis=0)
        return jax.lax.dot_general(_as_bf16(w), _as_bf16(xt), NT, preferred_element_type=F32)

    def win_block(nt, f0):
        return nt_dot(wint_v[f0 // 2:(f0 + RB) // 2, :], xn_v[nt * 64:(nt + 1) * 64, :])

    def win_group(src, hz, rb, emit, side):
        rt = (hz * FH + rb * RB) // 2
        rows = lambda r: slice(r, r + RB // 2)
        top, bot, sm = rows(rt), rows(rt + FH // 4), rows(hz * (FH // 4) + rb * RB // 2)
        ss = lambda q: wins_v[sm, q * 256:(q + 1) * 256]
        tt = lambda q: src[:, q * 256:(q + 1) * 256]
        rest = lambda r: wint_v[r, 512:640]

        def prod(w, xt):
            p = nt_dot(w, xt)
            side(p)
            return p

        m2 = prod(ss(1), tt(1))
        m4 = prod(wint_v[bot, 256:512], tt(3))
        emit(0, rb + NRB // 2, m2 + m4 + prod(rest(bot), src[:, 1920:2048]))
        m3 = prod(wint_v[top, 0:256], tt(2))
        m5 = prod(ss(2), tt(4))
        emit(1, rb, m3 + m5 + prod(rest(top), src[:, 1536:1664]))
        c11, c22 = m4 - m5, m3 - m2
        m1 = prod(ss(0), tt(0))
        emit(0, rb, c11 + m1 + prod(jnp.concatenate([ss(4), rest(top)], axis=1), src[:, 1664:2048]))
        emit(1, rb + NRB // 2,
             c22 + m1 + prod(jnp.concatenate([ss(3), rest(bot)], axis=1), src[:, 1280:1664]))

    def z2_emit(nt, rb, z):
        g = _gelu2(z)
        zg_v[nt, rb * RB:(rb + 1) * RB, :] = g
        g3 = g.reshape(NG, 8, 128)
        bm = jnp.sum(g3, axis=0) * (1.0 / NG)
        c = g3 - bm
        st_v[nt, rb * 8:(rb + 1) * 8, :] = bm
        st_v[nt, (NRB + rb) * 8:(NRB + rb + 1) * 8, :] = jnp.sum(c * c, axis=0)

    def z2_stats(nt):
        bm = st_v[nt, 0:NRB * 8, :]
        m = jnp.sum(bm, axis=0, keepdims=True) * (1.0 / (NRB * 8))
        dm = bm - m
        m2 = jnp.sum(st_v[nt, NRB * 8:2 * NRB * 8, :] + dm * dm * NG, axis=0, keepdims=True)
        r = jax.lax.rsqrt(m2 * (1.0 / FH) + 4.0 * EPS)
        return jnp.broadcast_to(m, (8, 128)), jnp.broadcast_to(r, (8, 128))

    def z2_norm(ne, tp, k, st, dep):
        (me, re), (mo, ro) = st
        me = pltpu.bitcast(pltpu.bitcast(me, U32) | dep, F32)
        mo = pltpu.bitcast(pltpu.bitcast(mo, U32) | dep, F32)
        nrm = lambda nt, f0, m, r: ((zg_v[nt, f0:f0 + 16, :].reshape(2, 8, 128) - m) * r).reshape(16, 128)
        a11, a21 = nrm(ne, 16 * k, me, re), nrm(ne, FH // 2 + 16 * k, me, re)
        a12, a22 = nrm(ne + 1, 16 * k, mo, ro), nrm(ne + 1, FH // 2 + 16 * k, mo, ro)
        ops = jnp.concatenate([a11 + a22, a21 + a22, a11, a22, a11 + a12, a21 - a11, a12 - a22], axis=1)
        za_v.at[tp][8 * k:8 * k + 8, :] = _as_u32(ops.astype(BF16))

    def z1_emit(tile, rb, z):
        z1t_v[rb * RB // 2:(rb + 1) * RB // 2, _lanes(tile)] = _as_u32(_gelu2(z).astype(BF16))

    def spread(tasks, slots):
        state = [0]

        def side(p):
            n = state[0]
            mine = tasks[n * len(tasks) // slots:(n + 1) * len(tasks) // slots]
            for q, fn in enumerate(mine):
                fn(dep_of(p[8 * ((q * NG) // len(mine)):]))
            state[0] += 1

        return side

    def mix(*kinds):
        order = sorted(((q + 0.5) / len(kd), kn, q) for kn, kd in enumerate(kinds) for q in range(len(kd)))
        return [kinds[kn][q] for _, kn, q in order]

    part = functools.partial
    NSLAB = FH // 32

    x_cps[0].wait()
    ln_rows(0, XCH)
    x_cps[1].wait()
    ln_rows(XCH, XCH)
    wint_cps[0].wait()
    for nt in range(T1):
        for rb in range(WIN_PIECES[0]):
            z2_emit(nt, rb, win_block(nt, FH + rb * RB))
    wint_cps[1].wait()
    side = spread([part(win_sums, 1, k) for k in range(NSLAB)], T1 * (NRB - WIN_PIECES[0]) - 1)
    for nt in range(T1):
        for rb in range(WIN_PIECES[0], NRB):
            z = win_block(nt, FH + rb * RB)
            z2_emit(nt, rb, z)
            side(z)
    wint_cps[2].wait()
    x_cps[2].wait()
    norms = []
    for ne in range(0, T1, 2):
        st = (z2_stats(ne), z2_stats(ne + 1))
        norms += [part(z2_norm, ne, ne // 2, k, st) for k in range(NSLAB)]
    side = spread(mix(norms, [part(win_sums, 0, k) for k in range(NSLAB)],
                      [part(ln_pair, T1 * 128, k, xa_v) for k in range(8)]), T1 * NRB - 1)
    for nt in range(T1):
        for rb in range(NRB):
            z = win_block(nt, rb * RB)
            z1_emit(nt, rb, z)
            side(z)
    x_cps[3].wait()
    pending.clear()

    def b1_body(i, carry):
        for ne in range(0, T1, 2):
            tile = i * T1 + ne
            src, dst = (xa_v, xb_v) if ne == 0 else (xb_v, xa_v)
            base = jnp.minimum(tile + 2, NTILE - 2) * 128
            lns = [part(ln_pair, base, k, dst) for k in range(8)]
            side = spread(lns[:LN_FIRST], 9 * NRB // 2)
            for rb in range(NRB // 2):
                win_group(src, 1, rb, lambda o, r, z: z2_emit(ne + o, r, z), side)
            st = (z2_stats(ne), z2_stats(ne + 1))
            norms = [part(z2_norm, ne, tile // 2, k, st) for k in range(NSLAB)]
            side = spread(mix(norms, lns[LN_FIRST:]) if LN_FIRST < 8 else norms, 9 * NRB // 2 - NORM_TAIL)
            for rb in range(NRB // 2):
                win_group(src, 0, rb, lambda o, r, z: z1_emit(tile + o, r, z), side)
        pending.clear()
        return carry

    jax.lax.fori_loop(1, NTILE // T1, b1_body, 0)

    wsp_cp.wait()
    wout_cp.wait()
    bsp_cp.wait()
    mem0_cp.wait()
    bsp32_v[...] = 0.5 * bsp_v[...].astype(F32)

    def split_block(p, bi, dep):
        a = stage_v[p, pl.ds(128 * bi, 64, stride=2), :] | dep
        b = stage_v[p, pl.ds(128 * bi + 1, 64, stride=2), :] | dep
        wqkv_v[2 * p, 64 * bi:64 * bi + 64, :] = (a & jnp.uint32(0xFFFF)) | (b << 16)
        wqkv_v[2 * p + 1, 64 * bi:64 * bi + 64, :] = (a >> 16) | (b & jnp.uint32(0xFFFF0000))

    def weight_sums(block, dst, rows, idx, dep):
        cache = {}

        def blk(ij):
            if ij not in cache:
                w = block(*ij)
                cache[ij] = up(w | dep[0:w.shape[0]])
            return cache[ij]

        mine = [un[2] for un in UNITS[idx] if un[0] == 'p' and len(un[2]) > 1]
        c0 = SUMS.index(mine[0])
        sums = jnp.concatenate([_signed_sum([(c, blk(ij)) for ij, c in r.items()]) for r in mine], axis=1)
        dst[rows, c0 * 128:(c0 + len(mine)) * 128] = _as_u32(sums.astype(BF16))

    fblocks = [(f0, min(128, FH - f0)) for f0 in range(0, FH, 128)]

    def u_transpose(tile):
        for f0, fn in fblocks:
            ut = _as_bf16(z1t_v[f0 // 2:(f0 + fn) // 2, _lanes(tile)]).astype(F32)
            u_v[:, f0:f0 + fn] = _as_u32(ut.T.astype(BF16))

    NK = NTILE // 2

    def t_piece(tp, k, dep):
        h0 = _mult(tp * 128, 128)
        we = wsp_v[pl.ds(h0, 64), k * 256:(k + 1) * 256]
        wo = wsp_v[pl.ds(h0 + 64, 64), k * 256:(k + 1) * 256]
        d = jnp.concatenate([dep, dep], axis=1)
        we, wo = up(we | d), up(wo | d)
        b11, b21, b12, b22 = we[:, 0:128], we[:, 128:256], wo[:, 0:128], wo[:, 128:256]
        ops = jnp.concatenate([b11 + b22, b12 - b22, b21 - b11, b11 + b12, b21 + b22], axis=1)
        z0 = pl.multiple_of(jnp.minimum(tp, 0) * 64, 64)
        ts_v[pl.ds(z0, 64), k * 640:(k + 1) * 640] = _as_u32(ops.astype(BF16))

    def b2_body(i, carry):
        group = stage_v.at[pl.ds(i * PPB, PPB), pl.ds(0, DM), :]
        pltpu.make_async_copy(group, group, sem_st.at[i]).wait()
        wo_copy(i).wait()

        @pl.when(i == 2)
        def _():
            wsp_cp2.wait()

        u_transpose(0)
        for lp in range(2):
            tp = i * 2 + lp
            he = pl.multiple_of(tp * 128, 128)
            raw = lambda odd_t, odd_s: lambda k: wsp_v[
                pl.ds(he + odd_t * 64, 64), (2 * k + odd_s) * 128:(2 * k + odd_s + 1) * 128]
            tj = lambda j: lambda k: ts_v[:, k * 640 + j * 128:k * 640 + (j + 1) * 128]
            rhs = [tj(0), raw(0, 0), tj(1), tj(2), raw(1, 1), tj(3), tj(4)]

            full = slice(0, 64)
            kinds = [[]]
            if lp == 0:
                kinds[0] = [(9, part(split_block, i * PPB + pp, bi)) for pp in range(PPB) for bi in range(GH)]
                kinds.append([])
                for sl in range(2):
                    gid = jnp.maximum(i, 2 * i - 2 + sl)
                    block = lambda bi, bj, gid=gid: wo_v[
                        pl.ds(pl.multiple_of((WOFF + gid * GH + bi) * 64, 64), 64), bj * 128:(bj + 1) * 128]
                    kinds[1] += [(30, part(weight_sums, block, woc_v.at[gid], full, idx)) for idx in range(GH)]
            else:
                for sl in range(5):
                    gid = jnp.minimum((9 * i) // 2 + sl, (9 * i + 9) // 2 - 1)
                    f0h = (gid // NGRP) * H + (gid % NGRP) * GH
                    block = lambda bi, bj, f0h=f0h: wqkv_v[f0h + bj, 64 * bi:64 * bi + 64, :]
                    kinds[0] += [(30, part(weight_sums, block, wc_v.at[gid], full, idx)) for idx in range(GH)]
            r8 = pl.multiple_of(8 * (2 * i + lp), 8)
            block = lambda bi, bj, r8=r8: wout_v[pl.ds(64 * bi + r8, 8), bj * 128:(bj + 1) * 128]
            kinds.append([(4, part(weight_sums, block, woutc_v, pl.ds(r8, 8), idx)) for idx in range(GH)])
            tasks = [(28, part(t_piece, tp, k)) for k in range(NK)] + mix(*kinds)
            budget = sum(c for c, _ in tasks) / (2 * 7 * len(SBLK) - SIDE_TAIL)
            state = [0.0]

            def side(p):
                state[0] += budget
                phase = 0
                while tasks and state[0] > 0:
                    c, fn = tasks.pop(0)
                    rows = p[0:128].reshape(8, 16, 128)[:, 8 * phase:8 * phase + 8, :]
                    fn((pltpu.bitcast(rows, U32) & zero_v[...]).reshape(64, 128))
                    state[0] -= c
                    phase = 1 - phase

            def prod(j, f0, fn):
                p = None
                for ks in (range(NK // 2), range(NK // 2, NK)):
                    lhs = jnp.concatenate(
                        [za_v[k, f0 // 2:(f0 + fn) // 2, j * 128:(j + 1) * 128] for k in ks], axis=1)
                    r = jnp.concatenate([rhs[j](k) for k in ks], axis=1)
                    q = jax.lax.dot_general(_as_bf16(lhs), _as_bf16(r), NT, preferred_element_type=F32)
                    side(q)
                    p = q if p is None else p + q
                return p

            def finish(c, f0, fn, odd_t):
                tile = tp * 2 + odd_t
                z1 = _as_bf16(z1t_v[f0 // 2:(f0 + fn) // 2, _lanes(tile)]).astype(F32)
                brow = bsp32_v[pl.ds(tile, 1), :]
                z1t_v[f0 // 2:(f0 + fn) // 2, _lanes(tile)] = _as_u32((z1 * (0.5 * c + brow)).astype(BF16))

            blocks = [(sum(SBLK[:q]), fn) for q, fn in enumerate(SBLK)]
            early = [(prod(1, f0, fn), prod(4, f0, fn)) for f0, fn in blocks]
            assert all(fn.func is not t_piece for _, fn in tasks)
            for (f0, fn), (m2, m5) in zip(blocks, early):
                m4 = prod(3, f0, fn)
                finish(m2 + m4, FH // 2 + f0, fn, 0)
                m1 = prod(0, f0, fn)
                finish(m4 - m5 + m1 + prod(6, f0, fn), f0, fn, 0)
                m3 = prod(2, f0, fn)
                finish(m3 + m5, f0, fn, 1)
                finish(m3 - m2 + m1 + prod(5, f0, fn), FH // 2 + f0, fn, 1)
            assert not tasks
        return carry

    jax.lax.fori_loop(0, NB2, b2_body, 0)

    dot = lambda l, r: jnp.dot(l, r, preferred_element_type=F32)

    def fast_units(lhs_of, both, raw, sums, acc, done):
        items = []
        for i, row in enumerate(UNITS):
            for q, un in enumerate(row):
                def fn(un=un, last=(q == len(row) - 1), i=i):
                    if un[0] == 'b':
                        p = dot(both(un[1]), raw(un[1], un[2]))
                        hr = p.shape[0] // 2
                        acc.add((0, un[2]), 1, p[0:hr])
                        acc.add((1, un[2]), 1, p[hr:])
                    else:
                        r = un[2]
                        p = dot(lhs_of(un), raw(*list(r)[0]) if len(r) == 1 else sums(SUMS.index(r)))
                        for k, f in un[3]:
                            for half in range(2):
                                if f[half]:
                                    acc.add((half, k), f[half], p)
                    if last:
                        done(i)
                items.append((16 if un[0] == 'b' else 8, fn))
        return items

    def step(n, h):
        odd = n % 2 == 1
        hb = h.astype(BF16)
        qb = 24 * n
        kb = 40 * (n // 2) + (0 if odd else 16)
        nq, nk = (24, 40) if odd else (16, 24)
        clock = [0]
        d_s, d_o, gap, lag_v = PIPE[n]
        ready, s_at, o_at, ps = {}, {}, {}, {}

        def put(buf, r0, t, v):
            buf[r0:r0 + v.shape[0] // 2, _lanes(t)] = _as_u32(v.astype(BF16))

        def put64(m, t, top, bot):
            buf = (q_v, k_v, v_v)[m]
            if m == 0:
                put(buf, 0, t, top)
                put(buf, 24 + 16, t, bot[0:16])
                put(buf, 72 + 16, t, bot[16:32])
            else:
                put(buf, 16, t, top)
                put(buf, 32, t, bot[0:16])
                put(buf, 40 + 32, t, bot[16:32])
            ready[m, t] = clock[0]

        def plain(m, t):
            r = dot(hb, _as_bf16(wqkv_v[m * H + t]))
            if n == 0:
                put64(m, t, r[0:32], r[32:64])
            else:
                put((q_v, k_v, v_v)[m], qb if m == 0 else kb, t, r)
                ready[m, t] = clock[0]

        work = []
        if n == 0:
            cols = lambda i: slice(i * 128, (i + 1) * 128)
            make = _lhs_operands([h[0:32, cols(i)] for i in range(GH)], [h[32:64, cols(i)] for i in range(GH)])
            ops = {id(un): make(un) for row in UNITS for un in row if un[0] == 'p'}
            for g in range(NGRP):
                for m in ORDER0:
                    if g == NGRP - 1 and m == 2:
                        work += [(80, functools.partial(plain, mm, t))
                                 for t in range(NGRP * GH, H) for mm in (1, 0)]
                    acc = _Acc()
                    work += fast_units(
                        lambda un: ops[id(un)], lambda i: hb[:, cols(i)],
                        lambda i, j, m=m, g=g: _as_bf16(wqkv_v[m * H + g * GH + j, 64 * i:64 * i + 64, :]),
                        lambda q, m=m, g=g: _as_bf16(wc_v[m * NGRP + g, :, q * 128:(q + 1) * 128]),
                        acc, lambda j, m=m, g=g, acc=acc: put64(m, g * GH + j, acc.pop((0, j)), acc.pop((1, j))))
            work += [(80, functools.partial(plain, 2, t)) for t in range(NGRP * GH, H)]
        else:
            for t in range(H + lag_v):
                for m, tt in ((1, t), (2, t - lag_v), (0, t)):
                    if 0 <= tt < H:
                        work.append((40, functools.partial(plain, m, tt)))
        work = [(c, fn, -1) for c, fn in work]

        res = []
        if n == 3:
            acc = _Acc()

            def head():
                part = dot(_as_bf16(o_v[:, 0:WOFF * DH]), _as_bf16(wo_v[0:WOFF * DH // 2, :]))
                for hf in range(2):
                    for j in range(GH):
                        acc.add((hf, j), 1, part[32 * hf:32 * hf + 32, j * 128:(j + 1) * 128])

            work.append((80 * WOFF, head, WOFF - 1))
            for g in range(NGRP):
                h0 = WOFF + g * GH
                hc = lambda i, h0=h0: slice((h0 + i) * DH, (h0 + i + 1) * DH)
                box = []

                def lhs_of(un, box=box, hc=hc):
                    if not box:
                        box.append(_lhs_operands([up(o_v[0:16, hc(i)]) for i in range(GH)],
                                                 [up(o_v[16:32, hc(i)]) for i in range(GH)]))
                    return box[0](un)

                items = fast_units(
                    lhs_of, lambda i, hc=hc: _as_bf16(o_v[:, hc(i)]),
                    lambda i, j, h0=h0: _as_bf16(wo_v[(h0 + i) * 64:(h0 + i + 1) * 64, j * 128:(j + 1) * 128]),
                    lambda q, g=g: _as_bf16(woc_v[g, :, q * 128:(q + 1) * 128]), acc, lambda j: None)
                work += [(c, fn, h0 + GH - 1) for c, fn in items]
            work.append((0, lambda: res.append(jnp.concatenate(
                [jnp.concatenate([acc.pop((hf, j)) for j in range(GH)], axis=1) for hf in range(2)],
                axis=0)), H - 1))
        else:
            def wgroup(g):
                c0, c1 = g * WG * DH, (g + 1) * WG * DH
                part = dot(_as_bf16(o_v[0:16, c0:c1]), _as_bf16(wo_v[c0 // 2:c1 // 2, :]))
                res[:] = [part + res[0]] if res else [part]

            work += [(40 * WG, functools.partial(wgroup, g), (g + 1) * WG - 1) for g in range(H // WG)]

        def scores(t):
            sc = jax.lax.dot_general(_as_bf16(q_v[qb:qb + nq, _lanes(t)]),
                                     _as_bf16(k_v[kb:kb + nk, _lanes(t)]), NT,
                                     preferred_element_type=F32) * SCALE
            cap = cap_v[n, 0:sc.shape[0], 0:sc.shape[1]]
            sc = jnp.where(cap == 0.0, sc, cap)
            e = jnp.exp(sc - jnp.max(sc, axis=-1, keepdims=True))
            l = jnp.sum(e, axis=-1, keepdims=True)
            inv = pl.reciprocal(l, approx=True)
            inv = inv * (2.0 - l * inv)
            ps[t] = (e * inv).astype(BF16)
            s_at[t] = clock[0]
            clock[0] += nq // 2

        def values(t):
            o = dot(ps.pop(t), _as_bf16(v_v[kb:kb + nk, _lanes(t)]))
            if n == 1:
                put(o_v, 0, t, o[0:32])
                put(o_v, 24, t, o[32:48])
            else:
                put(o_v, 0, t, o)
            o_at[t] = clock[0]
            clock[0] += nq // 2

        def drain(upto):
            while True:
                to, ts = len(o_at), len(s_at)
                if to < ts and (2, to) in ready and (
                        to <= upto or clock[0] >= max(s_at[to] + d_o, ready[2, to] + d_s)):
                    values(to)
                elif ts < H and (0, ts) in ready and (1, ts) in ready and (
                        ts <= upto or clock[0] >= max(ready[0, ts] + d_s, ready[1, ts] + d_s,
                                                      s_at.get(ts - 1, -gap) + gap)):
                    scores(ts)
                else:
                    return

        for c, fn, need in work:
            drain(need)
            clock[0] += c
            fn()
        return res[0]

    def gate_work():
        acc = _Acc()
        cols = lambda i: slice(i * 128, (i + 1) * 128)
        box = []

        def lhs_of(un):
            if not box:
                box.append(_lhs_operands([up(u_v[0:32, cols(i)]) for i in range(GH)],
                                         [up(u_v[32:64, cols(i)]) for i in range(GH)]))
            return box[0](un)

        items = [(2 * c, fn) for c, fn in fast_units(
            lhs_of, lambda i: _as_bf16(u_v[:, cols(i)]),
            lambda i, j: _as_bf16(wout_v[64 * i:64 * i + 64, cols(j)]),
            lambda q: _as_bf16(woutc_v[:, cols(q)]), acc, lambda j: None)]

        def rest(j):
            p = dot(_as_bf16(u_v[:, DM:FH]), _as_bf16(wout_v[DM // 2:FH // 2, cols(j)]))
            acc.add((0, j), 1, p[0:64])
            acc.add((1, j), 1, p[64:128])

        items = [(64, functools.partial(rest, j)) for j in range(GH)] + items

        def chunk(budget):
            box.clear()
            while items and budget > 0:
                c, fn = items.pop(0)
                fn()
                budget -= c

        def result():
            hb = 0.5 * jnp.concatenate(
                [jnp.concatenate([acc.pop((hf, j)) for j in range(GH)], axis=1) for hf in range(2)], axis=0)
            return hb + hb * jnp.tanh(hb)

        return chunk, result

    def tile_body(j, mem):
        r0 = pl.multiple_of(j * 128, 128)
        xs = _as_bf16(xn_v[pl.ds(pl.multiple_of(j * 64, 64), 64), :]).astype(F32)
        chunk, gate_result = gate_work()
        chunk(FILL[0])
        a0 = step(0, jnp.concatenate([mem, xs[0:40], xs[64:72], xs[96:104]], axis=0))
        chunk(FILL[1])
        a1 = step(1, jnp.concatenate([a0[0:MEM], xs[40:64]], axis=0))
        chunk(FILL[2])
        a2 = step(2, jnp.concatenate([a1[0:MEM], xs[72:96]], axis=0))
        chunk(10 ** 6)
        gate = gate_result()
        u_transpose(jnp.minimum(j + 1, NTILE - 1))
        a3 = step(3, jnp.concatenate([a2[0:MEM], xs[104:128]], axis=0))
        s_rows = jnp.concatenate([a0[8:32], a3[48:64], a1[8:32], a3[32:40], a2[8:32], a3[40:48], a3[8:32]],
                                 axis=0)
        res = x_v[pl.ds(r0, 128), :].astype(F32) + s_rows * gate
        out_v[pl.ds(r0, 128), :] = res.astype(BF16)
        pltpu.make_async_copy(out_v.at[pl.ds(r0, 128), :],
                              out_hbm.at[pl.ds(r0, 128), :], sem_out).start()
        return a3[0:MEM]

    jax.lax.fori_loop(0, NTILE, tile_body, mem0_v[...].astype(F32))
    pltpu.make_async_copy(out_v, out_hbm, sem_out).wait()


@jax.jit
def pallas_recurrent_scan__memory_aug_recurrent_mem_tr__mixer_gmlp__prompt_kernel(
    A_x: jax.Array,
    A_mem0: jax.Array,
    A_Wq: jax.Array,
    A_Wk: jax.Array,
    A_Wv: jax.Array,
    A_Wo: jax.Array,
    A_seg_len: jax.Array,
    B_x: jax.Array,
    B_w_in: jax.Array,
    B_w_sp: jax.Array,
    B_b_sp: jax.Array,
    B_w_out: jax.Array,
):
    del A_seg_len, B_x
    hbm = pl.BlockSpec(memory_space=pl.ANY)
    out = pl.pallas_call(
        _kernel,
        out_shape=jax.ShapeDtypeStruct((S, DM), BF16),
        in_specs=[hbm] * 10,
        out_specs=hbm,
        scratch_shapes=[
            pltpu.VMEM((S, DM), BF16),
            pltpu.VMEM((S // 2, DM), U32),
            pltpu.VMEM((64, 2048), U32),
            pltpu.VMEM((64, 2048), U32),
            pltpu.VMEM((MEM, DM), BF16),
            pltpu.VMEM((16, 128), BF16),
            pltpu.VMEM((16, 128), F32),
            pltpu.VMEM((8, 128), U32),
            pltpu.VMEM((FH, DM), U32),
            pltpu.VMEM((FH // 2, 1280), U32),
            pltpu.VMEM((S // 2, S), U32),
            pltpu.VMEM((FH // 2, DM), U32),
            pltpu.VMEM((64, NSUM * 128), U32),
            pltpu.VMEM((48, DM + 8, DH), U32),
            pltpu.VMEM((3 * H, DM // 2, DH), U32),
            pltpu.VMEM((3 * NGRP, 64, NSUM * 128), U32),
            pltpu.VMEM((H * DH // 2, DM), U32),
            pltpu.VMEM((NGRP, 64, NSUM * 128), U32),
            pltpu.VMEM((T1, FH, 128), F32),
            pltpu.VMEM((T1, 2 * (FH // RB) * 8, 128), F32),
            pltpu.VMEM((FH // 2, S), U32),
            pltpu.VMEM((NTILE // 2, FH // 4, 7 * 128), U32),
            pltpu.VMEM((64, 5 * S // 2), U32),
            pltpu.VMEM((64, FH), U32),
            pltpu.VMEM((96, H * DH), U32),
            pltpu.VMEM((80, H * DH), U32),
            pltpu.VMEM((80, H * DH), U32),
            pltpu.VMEM((32, H * DH), U32),
            pltpu.VMEM((4, 48, 80), F32),
            pltpu.VMEM((S, DM), BF16),
            pltpu.SemaphoreType.DMA((4,)),
            pltpu.SemaphoreType.DMA((8,)),
            pltpu.SemaphoreType.DMA((NTILE // T2,)),
            pltpu.SemaphoreType.DMA((NTILE // T2,)),
            pltpu.SemaphoreType.DMA,
        ],
        compiler_params=pltpu.CompilerParams(vmem_limit_bytes=112 * 1024 * 1024),
    )(
        A_x.reshape(S, DM),
        A_mem0.reshape(MEM, DM),
        A_Wq, A_Wk, A_Wv,
        A_Wo.reshape(H * DH, DM),
        B_w_in.T,
        B_w_sp,
        B_b_sp.reshape(16, 128),
        B_w_out,
    )
    return out.reshape(1, S, DM)
```

```python
import functools

import jax
import jax.numpy as jnp
import jax.experimental.pallas as pl
import jax.experimental.pallas.tpu as pltpu

F32 = jnp.float32
BF16 = jnp.bfloat16
U32 = jnp.uint32

S = 2048
DM = 640
H = 32
DH = 128
MEM = 8
SEG = 32
FH = 864
NTILE = S // 128
EPS = 1e-5
SCALE = DH ** (-0.5)
NEG = -1000000000.0

XCH = 256
T1 = 4
T2 = 4
RB = 144
WIN_PIECES = (2, 4, 6)
SBLK = (144, 144, 144)
SIDE_TAIL = 1
WSP_HEAD = 512
LN_DEADLINE = 10
LN_FIRST = 4
NORM_TAIL = 4
ORDER0 = (1, 0, 2)
PIPE = ((210, 490, 180, 0), (230, 540, 128, 1), (240, 570, 100, 3), (260, 540, 128, 1))
WG = 4
FILL = (320, 224, 224)

NT = (((1,), (1,)), ((), ()))


def _as_bf16(u):
    return pltpu.bitcast(u, BF16)


def _as_u32(b):
    return pltpu.bitcast(b, U32)


def _layernorm(v):
    m = jnp.mean(v, axis=-1, keepdims=True)
    c = v - m
    var = jnp.mean(c * c, axis=-1, keepdims=True)
    return c * jax.lax.rsqrt(var + EPS)


def _gelu2(v):
    c = 0.7978845608028654
    return v + v * jnp.tanh(v * (c + (c * 0.044715) * (v * v)))


def _mult(v, m):
    return v if isinstance(v, int) else pl.multiple_of(v, m)


def _lanes(tile):
    return pl.ds(_mult(tile * 128, 128), 128)


def _mask(qgroups, kgroups):
    shape = (8 * len(qgroups), 8 * len(kgroups))

    def table(groups, axis):
        idx = jax.lax.broadcasted_iota(jnp.int32, shape, axis)
        seg = jnp.full(shape, groups[-1][0], jnp.int32)
        pos = idx + (groups[-1][1] - 8 * (len(groups) - 1))
        for g in range(len(groups) - 2, -1, -1):
            inside = idx < 8 * (g + 1)
            seg = jnp.where(inside, groups[g][0], seg)
            pos = jnp.where(inside, idx + (groups[g][1] - 8 * g), pos)
        return seg, pos

    qseg, qpos = table(qgroups, 0)
    kseg, kpos = table(kgroups, 1)
    same = qseg == kseg
    keep = same & ((qpos < MEM) | (qpos >= kpos))
    return keep, jnp.where(same, NEG, -jnp.inf).astype(F32)


def _masks():
    own = lambda sg: [(sg, 0), (sg, 16), (sg, 24), (sg, 32)]
    k0 = [(0, 0), (0, 8), (0, 16), (0, 24), (0, 32), (1, 8)]
    k2 = own(2) + [(2, 8), (3, 8)]
    return [
        _mask(k0[:4], k0),
        _mask(own(1) + k0[4:], own(1) + k0),
        _mask(own(2), k2),
        _mask(own(3) + k2[4:], own(3) + k2),
    ]


def _fast_table(types):
    lines = {0: ((1, 0), (1, -1)), 1: ((0, 1), (1, -1)), 2: ((1, 0), (0, 1))}
    neg = lambda f: (-f[0], -f[1])

    def dual(u, v):
        det = u[0] * v[1] - u[1] * v[0]
        return (v[1] * det, -v[0] * det), (-u[1] * det, u[0] * det)

    n = len(types)
    diag = {(i, k): {(i, i): 1} for i in range(n) for k in range(2)}
    units = [[] for _ in range(n)]
    for i in range(n):
        u = lines[types[i]]
        units[i] += [('p', [(i, u[k])], diag[i, k], [(i, dual(*u)[k])]) for k in range(2)]
        for j in range(i + 1, n):
            if types[i] == types[j]:
                units[i] += [('b', i, j), ('b', j, i)]
                continue
            w = lines[types[j]]
            (ci, cj), = [(x, y) for x in range(2) for y in range(2) if u[x] == w[y]]
            (p, q), = [(x, y) for x in (u[1 - ci], neg(u[1 - ci])) for y in (w[1 - cj], neg(w[1 - cj]))
                       if (x[0] - y[0], x[1] - y[1]) == u[ci]]
            sd, td = dual(p, q)
            units[i] += [('p', [(i, p), (j, q)], {(i, j): 1, (j, i): 1}, [(i, td), (j, sd)]),
                         ('p', [(i, q), (j, q)], {(i, j): 1}, [(i, neg(td)), (j, td)]),
                         ('p', [(i, p), (j, p)], {(j, i): 1}, [(i, sd), (j, neg(sd))])]
            diag[i, ci][i, j] = 1
            diag[i, 1 - ci][j, i] = -1
            diag[j, 1 - cj][i, j] = -1
            diag[j, cj][j, i] = 1
    out = []
    for i in range(n):
        row = []
        for un in units[i]:
            if un[0] == 'p' and [c for c in un[1][0][1] if c][0] < 0:
                un = ('p', [(k, neg(f)) for k, f in un[1]], un[2], [(k, neg(f)) for k, f in un[3]])
            row.append(un)
        out.append(row)
    return out


GH = 5
NGRP = H // GH
WOFF = H - NGRP * GH
UNITS = _fast_table((0, 1, 2, 0, 1))


def _relabel(kmap, nmap):
    return [('p', [(kmap[i], f) for i, f in un[1]], {(kmap[i], nmap[j]): c for (i, j), c in un[2].items()},
             [(nmap[j], f) for j, f in un[3]]) for row in _fast_table((0, 1)) for un in row]


UNITS_N2 = [[('b', 2, 0), ('b', 2, 1)], _relabel((0, 1), (0, 1)), _relabel((3, 4), (0, 1))]
UNITS_K2 = [[('b', 0, 2), ('b', 1, 2)], _relabel((0, 1), (0, 1)), _relabel((0, 1), (3, 4))]


def _sums(units):
    return [un[2] for row in units for un in row if un[0] == 'p' and len(un[2]) > 1]


NSUM = len(_sums(UNITS))
NSUM2 = len(_sums(UNITS_N2))


def _signed_sum(terms):
    terms = sorted(terms, key=lambda cv: -cv[0])
    acc = terms[0][1]
    for c, v in terms[1:]:
        acc = acc + v if c > 0 else acc - v
    return acc


def _lhs_operands(top, bot):
    forms = {}

    def form(i, f):
        sign = 1 if [c for c in f if c][0] > 0 else -1
        key = (i, (sign * f[0], sign * f[1]))
        if key not in forms:
            forms[key] = {(1, 0): lambda: top[i], (0, 1): lambda: bot[i],
                          (1, -1): lambda: top[i] - bot[i]}[key[1]]()
        return sign, forms[key]

    ops = {}

    def operand(un):
        key = tuple(un[1])
        if key not in ops:
            ops[key] = _signed_sum([form(i, f) for i, f in un[1]]).astype(BF16)
        return ops[key]

    return operand


class _Acc:
    def __init__(self):
        self.v = {}

    def add(self, key, c, p):
        if key not in self.v:
            self.v[key] = (c, p)
        else:
            sign, v = self.v[key]
            self.v[key] = (sign, v + p if sign == c else v - p)

    def pop(self, key):
        sign, v = self.v.pop(key)
        return v if sign > 0 else -v


def _kernel(x_hbm, mem0_hbm, wq_hbm, wk_hbm, wv_hbm, wo_hbm, wint_hbm, wsp_hbm,
            bsp_hbm, wout_hbm, out_hbm,
            x_v, xn_v, xa_v, xb_v, mem0_v, bsp_v, bsp32_v, zero_v, wint_v, wins_v, wsp_v, wout_v, woutc_v,
            stage_v, wqkv_v, wc_v, wc2_v, wo_v, woc_v, zg_v, st_v, z1t_v, za_v, ts_v, u_v, q_v, k_v, v_v, o_v, cap_v, out_v,
            sem_x, sem_w, sem_st, sem_wo, sem_out):
    NRB = FH // RB
    NG = RB // 8
    NB2 = NTILE // T2
    PPB = 48 // NB2

    x_parts = [(0, XCH), (XCH, XCH), (2 * XCH, XCH), (3 * XCH, S - 3 * XCH)]
    x_cps = [pltpu.make_async_copy(x_hbm.at[pl.ds(o, n), :], x_v.at[pl.ds(o, n), :], sem_x.at[k])
             for k, (o, n) in enumerate(x_parts)]
    wint_u = wint_hbm.bitcast(U32)
    blk_row = lambda k: (FH + k * RB) if k < NRB else (k - NRB) * RB
    wint_cps, k0 = [], 0
    for k, nb in enumerate(WIN_PIECES):
        o, n = blk_row(k0) // 2, nb * RB // 2
        wint_cps.append(pltpu.make_async_copy(wint_u.at[pl.ds(o, n), :], wint_v.at[pl.ds(o, n), :],
                                              sem_w.at[k]))
        k0 += nb
    wsp_u = wsp_hbm.bitcast(U32)
    wsp_cp = pltpu.make_async_copy(wsp_u.at[pl.ds(0, WSP_HEAD), :], wsp_v.at[pl.ds(0, WSP_HEAD), :],
                                   sem_w.at[3])
    wsp_cp2 = pltpu.make_async_copy(wsp_u.at[pl.ds(WSP_HEAD, S // 2 - WSP_HEAD), :],
                                    wsp_v.at[pl.ds(WSP_HEAD, S // 2 - WSP_HEAD), :], sem_w.at[7])
    wout_cp = pltpu.make_async_copy(wout_hbm.bitcast(U32), wout_v, sem_w.at[4])
    WOQ = H * DH // 2 // NB2

    def wo_copy(i):
        r0 = _mult(i * WOQ, WOQ)
        return pltpu.make_async_copy(wo_hbm.bitcast(U32).at[pl.ds(r0, WOQ), :],
                                     wo_v.at[pl.ds(r0, WOQ), :], sem_wo.at[i])

    mem0_cp = pltpu.make_async_copy(mem0_hbm, mem0_v, sem_w.at[5])
    bsp_cp = pltpu.make_async_copy(bsp_hbm, bsp_v, sem_w.at[6])
    w_hbms = (wq_hbm, wk_hbm, wv_hbm)

    def stage_copy(m, j):
        p = m * 16 + j
        return pltpu.make_async_copy(w_hbms[m].bitcast(U32).at[:, j, :],
                                     stage_v.at[p, pl.ds(0, DM), :], sem_st.at[p // PPB])

    x_cps[0].start()
    x_cps[1].start()
    for cp in wint_cps:
        cp.start()
    x_cps[2].start()
    x_cps[3].start()
    bsp_cp.start()
    mem0_cp.start()
    wsp_cp.start()
    wout_cp.start()
    for p in range(48):
        stage_copy(p // 16, p % 16).start()
        if (p + 1) % PPB == 0:
            wo_copy(p // PPB).start()
        if p + 1 == 2 * PPB:
            wsp_cp2.start()

    zero_v[...] = jnp.zeros((8, 128), U32)
    for n, (keep, fill) in enumerate(_masks()):
        cap_v[n, 0:keep.shape[0], 0:keep.shape[1]] = jnp.where(keep, 0.0, fill)

    pending = []

    def dep_of(v):
        return pltpu.bitcast(v[0:8, 0:128], U32) & zero_v[...]

    def up(u):
        return _as_bf16(u).astype(F32)

    def ln_rows(r0, n, dep=None):
        xr = x_v[pl.ds(r0, n), :].astype(F32)
        if dep is not None:
            d = jnp.concatenate([dep] * (n // 8), axis=0)
            xr = pltpu.bitcast(pltpu.bitcast(xr, U32) | jnp.concatenate([d] * (DM // 128), axis=1), F32)
        xn = _layernorm(xr)
        xn_v[pl.ds(_mult(r0 // 2, n // 2), n // 2), :] = _as_u32(xn.astype(BF16))
        return xn

    def ln_pair(base, k, dst, dep):
        xe = ln_rows(_mult(base + 16 * k, 16), 16, dep)
        xo = ln_rows(_mult(base + 128 + 16 * k, 16), 16, dep)
        b11, b21, b12, b22 = xe[:, 0:256], xe[:, 256:512], xo[:, 0:256], xo[:, 256:512]
        ops = jnp.concatenate([b11 + b22, b11, b12 - b22, b21 - b11, b22,
                               b11 + b12, xo[:, 512:], b21 + b22, xe[:, 512:]], axis=1)
        dst[8 * k:8 * k + 8, :] = _as_u32(ops.astype(BF16))
        pending.append([LN_DEADLINE, dst[8 * k:8 * k + 8, 0:128] & zero_v[...]])

    def win_sums(hz, k, dep):
        d = jnp.concatenate([dep] * 4, axis=1)
        r0 = hz * (FH // 2) + 8 * k
        top, bot = up(wint_v[r0:r0 + 8, 0:512] | d), up(wint_v[r0 + FH // 4:r0 + FH // 4 + 8, 0:512] | d)
        a11, a12, a21, a22 = top[:, 0:256], top[:, 256:512], bot[:, 0:256], bot[:, 256:512]
        ops = jnp.concatenate([a11 + a22, a21 + a22, a11 + a12, a21 - a11, a12 - a22], axis=1)
        wins_v[hz * (FH // 4) + 8 * k:hz * (FH // 4) + 8 * k + 8, :] = _as_u32(ops.astype(BF16))

    def nt_dot(w, xt):
        due = None
        for e in pending:
            e[0] -= 1
            if e[0] == 0:
                due = e[1] if due is None else due | e[1]
        pending[:] = [e for e in pending if e[0] > 0]
        if due is not None:
            top = w[0:8, 0:128] | due
            if w.shape[1] > 128:
                top = jnp.concatenate([top, w[0:8, 128:]], axis=1)
            w = jnp.concatenate([top, w[8:]], axis=0)
        return jax.lax.dot_general(_as_bf16(w), _as_bf16(xt), NT, preferred_element_type=F32)

    def win_block(nt, f0):
        return nt_dot(wint_v[f0 // 2:(f0 + RB) // 2, :], xn_v[nt * 64:(nt + 1) * 64, :])

    def win_group(src, hz, rb, emit, side):
        rt = (hz * FH + rb * RB) // 2
        rows = lambda r: slice(r, r + RB // 2)
        top, bot, sm = rows(rt), rows(rt + FH // 4), rows(hz * (FH // 4) + rb * RB // 2)
        ss = lambda q: wins_v[sm, q * 256:(q + 1) * 256]
        tt = lambda q: src[:, q * 256:(q + 1) * 256]
        rest = lambda r: wint_v[r, 512:640]

        def prod(w, xt):
            p = nt_dot(w, xt)
            side(p)
            return p

        m2 = prod(ss(1), tt(1))
        m4 = prod(wint_v[bot, 256:512], tt(3))
        emit(0, rb + NRB // 2, m2 + m4 + prod(rest(bot), src[:, 1920:2048]))
        m3 = prod(wint_v[top, 0:256], tt(2))
        m5 = prod(ss(2), tt(4))
        emit(1, rb, m3 + m5 + prod(rest(top), src[:, 1536:1664]))
        c11, c22 = m4 - m5, m3 - m2
        m1 = prod(ss(0), tt(0))
        emit(0, rb, c11 + m1 + prod(jnp.concatenate([ss(4), rest(top)], axis=1), src[:, 1664:2048]))
        emit(1, rb + NRB // 2,
             c22 + m1 + prod(jnp.concatenate([ss(3), rest(bot)], axis=1), src[:, 1280:1664]))

    def z2_emit(nt, rb, z):
        g = _gelu2(z)
        zg_v[nt, rb * RB:(rb + 1) * RB, :] = g
        g3 = g.reshape(NG, 8, 128)
        bm = jnp.sum(g3, axis=0) * (1.0 / NG)
        c = g3 - bm
        st_v[nt, rb * 8:(rb + 1) * 8, :] = bm
        st_v[nt, (NRB + rb) * 8:(NRB + rb + 1) * 8, :] = jnp.sum(c * c, axis=0)

    def z2_stats(nt):
        bm = st_v[nt, 0:NRB * 8, :]
        m = jnp.sum(bm, axis=0, keepdims=True) * (1.0 / (NRB * 8))
        dm = bm - m
        m2 = jnp.sum(st_v[nt, NRB * 8:2 * NRB * 8, :] + dm * dm * NG, axis=0, keepdims=True)
        r = jax.lax.rsqrt(m2 * (1.0 / FH) + 4.0 * EPS)
        return jnp.broadcast_to(m, (8, 128)), jnp.broadcast_to(r, (8, 128))

    def z2_norm(ne, tp, k, st, dep):
        (me, re), (mo, ro) = st
        me = pltpu.bitcast(pltpu.bitcast(me, U32) | dep, F32)
        mo = pltpu.bitcast(pltpu.bitcast(mo, U32) | dep, F32)
        nrm = lambda nt, f0, m, r: ((zg_v[nt, f0:f0 + 16, :].reshape(2, 8, 128) - m) * r).reshape(16, 128)
        a11, a21 = nrm(ne, 16 * k, me, re), nrm(ne, FH // 2 + 16 * k, me, re)
        a12, a22 = nrm(ne + 1, 16 * k, mo, ro), nrm(ne + 1, FH // 2 + 16 * k, mo, ro)
        ops = jnp.concatenate([a11 + a22, a21 + a22, a11, a22, a11 + a12, a21 - a11, a12 - a22], axis=1)
        za_v.at[tp][8 * k:8 * k + 8, :] = _as_u32(ops.astype(BF16))

    def z1_emit(tile, rb, z):
        z1t_v[rb * RB // 2:(rb + 1) * RB // 2, _lanes(tile)] = _as_u32(_gelu2(z).astype(BF16))

    def spread(tasks, slots):
        state = [0]

        def side(p):
            n = state[0]
            mine = tasks[n * len(tasks) // slots:(n + 1) * len(tasks) // slots]
            for q, fn in enumerate(mine):
                fn(dep_of(p[8 * ((q * NG) // len(mine)):]))
            state[0] += 1

        return side

    def mix(*kinds):
        order = sorted(((q + 0.5) / len(kd), kn, q) for kn, kd in enumerate(kinds) for q in range(len(kd)))
        return [kinds[kn][q] for _, kn, q in order]

    part = functools.partial
    NSLAB = FH // 32

    x_cps[0].wait()
    ln_rows(0, XCH)
    x_cps[1].wait()
    ln_rows(XCH, XCH)
    wint_cps[0].wait()
    for nt in range(T1):
        for rb in range(WIN_PIECES[0]):
            z2_emit(nt, rb, win_block(nt, FH + rb * RB))
    wint_cps[1].wait()
    side = spread([part(win_sums, 1, k) for k in range(NSLAB)], T1 * (NRB - WIN_PIECES[0]) - 1)
    for nt in range(T1):
        for rb in range(WIN_PIECES[0], NRB):
            z = win_block(nt, FH + rb * RB)
            z2_emit(nt, rb, z)
            side(z)
    wint_cps[2].wait()
    x_cps[2].wait()
    norms = []
    for ne in range(0, T1, 2):
        st = (z2_stats(ne), z2_stats(ne + 1))
        norms += [part(z2_norm, ne, ne // 2, k, st) for k in range(NSLAB)]
    side = spread(mix(norms, [part(win_sums, 0, k) for k in range(NSLAB)],
                      [part(ln_pair, T1 * 128, k, xa_v) for k in range(8)]), T1 * NRB - 1)
    for nt in range(T1):
        for rb in range(NRB):
            z = win_block(nt, rb * RB)
            z1_emit(nt, rb, z)
            side(z)
    x_cps[3].wait()
    pending.clear()

    def b1_body(i, carry):
        for ne in range(0, T1, 2):
            tile = i * T1 + ne
            src, dst = (xa_v, xb_v) if ne == 0 else (xb_v, xa_v)
            base = jnp.minimum(tile + 2, NTILE - 2) * 128
            lns = [part(ln_pair, base, k, dst) for k in range(8)]
            side = spread(lns[:LN_FIRST], 9 * NRB // 2)
            for rb in range(NRB // 2):
                win_group(src, 1, rb, lambda o, r, z: z2_emit(ne + o, r, z), side)
            st = (z2_stats(ne), z2_stats(ne + 1))
            norms = [part(z2_norm, ne, tile // 2, k, st) for k in range(NSLAB)]
            side = spread(mix(norms, lns[LN_FIRST:]) if LN_FIRST < 8 else norms, 9 * NRB // 2 - NORM_TAIL)
            for rb in range(NRB // 2):
                win_group(src, 0, rb, lambda o, r, z: z1_emit(tile + o, r, z), side)
        pending.clear()
        return carry

    jax.lax.fori_loop(1, NTILE // T1, b1_body, 0)

    wsp_cp.wait()
    wout_cp.wait()
    bsp_cp.wait()
    mem0_cp.wait()
    bsp32_v[...] = 0.5 * bsp_v[...].astype(F32)

    def split_block(p, bi, dep):
        a = stage_v[p, pl.ds(128 * bi, 64, stride=2), :] | dep
        b = stage_v[p, pl.ds(128 * bi + 1, 64, stride=2), :] | dep
        wqkv_v[2 * p, 64 * bi:64 * bi + 64, :] = (a & jnp.uint32(0xFFFF)) | (b << 16)
        wqkv_v[2 * p + 1, 64 * bi:64 * bi + 64, :] = (a >> 16) | (b & jnp.uint32(0xFFFF0000))

    def weight_sums(units, block, dst, rows, idx, dep):
        cache = {}

        def blk(ij):
            if ij not in cache:
                w = block(*ij)
                cache[ij] = up(w | dep[0:w.shape[0]])
            return cache[ij]

        mine = _sums(units[idx:idx + 1])
        c0 = _sums(units).index(mine[0])
        sums = jnp.concatenate([_signed_sum([(c, blk(ij)) for ij, c in r.items()]) for r in mine], axis=1)
        dst[rows, c0 * 128:(c0 + len(mine)) * 128] = _as_u32(sums.astype(BF16))

    fblocks = [(f0, min(128, FH - f0)) for f0 in range(0, FH, 128)]

    def u_transpose(tile):
        for f0, fn in fblocks:
            ut = _as_bf16(z1t_v[f0 // 2:(f0 + fn) // 2, _lanes(tile)]).astype(F32)
            u_v[:, f0:f0 + fn] = _as_u32(ut.T.astype(BF16))

    NK = NTILE // 2

    def t_piece(tp, k, dep):
        h0 = _mult(tp * 128, 128)
        we = wsp_v[pl.ds(h0, 64), k * 256:(k + 1) * 256]
        wo = wsp_v[pl.ds(h0 + 64, 64), k * 256:(k + 1) * 256]
        d = jnp.concatenate([dep, dep], axis=1)
        we, wo = up(we | d), up(wo | d)
        b11, b21, b12, b22 = we[:, 0:128], we[:, 128:256], wo[:, 0:128], wo[:, 128:256]
        ops = jnp.concatenate([b11 + b22, b12 - b22, b21 - b11, b11 + b12, b21 + b22], axis=1)
        z0 = pl.multiple_of(jnp.minimum(tp, 0) * 64, 64)
        ts_v[pl.ds(z0, 64), k * 640:(k + 1) * 640] = _as_u32(ops.astype(BF16))

    def b2_body(i, carry):
        group = stage_v.at[pl.ds(i * PPB, PPB), pl.ds(0, DM), :]
        pltpu.make_async_copy(group, group, sem_st.at[i]).wait()
        wo_copy(i).wait()

        @pl.when(i == 2)
        def _():
            wsp_cp2.wait()

        u_transpose(0)
        for lp in range(2):
            tp = i * 2 + lp
            he = pl.multiple_of(tp * 128, 128)
            raw = lambda odd_t, odd_s: lambda k: wsp_v[
                pl.ds(he + odd_t * 64, 64), (2 * k + odd_s) * 128:(2 * k + odd_s + 1) * 128]
            tj = lambda j: lambda k: ts_v[:, k * 640 + j * 128:k * 640 + (j + 1) * 128]
            rhs = [tj(0), raw(0, 0), tj(1), tj(2), raw(1, 1), tj(3), tj(4)]

            full = slice(0, 64)
            kinds = [[]]
            if lp == 0:
                kinds[0] = [(9, part(split_block, i * PPB + pp, bi)) for pp in range(PPB) for bi in range(GH)]
                kinds.append([])
                for sl in range(2):
                    gid = jnp.maximum(i, 2 * i - 2 + sl)
                    block = lambda bi, bj, gid=gid: wo_v[
                        pl.ds(pl.multiple_of((WOFF + gid * GH + bi) * 64, 64), 64), bj * 128:(bj + 1) * 128]
                    kinds[1] += [(30, part(weight_sums, UNITS, block, woc_v.at[gid], full, idx)) for idx in range(GH)]
            else:
                for sl in range(5):
                    gid = jnp.minimum((9 * i) // 2 + sl, (9 * i + 9) // 2 - 1)
                    f0h = (gid // NGRP) * H + (gid % NGRP) * GH
                    block = lambda bi, bj, f0h=f0h: wqkv_v[f0h + bj, 64 * bi:64 * bi + 64, :]
                    kinds[0] += [(30, part(weight_sums, UNITS, block, wc_v.at[gid], full, idx)) for idx in range(GH)]
                m2 = jnp.maximum(i - 1, 0)
                f0h = jnp.minimum(i, 1) * (m2 * H + NGRP * GH)
                block = lambda bi, bj, f0h=f0h: wqkv_v[f0h + bj, 64 * bi:64 * bi + 64, :]
                kinds.append([(24, part(weight_sums, UNITS_N2, block, wc2_v.at[m2], full, idx)) for idx in (1, 2)])
            r8 = pl.multiple_of(8 * (2 * i + lp), 8)
            block = lambda bi, bj, r8=r8: wo_v[pl.ds(64 * bi + r8, 8), bj * 128:(bj + 1) * 128]
            kinds.append([(3, part(weight_sums, UNITS_K2, block, wc2_v.at[3], pl.ds(r8, 8), idx)) for idx in (1, 2)])
            block = lambda bi, bj, r8=r8: wout_v[pl.ds(64 * bi + r8, 8), bj * 128:(bj + 1) * 128]
            kinds.append([(4, part(weight_sums, UNITS, block, woutc_v, pl.ds(r8, 8), idx)) for idx in range(GH)])
            tasks = [(28, part(t_piece, tp, k)) for k in range(NK)] + mix(*kinds)
            budget = sum(c for c, _ in tasks) / (2 * 7 * len(SBLK) - SIDE_TAIL)
            state = [0.0]

            def side(p):
                state[0] += budget
                phase = 0
                while tasks and state[0] > 0:
                    c, fn = tasks.pop(0)
                    rows = p[0:128].reshape(8, 16, 128)[:, 8 * phase:8 * phase + 8, :]
                    fn((pltpu.bitcast(rows, U32) & zero_v[...]).reshape(64, 128))
                    state[0] -= c
                    phase = 1 - phase

            def prod(j, f0, fn):
                p = None
                for ks in (range(NK // 2), range(NK // 2, NK)):
                    lhs = jnp.concatenate(
                        [za_v[k, f0 // 2:(f0 + fn) // 2, j * 128:(j + 1) * 128] for k in ks], axis=1)
                    r = jnp.concatenate([rhs[j](k) for k in ks], axis=1)
                    q = jax.lax.dot_general(_as_bf16(lhs), _as_bf16(r), NT, preferred_element_type=F32)
                    side(q)
                    p = q if p is None else p + q
                return p

            def finish(c, f0, fn, odd_t):
                tile = tp * 2 + odd_t
                z1 = _as_bf16(z1t_v[f0 // 2:(f0 + fn) // 2, _lanes(tile)]).astype(F32)
                brow = bsp32_v[pl.ds(tile, 1), :]
                z1t_v[f0 // 2:(f0 + fn) // 2, _lanes(tile)] = _as_u32((z1 * (0.5 * c + brow)).astype(BF16))

            blocks = [(sum(SBLK[:q]), fn) for q, fn in enumerate(SBLK)]
            early = [(prod(1, f0, fn), prod(4, f0, fn)) for f0, fn in blocks]
            assert all(fn.func is not t_piece for _, fn in tasks)
            for (f0, fn), (m2, m5) in zip(blocks, early):
                m4 = prod(3, f0, fn)
                finish(m2 + m4, FH // 2 + f0, fn, 0)
                m1 = prod(0, f0, fn)
                finish(m4 - m5 + m1 + prod(6, f0, fn), f0, fn, 0)
                m3 = prod(2, f0, fn)
                finish(m3 + m5, f0, fn, 1)
                finish(m3 - m2 + m1 + prod(5, f0, fn), FH // 2 + f0, fn, 1)
            assert not tasks
        return carry

    jax.lax.fori_loop(0, NB2, b2_body, 0)

    dot = lambda l, r: jnp.dot(l, r, preferred_element_type=F32)

    def fast_units(units, lhs_of, both, raw, sums, acc, done):
        items = []
        for i, row in enumerate(units):
            for q, un in enumerate(row):
                def fn(un=un, last=(q == len(row) - 1), i=i):
                    if un[0] == 'b':
                        p = dot(both(un[1]), raw(un[1], un[2]))
                        hr = p.shape[0] // 2
                        acc.add((0, un[2]), 1, p[0:hr])
                        acc.add((1, un[2]), 1, p[hr:])
                    else:
                        r = un[2]
                        p = dot(lhs_of(un), raw(*list(r)[0]) if len(r) == 1 else sums(_sums(units).index(r)))
                        for k, f in un[3]:
                            for half in range(2):
                                if f[half]:
                                    acc.add((half, k), f[half], p)
                    if last:
                        done(i)
                items.append((16 if un[0] == 'b' else 8, fn))
        return items

    def step(n, h):
        odd = n % 2 == 1
        hb = h.astype(BF16)
        qb = 24 * n
        kb = 40 * (n // 2) + (0 if odd else 16)
        nq, nk = (24, 40) if odd else (16, 24)
        clock = [0]
        d_s, d_o, gap, lag_v = PIPE[n]
        ready, s_at, o_at, ps = {}, {}, {}, {}

        def put(buf, r0, t, v):
            buf[r0:r0 + v.shape[0] // 2, _lanes(t)] = _as_u32(v.astype(BF16))

        def put64(m, t, top, bot):
            buf = (q_v, k_v, v_v)[m]
            if m == 0:
                put(buf, 0, t, top)
                put(buf, 24 + 16, t, bot[0:16])
                put(buf, 72 + 16, t, bot[16:32])
            else:
                put(buf, 16, t, top)
                put(buf, 32, t, bot[0:16])
                put(buf, 40 + 32, t, bot[16:32])
            ready[m, t] = clock[0]

        def plain(m, t):
            put((q_v, k_v, v_v)[m], qb if m == 0 else kb, t, dot(hb, _as_bf16(wqkv_v[m * H + t])))
            ready[m, t] = clock[0]

        work = []
        if n == 0:
            cols = lambda i: slice(i * 128, (i + 1) * 128)
            make = _lhs_operands([h[0:32, cols(i)] for i in range(GH)], [h[32:64, cols(i)] for i in range(GH)])
            for row in UNITS:
                for un in row:
                    if un[0] == 'p':
                        make(un)

            def group(m, t0, units, sums):
                acc = _Acc()

                def done(j):
                    for jj in ([j] if units is UNITS else range(2) if j == len(units) - 1 else []):
                        put64(m, t0 + jj, acc.pop((0, jj)), acc.pop((1, jj)))

                return fast_units(units, make, lambda i: hb[:, cols(i)],
                                  lambda i, j: _as_bf16(wqkv_v[m * H + t0 + j, 64 * i:64 * i + 64, :]),
                                  lambda q: _as_bf16(sums[:, cols(q)]), acc, done)

            last = lambda m: group(m, NGRP * GH, UNITS_N2, wc2_v.at[m])
            for g in range(NGRP):
                for m in ORDER0:
                    if g == NGRP - 1 and m == 2:
                        work += last(1) + last(0)
                    work += group(m, g * GH, UNITS, wc_v.at[m * NGRP + g])
            work += last(2)
        else:
            for t in range(H + lag_v):
                for m, tt in ((1, t), (2, t - lag_v), (0, t)):
                    if 0 <= tt < H:
                        work.append((40, functools.partial(plain, m, tt)))
        work = [(c, fn, -1) for c, fn in work]

        res = []
        if n == 3:
            acc = _Acc()

            def wo_group(h0, nh, units, sums):
                hc = lambda i: slice((h0 + i) * DH, (h0 + i + 1) * DH)
                box = []

                def lhs_of(un):
                    if not box:
                        box.append(_lhs_operands([up(o_v[0:16, hc(i)]) for i in range(nh)],
                                                 [up(o_v[16:32, hc(i)]) for i in range(nh)]))
                    return box[0](un)

                items = fast_units(
                    units, lhs_of, lambda i: _as_bf16(o_v[:, hc(i)]),
                    lambda i, j: _as_bf16(wo_v[(h0 + i) * 64:(h0 + i + 1) * 64, j * 128:(j + 1) * 128]),
                    lambda q: _as_bf16(sums[:, q * 128:(q + 1) * 128]), acc, lambda j: None)
                return [(c, fn, h0 + nh - 1) for c, fn in items]

            work += wo_group(0, WOFF, UNITS_K2, wc2_v.at[3])
            for g in range(NGRP):
                work += wo_group(WOFF + g * GH, GH, UNITS, woc_v.at[g])
            work.append((0, lambda: res.append(jnp.concatenate(
                [jnp.concatenate([acc.pop((hf, j)) for j in range(GH)], axis=1) for hf in range(2)],
                axis=0)), H - 1))
        else:
            def wgroup(g):
                c0, c1 = g * WG * DH, (g + 1) * WG * DH
                part = dot(_as_bf16(o_v[0:16, c0:c1]), _as_bf16(wo_v[c0 // 2:c1 // 2, :]))
                res[:] = [part + res[0]] if res else [part]

            work += [(40 * WG, functools.partial(wgroup, g), (g + 1) * WG - 1) for g in range(H // WG)]

        def scores(t):
            sc = jax.lax.dot_general(_as_bf16(q_v[qb:qb + nq, _lanes(t)]),
                                     _as_bf16(k_v[kb:kb + nk, _lanes(t)]), NT,
                                     preferred_element_type=F32) * SCALE
            cap = cap_v[n, 0:sc.shape[0], 0:sc.shape[1]]
            sc = jnp.where(cap == 0.0, sc, cap)
            e = jnp.exp(sc - jnp.max(sc, axis=-1, keepdims=True))
            l = jnp.sum(e, axis=-1, keepdims=True)
            inv = pl.reciprocal(l, approx=True)
            inv = inv * (2.0 - l * inv)
            ps[t] = (e * inv).astype(BF16)
            s_at[t] = clock[0]
            clock[0] += nq // 2

        def values(t):
            o = dot(ps.pop(t), _as_bf16(v_v[kb:kb + nk, _lanes(t)]))
            if n == 1:
                put(o_v, 0, t, o[0:32])
                put(o_v, 24, t, o[32:48])
            else:
                put(o_v, 0, t, o)
            o_at[t] = clock[0]
            clock[0] += nq // 2

        def drain(upto):
            while True:
                to, ts = len(o_at), len(s_at)
                if to < ts and (2, to) in ready and (
                        to <= upto or clock[0] >= max(s_at[to] + d_o, ready[2, to] + d_s)):
                    values(to)
                elif ts < H and (0, ts) in ready and (1, ts) in ready and (
                        ts <= upto or clock[0] >= max(ready[0, ts] + d_s, ready[1, ts] + d_s,
                                                      s_at.get(ts - 1, -gap) + gap)):
                    scores(ts)
                else:
                    return

        for c, fn, need in work:
            drain(need)
            clock[0] += c
            fn()
        return res[0]

    def gate_work():
        acc = _Acc()
        cols = lambda i: slice(i * 128, (i + 1) * 128)
        box = []

        def lhs_of(un):
            if not box:
                box.append(_lhs_operands([up(u_v[0:32, cols(i)]) for i in range(GH)],
                                         [up(u_v[32:64, cols(i)]) for i in range(GH)]))
            return box[0](un)

        items = [(2 * c, fn) for c, fn in fast_units(
            UNITS, lhs_of, lambda i: _as_bf16(u_v[:, cols(i)]),
            lambda i, j: _as_bf16(wout_v[64 * i:64 * i + 64, cols(j)]),
            lambda q: _as_bf16(woutc_v[:, cols(q)]), acc, lambda j: None)]

        def rest(j):
            p = dot(_as_bf16(u_v[:, DM:FH]), _as_bf16(wout_v[DM // 2:FH // 2, cols(j)]))
            acc.add((0, j), 1, p[0:64])
            acc.add((1, j), 1, p[64:128])

        items = [(64, functools.partial(rest, j)) for j in range(GH)] + items

        def chunk(budget):
            box.clear()
            while items and budget > 0:
                c, fn = items.pop(0)
                fn()
                budget -= c

        def result():
            hb = 0.5 * jnp.concatenate(
                [jnp.concatenate([acc.pop((hf, j)) for j in range(GH)], axis=1) for hf in range(2)], axis=0)
            return hb + hb * jnp.tanh(hb)

        return chunk, result

    def tile_body(j, mem):
        r0 = pl.multiple_of(j * 128, 128)
        xs = _as_bf16(xn_v[pl.ds(pl.multiple_of(j * 64, 64), 64), :]).astype(F32)
        chunk, gate_result = gate_work()
        chunk(FILL[0])
        a0 = step(0, jnp.concatenate([mem, xs[0:40], xs[64:72], xs[96:104]], axis=0))
        chunk(FILL[1])
        a1 = step(1, jnp.concatenate([a0[0:MEM], xs[40:64]], axis=0))
        chunk(FILL[2])
        a2 = step(2, jnp.concatenate([a1[0:MEM], xs[72:96]], axis=0))
        chunk(10 ** 6)
        gate = gate_result()
        u_transpose(jnp.minimum(j + 1, NTILE - 1))
        a3 = step(3, jnp.concatenate([a2[0:MEM], xs[104:128]], axis=0))
        s_rows = jnp.concatenate([a0[8:32], a3[48:64], a1[8:32], a3[32:40], a2[8:32], a3[40:48], a3[8:32]],
                                 axis=0)
        res = x_v[pl.ds(r0, 128), :].astype(F32) + s_rows * gate
        out_v[pl.ds(r0, 128), :] = res.astype(BF16)
        pltpu.make_async_copy(out_v.at[pl.ds(r0, 128), :],
                              out_hbm.at[pl.ds(r0, 128), :], sem_out).start()
        return a3[0:MEM]

    jax.lax.fori_loop(0, NTILE, tile_body, mem0_v[...].astype(F32))
    pltpu.make_async_copy(out_v, out_hbm, sem_out).wait()


@jax.jit
def pallas_recurrent_scan__memory_aug_recurrent_mem_tr__mixer_gmlp__prompt_kernel(
    A_x: jax.Array,
    A_mem0: jax.Array,
    A_Wq: jax.Array,
    A_Wk: jax.Array,
    A_Wv: jax.Array,
    A_Wo: jax.Array,
    A_seg_len: jax.Array,
    B_x: jax.Array,
    B_w_in: jax.Array,
    B_w_sp: jax.Array,
    B_b_sp: jax.Array,
    B_w_out: jax.Array,
):
    del A_seg_len, B_x
    hbm = pl.BlockSpec(memory_space=pl.ANY)
    out = pl.pallas_call(
        _kernel,
        out_shape=jax.ShapeDtypeStruct((S, DM), BF16),
        in_specs=[hbm] * 10,
        out_specs=hbm,
        scratch_shapes=[
            pltpu.VMEM((S, DM), BF16),
            pltpu.VMEM((S // 2, DM), U32),
            pltpu.VMEM((64, 2048), U32),
            pltpu.VMEM((64, 2048), U32),
            pltpu.VMEM((MEM, DM), BF16),
            pltpu.VMEM((16, 128), BF16),
            pltpu.VMEM((16, 128), F32),
            pltpu.VMEM((8, 128), U32),
            pltpu.VMEM((FH, DM), U32),
            pltpu.VMEM((FH // 2, 1280), U32),
            pltpu.VMEM((S // 2, S), U32),
            pltpu.VMEM((FH // 2, DM), U32),
            pltpu.VMEM((64, NSUM * 128), U32),
            pltpu.VMEM((48, DM + 8, DH), U32),
            pltpu.VMEM((3 * H, DM // 2, DH), U32),
            pltpu.VMEM((3 * NGRP, 64, NSUM * 128), U32),
            pltpu.VMEM((4, 64, NSUM2 * 128), U32),
            pltpu.VMEM((H * DH // 2, DM), U32),
            pltpu.VMEM((NGRP, 64, NSUM * 128), U32),
            pltpu.VMEM((T1, FH, 128), F32),
            pltpu.VMEM((T1, 2 * (FH // RB) * 8, 128), F32),
            pltpu.VMEM((FH // 2, S), U32),
            pltpu.VMEM((NTILE // 2, FH // 4, 7 * 128), U32),
            pltpu.VMEM((64, 5 * S // 2), U32),
            pltpu.VMEM((64, FH), U32),
            pltpu.VMEM((96, H * DH), U32),
            pltpu.VMEM((80, H * DH), U32),
            pltpu.VMEM((80, H * DH), U32),
            pltpu.VMEM((32, H * DH), U32),
            pltpu.VMEM((4, 48, 80), F32),
            pltpu.VMEM((S, DM), BF16),
            pltpu.SemaphoreType.DMA((4,)),
            pltpu.SemaphoreType.DMA((8,)),
            pltpu.SemaphoreType.DMA((NTILE // T2,)),
            pltpu.SemaphoreType.DMA((NTILE // T2,)),
            pltpu.SemaphoreType.DMA,
        ],
        compiler_params=pltpu.CompilerParams(vmem_limit_bytes=112 * 1024 * 1024),
    )(
        A_x.reshape(S, DM),
        A_mem0.reshape(MEM, DM),
        A_Wq, A_Wk, A_Wv,
        A_Wo.reshape(H * DH, DM),
        B_w_in.T,
        B_w_sp,
        B_b_sp.reshape(16, 128),
        B_w_out,
    )
    return out.reshape(1, S, DM)
```
